```python
import jax
import jax.numpy as jnp

def _softmax(x, axis=-1):
    return jax.nn.softmax(x, axis=axis)

def _gelu(x):
    return jax.nn.gelu(x, approximate=True)

def _silu(x):
    return jax.nn.silu(x)

def _sigmoid(x):
    return jax.nn.sigmoid(x)

def _layernorm(x, axis=-1, eps=1e-05):
    m = jnp.mean(x, axis=axis, keepdims=True)
    v = jnp.var(x, axis=axis, keepdims=True)
    return (x - m) / jnp.sqrt(v + eps)

def _scatter_add(tgt, idx, src, axis=0):
    return tgt.at[idx].add(src)

def _segment_sum(src, seg, n):
    return jax.ops.segment_sum(src, seg, n)

class _Rng:

    def __init__(self, key):
        self._k = key

    def _next(self):
        self._k, sub = jax.random.split(self._k)
        return sub

    def normal(self, shape):
        return jax.random.normal(self._next(), shape, dtype=jnp.bfloat16)

    def randint(self, lo, hi, shape):
        return jax.random.randint(self._next(), shape, lo, hi, dtype=jnp.int32)

    def uniform(self, shape, lo=0.0, hi=1.0):
        return jax.random.uniform(self._next(), shape, jnp.bfloat16, lo, hi)

    def permutation(self, n):
        return jax.random.permutation(self._next(), n)
kernel_name = 'adaLN_cond__sliding_local_dilated__swiglu_ffn__prompt'

def setup_inputs():
    _rng = _Rng(jax.random.key(int.from_bytes(__import__("os").urandom(4), "little")))
    _w = lambda a: (lambda t: t.astype(jnp.bfloat16) if jnp.issubdtype(t.dtype, jnp.floating) else t)(jnp.asarray(a))

    def _A_setup():
        B, S, D = (1, 2048, 1024)
        return {'x': _w((lambda *s: _rng.normal(s) * 0.05)(B, S, D)), 'wqkv': _w((lambda *s: _rng.normal(s) * 0.05)(D, 3 * D)), 'wo': _w((lambda *s: _rng.normal(s) * 0.05)(D, D))}
    _A_in = _A_setup()

    def _B_setup():
        B, S, D, F = (1, 2048, 1024, 3584)
        return {'x': _w((lambda *s: _rng.normal(s) * 0.05)(B, S, D)), 'w_gate': _w((lambda *s: _rng.normal(s) * 0.05)(D, F)), 'w_up': _w((lambda *s: _rng.normal(s) * 0.05)(D, F)), 'w_down': _w((lambda *s: _rng.normal(s) * 0.05)(F, D))}
    _B_in = _B_setup()
    return {'A_x': _A_in['x'], 'A_wqkv': _A_in['wqkv'], 'A_wo': _A_in['wo'], 'B_x': _B_in['x'], 'B_w_gate': _B_in['w_gate'], 'B_w_up': _B_in['w_up'], 'B_w_down': _B_in['w_down'], 'c': _w((lambda *s: _rng.normal(s) * 0.05)(1, 1024)), 'w_mod': _w((lambda *s: _rng.normal(s) * 0.05)(1024, 6 * 1024) * 1024 ** (-0.5))}

def reference(A_x, A_wqkv, A_wo, B_x, B_w_gate, B_w_up, B_w_down, c, w_mod):

    def _A_ref(x, wqkv, wo):
        B, S, D = x.shape
        H = 32
        Dh = D // H
        W, dil = (8, 2)
        qkv = (lambda x, *d: x.transpose(*d))((x @ wqkv).reshape(B, S, 3, H, Dh), 2, 0, 3, 1, 4)
        q, k, v = (qkv[0], qkv[1], qkv[2])
        scale = Dh ** (-0.5)
        pos = jnp.arange(S)
        off = jnp.arange(W) * dil
        idx = pos[:, None] - off[None, :]
        mask = idx >= 0
        idx_c = jnp.where(mask, idx, 0).reshape(-1)
        kg = k[:, :, idx_c, :].reshape(B, H, S, W, Dh)
        vg = v[:, :, idx_c, :].reshape(B, H, S, W, Dh)
        logits = jnp.einsum('bhsd,bhswd->bhsw', q, kg) * scale
        logits = jnp.where(mask[None, None, :, :], logits, -1000000000.0)
        attn = _softmax(logits, axis=-1)
        o = jnp.einsum('bhsw,bhswd->bhsd', attn, vg)
        return (lambda x, *d: x.transpose(*d))(o, 0, 2, 1, 3).reshape(B, S, D) @ wo

    def _B_ref(x, w_gate, w_up, w_down):
        g = _silu(x @ w_gate)
        u = x @ w_up
        return g * u @ w_down
    x = A_x
    mod = (_silu(c) @ w_mod).reshape(c.shape[0], 6, 1, -1)
    sa, ca, ga, sb, cb, gb = (mod[:, 0].copy(), mod[:, 1].copy(), mod[:, 2].copy(), mod[:, 3].copy(), mod[:, 4].copy(), mod[:, 5].copy())
    h = _layernorm(x, axis=-1) * (1 + ca) + sa
    x = x + ga * _A_ref(h, A_wqkv, A_wo)
    h = _layernorm(x, axis=-1) * (1 + cb) + sb
    x = x + gb * _B_ref(h, B_w_gate, B_w_up, B_w_down)
    return x
```

```python
import jax
import jax.numpy as jnp
from jax import lax
from jax.experimental import pallas as pl
from jax.experimental.pallas import tpu as pltpu

S, D, F = 2048, 1024, 3584
DH, W = 32, 8
HG, GW = 4, 256
NJ = 8
TM1 = 512
TM = 512
FC = 512
EPS = 1e-5
F32, BF16, U32 = jnp.float32, jnp.bfloat16, jnp.uint32


def _dot(a, b):
    return jnp.dot(a, b, preferred_element_type=F32)


def _ln_mod(x, scale1, shift):
    m = jnp.mean(x, axis=-1, keepdims=True)
    xc = x - m
    v = jnp.mean(xc * xc, axis=-1, keepdims=True)
    return xc * lax.rsqrt(v + EPS) * scale1 + shift


def _unpack(w):
    lo = lax.bitcast_convert_type(w << 16, F32)
    hi = lax.bitcast_convert_type(w & jnp.uint32(0xFFFF0000), F32)
    return lo, hi


def _bf16_bits(x):
    return lax.bitcast_convert_type(x.astype(BF16).astype(F32), U32)


def _kernel(x_hbm, wqkv_hbm, wo_hbm, wg_hbm, wu_hbm, wd_hbm, c_ref, wmod_hbm, out_hbm,
            x_v, wqkv_v, wo_v, wg_v, wu_v, wd_v, wmod_v, h_v, qkv_v, t_v, q_s, k_s, v_s,
            ot_v, o_v, x1_v, a_v, ob_v, scol_v, mod_v, sem_x, sem_qkv, sem_mod, sem_w, sem_o):
    nb1 = S // TM1

    def x_cp(i):
        r = pl.ds(i * TM1, TM1)
        return pltpu.make_async_copy(x_hbm.at[r], x_v.at[r], sem_x.at[i])

    def qkv_cp(g, t):
        return pltpu.make_async_copy(wqkv_hbm.at[:, pl.ds(t * D + g * GW, GW)],
                                     wqkv_v.at[g, :, pl.ds(t * GW, GW)], sem_qkv.at[g * 3 + t])

    def mod_cp(i):
        return pltpu.make_async_copy(wmod_hbm.at[:, pl.ds(i * D, D)], wmod_v.at[i], sem_mod.at[i])

    w_cps = [pltpu.make_async_copy(s, d, sem_w.at[i]) for i, (s, d) in enumerate(
        ((wo_hbm, wo_v), (wg_hbm, wg_v), (wu_hbm, wu_v), (wd_hbm, wd_v)))]

    def out_cp(i, slot):
        return pltpu.make_async_copy(ob_v.at[slot], out_hbm.at[pl.ds(i * TM, TM)], sem_o.at[slot])

    first = [mod_cp(0), mod_cp(1), x_cp(0)] + [qkv_cp(0, t) for t in range(3)]
    first += [x_cp(i) for i in range(1, nb1)]
    for cp in first:
        cp.start()

    cf = c_ref[...].astype(F32)
    sc = (cf * jax.nn.sigmoid(cf)).astype(BF16)
    scol_v[...] = jnp.broadcast_to(sc.astype(F32), (128, D)).T
    sc8 = jnp.broadcast_to(sc, (16, D))
    for i in range(2):
        mod_cp(i).wait()
        mod_v[i] = _dot(sc8, wmod_v[i])[:8]

    def mod_vpu(i):
        for n in range(D // 128):
            cs = pl.ds(n * 128, 128)
            p = wmod_v[i, :, cs].astype(F32) * scol_v[...]
            mod_v[i, :, cs] = jnp.broadcast_to(jnp.sum(p, axis=0, keepdims=True), (8, 128))

    def mod_row(i):
        return mod_v[i, pl.ds(0, 1), :]

    def proj(g, i):
        r = pl.ds(pl.multiple_of(i * TM1, TM1), TM1)
        y = _dot(h_v[r, :], wqkv_v[g]).astype(BF16)
        for n in range(6):
            qkv_v[(g % 2) * 6 + n, r, :] = y[:, n * 128:(n + 1) * 128]

    def att_load(g):
        for t, dst in enumerate((q_s, k_s, v_s)):
            for n in range(2):
                src = qkv_v.at[(g % 2) * 6 + t * 2 + n].bitcast(U32)
                for j in range(NJ):
                    t_v[t * NJ + j, pl.ds(n * 128, 128), :] = src[pl.ds(j, 128, stride=NJ), :].T
            for j in range(NJ):
                for d in range(DH):
                    w = t_v[t * NJ + j, pl.ds(d, 8, stride=DH), :]
                    rows = pl.ds(d * 8, 8)
                    base = 0 if t == 0 else NJ - 1
                    dst[0, base + j, rows, :], dst[1, base + j, rows, :] = _unpack(w)
                    if t > 0 and j > 0:
                        dst[0, j - 1, rows, :], dst[1, j - 1, rows, :] = _unpack(pltpu.roll(w, 1, 1))

    def att_core(j):
        lane0 = lax.broadcasted_iota(jnp.int32, (8, 128), 1) == 0
        probs = []
        for p in range(2):
            acc = [None] * W
            for d in range(DH):
                rows = pl.ds(d * 8, 8)
                q = q_s[p, j, rows, :]
                for w in range(W):
                    t = q * k_s[p, j + (NJ - 1 - w), rows, :]
                    acc[w] = t if d == 0 else acc[w] + t
            lg = [acc[0] * DH ** -0.5]
            for w in range(1, W):
                lg.append(jnp.where(jnp.logical_and(lane0, j < w), -1e9, acc[w] * DH ** -0.5))
            m = lg[0]
            for w in range(1, W):
                m = jnp.maximum(m, lg[w])
            e = [jnp.exp(l - m) for l in lg]
            den = e[0]
            for w in range(1, W):
                den = den + e[w]
            inv = 1.0 / den
            probs.append([x * inv for x in e])
        for d in range(DH):
            rows = pl.ds(d * 8, 8)
            o = []
            for p in range(2):
                acc = probs[p][0] * v_s[p, j + NJ - 1, rows, :]
                for w in range(1, W):
                    acc = acc + probs[p][w] * v_s[p, j + (NJ - 1 - w), rows, :]
                o.append(_bf16_bits(acc))
            ot_v[j, pl.ds(d, 8, stride=DH), :] = (o[0] >> 16) | o[1]

    def att_store(g):
        for n in range(2):
            dst = o_v.at[g * 2 + n].bitcast(U32)
            for j in range(NJ):
                dst[pl.ds(j, 128, stride=NJ), :] = ot_v[j, pl.ds(n * 128, 128), :].T

    def o_cols(r, g0, g1):
        return jnp.concatenate([o_v[n, r, :] for n in range(2 * g0, 2 * g1)], axis=1)

    for t in range(3):
        qkv_cp(0, t).wait()
    rest = [qkv_cp(g, t) for g in range(1, HG) for t in range(3)]
    rest += [mod_cp(i) for i in range(2, 6)] + w_cps
    for cp in rest:
        cp.start()

    def first_body(i, carry):
        x_cp(i).wait()
        r = pl.ds(pl.multiple_of(i * TM1, TM1), TM1)
        h_v[r, :] = _ln_mod(x_v[r, :].astype(F32), 1.0 + mod_row(1), mod_row(0)).astype(BF16)
        proj(0, i)
        return carry
    lax.fori_loop(0, nb1, first_body, 0)

    jpb = NJ // nb1

    def group_body(g, carry):
        for t in range(3):
            qkv_cp(g, t).wait()
        mod_cp(g + 1).wait()
        att_load(g - 1)
        mod_vpu(g + 1)

        def body(i, c):
            proj(g, i)
            for jj in range(jpb):
                att_core(i * jpb + jj)
            return c
        lax.fori_loop(0, nb1, body, 0)
        att_store(g - 1)
        return carry
    lax.fori_loop(1, HG, group_body, 0)

    mod_cp(5).wait()
    w_cps[0].wait()
    att_load(HG - 1)
    mod_vpu(5)

    def wo_body(i, c):
        r = pl.ds(pl.multiple_of(i * TM1, TM1), TM1)
        x1_v[r, :] = _dot(o_cols(r, 0, HG - 1), wo_v[pl.ds(0, (HG - 1) * GW), :])
        for jj in range(jpb):
            att_core(i * jpb + jj)
        return c
    lax.fori_loop(0, nb1, wo_body, 0)
    att_store(HG - 1)
    for cp in w_cps[1:]:
        cp.wait()

    def ffn_body(i, c):
        r = pl.ds(pl.multiple_of(i * TM, TM), TM)
        slot = i % 2
        y = x1_v[r, :] + _dot(o_cols(r, HG - 1, HG), wo_v[pl.ds((HG - 1) * GW, GW), :])
        x1 = x_v[r, :].astype(F32) + mod_row(2) * y
        x1_v[r, :] = x1
        h = _ln_mod(x1, 1.0 + mod_row(4), mod_row(3)).astype(BF16)
        for f in range(F // FC):
            cs = pl.ds(f * FC, FC)
            gate = _dot(h, wg_v[:, cs])
            up = _dot(h, wu_v[:, cs])
            a_v[:, cs] = (gate * jax.nn.sigmoid(gate) * up).astype(BF16)

        @pl.when(i >= 2)
        def _():
            out_cp(i - 2, slot).wait()
        ob_v[slot] = (x1_v[r, :] + mod_row(5) * _dot(a_v[...], wd_v[...])).astype(BF16)
        out_cp(i, slot).start()
        return c
    nb = S // TM
    lax.fori_loop(0, nb, ffn_body, 0)
    for i in range(nb - 2, nb):
        out_cp(i, i % 2).wait()


@jax.jit
def pallas_adaLN_cond__sliding_local_dilated__swiglu_ffn__prompt_kernel(
    A_x: jax.Array,
    A_wqkv: jax.Array,
    A_wo: jax.Array,
    B_x: jax.Array,
    B_w_gate: jax.Array,
    B_w_up: jax.Array,
    B_w_down: jax.Array,
    c: jax.Array,
    w_mod: jax.Array,
):
    del B_x
    hbm = pl.BlockSpec(memory_space=pl.ANY)
    dma = pltpu.SemaphoreType.DMA
    out = pl.pallas_call(
        _kernel,
        out_shape=jax.ShapeDtypeStruct((S, D), BF16),
        in_specs=[hbm] * 6 + [pl.BlockSpec(memory_space=pltpu.VMEM), hbm],
        out_specs=hbm,
        scratch_shapes=[
            pltpu.VMEM((S, D), BF16),
            pltpu.VMEM((HG, D, 3 * GW), BF16),
            pltpu.VMEM((D, D), BF16),
            pltpu.VMEM((D, F), BF16),
            pltpu.VMEM((D, F), BF16),
            pltpu.VMEM((F, D), BF16),
            pltpu.VMEM((6, D, D), BF16),
            pltpu.VMEM((S, D), BF16),
            pltpu.VMEM((2 * 6, S, 128), BF16),
            pltpu.VMEM((3 * NJ, GW, 128), U32),
            pltpu.VMEM((2, NJ, GW, 128), F32),
            pltpu.VMEM((2, 2 * NJ - 1, GW, 128), F32),
            pltpu.VMEM((2, 2 * NJ - 1, GW, 128), F32),
            pltpu.VMEM((NJ, GW, 128), U32),
            pltpu.VMEM((2 * HG, S, 128), BF16),
            pltpu.VMEM((S, D), F32),
            pltpu.VMEM((TM, F), BF16),
            pltpu.VMEM((2, TM, D), BF16),
            pltpu.VMEM((D, 128), F32),
            pltpu.VMEM((6, 8, D), F32),
            dma((S // TM1,)), dma((HG * 3,)), dma((6,)), dma((4,)), dma((2,)),
        ],
        compiler_params=pltpu.CompilerParams(vmem_limit_bytes=120 * 1024 * 1024),
    )(A_x.reshape(S, D), A_wqkv, A_wo, B_w_gate, B_w_up, B_w_down, c, w_mod)
    return out.reshape(1, S, D)
```

```python
import jax
import jax.numpy as jnp
from jax import lax
from jax.experimental import pallas as pl
from jax.experimental.pallas import tpu as pltpu

S, D, F = 2048, 1024, 3584
DH, W = 32, 8
HG, GW = 4, 256
NJ = 8
TM1 = 256
TM = 512
FC = 512
DC = 512
LB = TM * DC // D
HP = 36
EPS = 1e-5
F32, BF16, U32 = jnp.float32, jnp.bfloat16, jnp.uint32


def _dot(a, b):
    return jnp.dot(a, b, preferred_element_type=F32)


def _ln_mod(x, scale1, shift):
    m = jnp.mean(x, axis=-1, keepdims=True)
    xc = x - m
    v = jnp.mean(xc * xc, axis=-1, keepdims=True)
    return xc * lax.rsqrt(v + EPS) * scale1 + shift


def _unpack(w):
    lo = lax.bitcast_convert_type(w << 16, F32)
    hi = lax.bitcast_convert_type(w & jnp.uint32(0xFFFF0000), F32)
    return lo, hi


def _ld(ref, r):
    return pltpu.bitcast(ref[r, :], BF16)


def _bf16_bits(x):
    return lax.bitcast_convert_type(x.astype(BF16).astype(F32), U32)


def _kernel(x_hbm, wqkv_hbm, wo_hbm, wg_hbm, wu_hbm, wd_hbm, c_ref, wmod_hbm, out_hbm,
            x_v, wqkv_v, wo_v, wg_v, wu_v, wd_v, wmod_v, h_v, qkv_v, t_v, q_s, k_s, v_s,
            ot_v, o_v, x1_v, a_v, ob_v, scol_v, mod_v, sem_x, sem_qkv, sem_mod, sem_w, sem_o):
    nb1 = S // TM1

    def x_cp(i):
        r = pl.ds(i * TM1, TM1)
        return pltpu.make_async_copy(x_hbm.at[r], x_v.at[r], sem_x.at[i])

    def qkv_cp(g, t):
        return pltpu.make_async_copy(wqkv_hbm.at[:, pl.ds(t * D + g * GW, GW)],
                                     wqkv_v.at[g, :, pl.ds(t * GW, GW)], sem_qkv.at[g * 3 + t])

    def mod_cp(i):
        return pltpu.make_async_copy(wmod_hbm.at[:, pl.ds(i * D, D)], wmod_v.at[i], sem_mod.at[i])

    w_cps = [pltpu.make_async_copy(s, d, sem_w.at[i]) for i, (s, d) in enumerate(
        ((wo_hbm, wo_v), (wg_hbm, wg_v), (wu_hbm, wu_v), (wd_hbm, wd_v)))]

    def out_cp(i, slot):
        return pltpu.make_async_copy(ob_v.at[slot], out_hbm.at[pl.ds(i * TM, TM)], sem_o.at[slot])

    first = [mod_cp(0), mod_cp(1), x_cp(0)] + [qkv_cp(0, t) for t in range(3)]
    first += [x_cp(i) for i in range(1, nb1)]
    for cp in first:
        cp.start()

    cf = c_ref[...].astype(F32)
    sc = (cf * jax.nn.sigmoid(cf)).astype(BF16)
    scol_v[...] = jnp.broadcast_to(sc.astype(F32), (128, D)).T
    sc8 = jnp.broadcast_to(sc, (16, D))
    for i in range(2):
        mod_cp(i).wait()
        mod_v[i] = _dot(sc8, wmod_v[i])[:8]

    def mod_vpu(i, n):
        cs = pl.ds(pl.multiple_of(n * 128, 128), 128)
        p = wmod_v[i, :, cs].astype(F32) * scol_v[...]
        mod_v[i, :, cs] = jnp.broadcast_to(jnp.sum(p, axis=0, keepdims=True), (8, 128))

    def mod_row(i):
        return mod_v[i, pl.ds(0, 1), :]

    def rows(i, n):
        return pl.ds(pl.multiple_of(i * n, n), n)

    def proj(g, i):
        h = _ld(h_v, rows(i, TM1 // 2))
        for t in range(3):
            y = _dot(h, wqkv_v[g, :, pl.ds(t * GW, GW)])
            y = pltpu.bitcast(y.astype(BF16), U32)
            for n in range(2):
                qkv_v[(g % 2) * 6 + t * 2 + n, rows(i, TM1 // 2), :] = y[:, n * 128:(n + 1) * 128]

    def att_load(g, j):
        for t, dst in enumerate((q_s, k_s, v_s)):
            for n in range(2):
                w = qkv_v[(g % 2) * 6 + t * 2 + n, pl.ds(j, 128, stride=NJ), :]
                wt = w.T
                for h in range(4):
                    t_v[t, pl.ds((n * 4 + h) * HP, DH), :] = wt[h * DH:(h + 1) * DH]
            for d in range(DH):
                w = t_v[t, pl.ds(d, 8, stride=HP), :]
                r = pl.ds(d * 8, 8)
                if t == 0:
                    dst[0, j, r, :], dst[1, j, r, :] = _unpack(w)
                else:
                    dst[0, NJ + j, r, :], dst[1, NJ + j, r, :] = _unpack(w)
                    dst[0, j, r, :], dst[1, j, r, :] = _unpack(pltpu.roll(w, 1, 1))

    def att_core(g, j):
        lane0 = lax.broadcasted_iota(jnp.int32, (8, 128), 1) == 0
        probs = []
        for p in range(2):
            acc = [None] * W
            for d in range(DH):
                r = pl.ds(d * 8, 8)
                q = q_s[p, j, r, :]
                for w in range(W):
                    t = q * k_s[p, j + (NJ - w), r, :]
                    acc[w] = t if d == 0 else acc[w] + t
            lg = [acc[0] * DH ** -0.5]
            for w in range(1, W):
                lg.append(jnp.where(jnp.logical_and(lane0, j < w), -1e9, acc[w] * DH ** -0.5))
            m = lg[0]
            for w in range(1, W):
                m = jnp.maximum(m, lg[w])
            e = [jnp.exp(l - m) for l in lg]
            den = e[0]
            for w in range(1, W):
                den = den + e[w]
            inv = 1.0 / den
            probs.append([x * inv for x in e])
        for d in range(DH):
            r = pl.ds(d * 8, 8)
            o = []
            for p in range(2):
                acc = probs[p][0] * v_s[p, j + NJ, r, :]
                for w in range(1, W):
                    acc = acc + probs[p][w] * v_s[p, j + (NJ - w), r, :]
                o.append(_bf16_bits(acc))
            ot_v[pl.ds(d, 8, stride=HP), :] = (o[0] >> 16) | o[1]
        for n in range(2):
            ot = jnp.concatenate([ot_v[pl.ds((n * 4 + h) * HP, DH), :] for h in range(4)], axis=0)
            o_v[g * 2 + n, pl.ds(j, 128, stride=NJ), :] = ot.T

    def o_cols(r, g0, g1):
        return jnp.concatenate([_ld(o_v.at[n], r) for n in range(2 * g0, 2 * g1)], axis=1)

    def ln1(i):
        h = _ln_mod(x_v[rows(i, TM1), :].astype(F32), 1.0 + mod_row(1), mod_row(0))
        h_v[rows(i, TM1 // 2), :] = pltpu.bitcast(h.astype(BF16), U32)

    def ln2(i):
        r = rows(i, LB)
        y = x1_v[r, :] + _dot(o_cols(rows(i, LB // 2), HG - 1, HG), wo_v[pl.ds((HG - 1) * GW, GW), :])
        x1 = x_v[r, :].astype(F32) + mod_row(2) * y
        x1_v[r, :] = x1
        h = _ln_mod(x1, 1.0 + mod_row(4), mod_row(3))
        h_v[rows(i, LB // 2), :] = pltpu.bitcast(h.astype(BF16), U32)

    rest = [qkv_cp(g, t) for g in range(1, HG) for t in range(3)]
    rest += [mod_cp(i) for i in range(2, 6)] + w_cps
    x_cp(0).wait()
    ln1(0)
    for t in range(3):
        qkv_cp(0, t).wait()
    for cp in rest:
        cp.start()

    def first_body(i, carry):
        x_cp(i + 1).wait()
        proj(0, i)
        ln1(i + 1)
        return carry
    lax.fori_loop(0, nb1 - 1, first_body, 0)
    proj(0, nb1 - 1)

    half = nb1 // 2
    jpb = NJ // half

    def group_body(g, carry):
        for t in range(3):
            qkv_cp(g, t).wait()
        mod_cp(g + 1).wait()

        def body_a(i, c):
            proj(g, i)
            for jj in range(jpb):
                att_load(g - 1, i * jpb + jj)
                mod_vpu(g + 1, i * jpb + jj)
            return c
        lax.fori_loop(0, half, body_a, 0)

        def body_b(i, c):
            proj(g, half + i)
            for jj in range(jpb):
                att_core(g - 1, i * jpb + jj)
            return c
        lax.fori_loop(0, half, body_b, 0)
        return carry
    lax.fori_loop(1, HG, group_body, 0)

    mod_cp(5).wait()
    w_cps[0].wait()

    def wo_part(i):
        x1_v[rows(i, TM1), :] = _dot(o_cols(rows(i, TM1 // 2), 0, HG - 1), wo_v[pl.ds(0, (HG - 1) * GW), :])

    def wo_a(i, c):
        wo_part(i)
        for jj in range(jpb):
            att_load(HG - 1, i * jpb + jj)
            mod_vpu(5, i * jpb + jj)
        return c
    lax.fori_loop(0, half, wo_a, 0)

    def wo_b(i, c):
        wo_part(half + i)
        for jj in range(jpb):
            att_core(HG - 1, i * jpb + jj)
        return c
    lax.fori_loop(0, half, wo_b, 0)
    for cp in w_cps[1:]:
        cp.wait()

    nb, nd = S // TM, D // DC
    lax.fori_loop(0, nd, lambda n, c: ln2(n), None)

    def ffn_body(i, c):
        r = rows(i, TM)
        slot = i % 2

        def gu(f, c2):
            cs = rows(f, FC)
            h = _ld(h_v, rows(i, TM // 2))
            gate = _dot(h, wg_v[:, cs])
            up = _dot(h, wu_v[:, cs])
            a_v[:, cs] = pltpu.bitcast((gate * jax.nn.sigmoid(gate) * up).astype(BF16), U32)
            return c2
        lax.fori_loop(0, F // FC, gu, 0)

        @pl.when(i >= 2)
        def _():
            out_cp(i - 2, slot).wait()

        def dn(n, with_ln):
            cs = rows(n, DC)
            y2 = _dot(_ld(a_v, slice(None)), wd_v[:, cs])
            ob_v[slot, :, cs] = (x1_v[r, cs] + mod_v[5, pl.ds(0, 1), cs] * y2).astype(BF16)
            if with_ln:
                ln2((i + 1) * nd + n)

        @pl.when(i < nb - 1)
        def _():
            lax.fori_loop(0, nd, lambda n, c2: dn(n, True), None)

        @pl.when(i == nb - 1)
        def _():
            lax.fori_loop(0, nd, lambda n, c2: dn(n, False), None)
        out_cp(i, slot).start()
        return c
    lax.fori_loop(0, nb, ffn_body, 0)
    for i in range(nb - 2, nb):
        out_cp(i, i % 2).wait()


@jax.jit
def pallas_adaLN_cond__sliding_local_dilated__swiglu_ffn__prompt_kernel(
    A_x: jax.Array,
    A_wqkv: jax.Array,
    A_wo: jax.Array,
    B_x: jax.Array,
    B_w_gate: jax.Array,
    B_w_up: jax.Array,
    B_w_down: jax.Array,
    c: jax.Array,
    w_mod: jax.Array,
):
    del B_x
    hbm = pl.BlockSpec(memory_space=pl.ANY)
    dma = pltpu.SemaphoreType.DMA
    out = pl.pallas_call(
        _kernel,
        out_shape=jax.ShapeDtypeStruct((S, D), BF16),
        in_specs=[hbm] * 6 + [pl.BlockSpec(memory_space=pltpu.VMEM), hbm],
        out_specs=hbm,
        scratch_shapes=[
            pltpu.VMEM((S, D), BF16),
            pltpu.VMEM((HG, D, 3 * GW), BF16),
            pltpu.VMEM((D, D), BF16),
            pltpu.VMEM((D, F), BF16),
            pltpu.VMEM((D, F), BF16),
            pltpu.VMEM((F, D), BF16),
            pltpu.VMEM((6, D, D), BF16),
            pltpu.VMEM((S // 2, D), U32),
            pltpu.VMEM((2 * 6, S // 2, 128), U32),
            pltpu.VMEM((3, 8 * HP, 128), U32),
            pltpu.VMEM((2, NJ, GW, 128), F32),
            pltpu.VMEM((2, 2 * NJ, GW, 128), F32),
            pltpu.VMEM((2, 2 * NJ, GW, 128), F32),
            pltpu.VMEM((8 * HP, 128), U32),
            pltpu.VMEM((2 * HG, S // 2, 128), U32),
            pltpu.VMEM((S, D), F32),
            pltpu.VMEM((TM // 2, F), U32),
            pltpu.VMEM((2, TM, D), BF16),
            pltpu.VMEM((D, 128), F32),
            pltpu.VMEM((6, 8, D), F32),
            dma((S // TM1,)), dma((HG * 3,)), dma((6,)), dma((4,)), dma((2,)),
        ],
        compiler_params=pltpu.CompilerParams(vmem_limit_bytes=120 * 1024 * 1024),
    )(A_x.reshape(S, D), A_wqkv, A_wo, B_w_gate, B_w_up, B_w_down, c, w_mod)
    return out.reshape(1, S, D)
```

```python
import jax
import jax.numpy as jnp
from jax import lax
from jax.experimental import pallas as pl
from jax.experimental.pallas import tpu as pltpu

S, D, F = 2048, 1024, 3584
DH, W = 32, 8
HG, GW = 4, 256
NJ = 8
TM1 = 256
TM = 512
FC = 512
DC = 256
LB = TM * DC // D
HP = 36
CFG_G = (((2, 2), 1), ((2, 2), 1))
CFG_W = (((2, 2), 1), ((2, 2), 1))
MC = 512
AHEAD = 5
EPS = 1e-5
F32, BF16, U32 = jnp.float32, jnp.bfloat16, jnp.uint32


def _dot(a, b):
    return jnp.dot(a, b, preferred_element_type=F32)


def _ln_mod(x, scale1, shift):
    m = jnp.mean(x, axis=-1, keepdims=True)
    xc = x - m
    v = jnp.mean(xc * xc, axis=-1, keepdims=True)
    return xc * lax.rsqrt(v + EPS) * scale1 + shift


def _unpack(w):
    lo = lax.bitcast_convert_type(w << 16, F32)
    hi = lax.bitcast_convert_type(w & jnp.uint32(0xFFFF0000), F32)
    return lo, hi


def _ld(ref, r):
    return pltpu.bitcast(ref[r, :], BF16)


def _mix(a, na=1, b=(), nb=0):
    b = iter(b)
    done = 0
    for k, _ in enumerate(a):
        while done * na < (k + 1) * nb:
            next(b)
            done += 1
    for _ in b:
        pass


def _bf16_bits(x):
    return lax.bitcast_convert_type(x.astype(BF16).astype(F32), U32)


def _kernel(x_hbm, wqkv_hbm, wo_hbm, wg_hbm, wu_hbm, wd_hbm, c_ref, wmod_hbm, out_hbm,
            x_v, wqkv_v, wo_v, wg_v, wu_v, wd_v, wmod_v, h_v, qkv0_v, qkv1_v, t_v, q_s, k_s, v_s,
            ot_v, o_v, o3_v, x1_v, a_v, ob_v, scol_v, mod_v, sem_x, sem_qkv, sem_mod, sem_head, sem_w, sem_o):
    nb1 = S // TM1
    qkv_v = (qkv0_v, qkv1_v)

    def x_cp(i):
        r = pl.ds(i * TM1, TM1)
        return pltpu.make_async_copy(x_hbm.at[r], x_v.at[r], sem_x.at[i])

    def qkv_cp(g, t):
        return pltpu.make_async_copy(wqkv_hbm.at[:, pl.ds(t * D + g * GW, GW)],
                                     wqkv_v.at[g, :, pl.ds(t * GW, GW)], sem_qkv.at[g * 3 + t])

    def mod_cp(i):
        return pltpu.make_async_copy(wmod_hbm.at[:, pl.ds(i * D, D)], wmod_v.at[i], sem_mod.at[i])

    def mod_head_cp(i):
        return pltpu.make_async_copy(wmod_hbm.at[:, pl.ds(i * MC, MC)],
                                     wmod_v.at[i * MC // D, :, pl.ds(i * MC % D, MC)], sem_head.at[i])

    w_cps = [pltpu.make_async_copy(s, d, sem_w.at[i]) for i, (s, d) in enumerate(
        ((wo_hbm, wo_v), (wg_hbm, wg_v), (wu_hbm, wu_v), (wd_hbm, wd_v)))]

    def out_cp(i, slot):
        return pltpu.make_async_copy(ob_v.at[slot], out_hbm.at[pl.ds(i * TM, TM)], sem_o.at[slot])

    nm = 2 * D // MC
    head = [mod_head_cp(i) for i in range(nm)] + [x_cp(0)] + [qkv_cp(0, t) for t in range(3)]
    head += [x_cp(i) for i in range(1, nb1)]
    for cp in head[:AHEAD]:
        cp.start()

    cf = c_ref[...].astype(F32)
    sc = (cf * jax.nn.sigmoid(cf)).astype(BF16)
    scol_v[...] = jnp.broadcast_to(sc.astype(F32), (128, D)).T
    sc8 = jnp.broadcast_to(sc, (16, D))
    for i in range(nm):
        mod_head_cp(i).wait()
        for cp in head[AHEAD + i:AHEAD + i + 1] if i + 1 < nm else head[AHEAD + i:]:
            cp.start()
        cs = pl.ds(i * MC % D, MC)
        mod_v[i * MC // D, :, cs] = _dot(sc8, wmod_v[i * MC // D, :, cs])[:8]

    def mod_vpu(i, n):
        cs = pl.ds(pl.multiple_of(n * 128, 128), 128)
        p = wmod_v[i, :, cs].astype(F32) * scol_v[...]
        mod_v[i, :, cs] = jnp.broadcast_to(jnp.sum(p, axis=0, keepdims=True), (8, 128))
        yield

    def mod_row(i):
        return mod_v[i, pl.ds(0, 1), :]

    def rows(i, n):
        return pl.ds(pl.multiple_of(i * n, n), n)

    def proj(g, i):
        for t in range(3):
            y = _dot(_ld(h_v, rows(i, TM1 // 2)), wqkv_v[g, :, pl.ds(t * GW, GW)])
            y = pltpu.bitcast(y.astype(BF16), U32)
            for n in range(2):
                qkv_v[g % 2][t * 2 + n, rows(i, TM1 // 2), :] = y[:, n * 128:(n + 1) * 128]
            yield

    def att_load(g, j, u):
        for t, dst in enumerate((q_s, k_s, v_s)):
            for n in range(2):
                w = qkv_v[g % 2][t * 2 + n, pl.ds(j, 128, stride=NJ), :]
                wt = w.T
                for h in range(4):
                    t_v[u * 3 + t, pl.ds((n * 4 + h) * HP, DH), :] = wt[h * DH:(h + 1) * DH]
            for d in range(DH):
                w = t_v[u * 3 + t, pl.ds(d, 8, stride=HP), :]
                r = pl.ds(d * 8, 8)
                if t == 0:
                    dst[0, j, r, :], dst[1, j, r, :] = _unpack(w)
                else:
                    dst[0, NJ + j, r, :], dst[1, NJ + j, r, :] = _unpack(w)
                    dst[0, j, r, :], dst[1, j, r, :] = _unpack(pltpu.roll(w, 1, 1))
            yield

    def att_core(g, j, u, last, qws, ch):
        lane0 = lax.broadcasted_iota(jnp.int32, (8, 128), 1) == 0
        probs = []
        for p in range(2):
            acc = [None] * W
            qw = qws[p]
            for w0 in range(0, W, qw):
                for d in range(DH):
                    r = pl.ds(d * 8, 8)
                    q = q_s[p, j, r, :]
                    if d == 0 and dep[0] is not None:
                        q = jnp.where(j < 0, dep[0], q)
                    for w in range(w0, w0 + qw):
                        t = q * k_s[p, j + (NJ - w), r, :]
                        acc[w] = t if d == 0 else acc[w] + t
                dep[0] = acc[w0]
            lg = [acc[0] * DH ** -0.5]
            for w in range(1, W):
                lg.append(jnp.where(jnp.logical_and(lane0, j < w), -1e9, acc[w] * DH ** -0.5))
            m = lg[0]
            for w in range(1, W):
                m = jnp.maximum(m, lg[w])
            e = [jnp.exp(l - m) for l in lg]
            den = e[0]
            for w in range(1, W):
                den = den + e[w]
            inv = 1.0 / den
            probs.append([x * inv for x in e])
            dep[0] = inv
            yield
        for d in range(DH):
            r = pl.ds(d * 8, 8)
            o = []
            for p in range(2):
                acc = probs[p][0] * v_s[p, j + NJ, r, :]
                for w in range(1, W):
                    acc = acc + probs[p][w] * v_s[p, j + (NJ - w), r, :]
                o.append(_bf16_bits(acc))
                if d % ch == ch - 1:
                    probs[p][0] = jnp.where(j < 0, acc, probs[p][0])
                    dep[0] = acc
            ot_v[u, pl.ds(d, 8, stride=HP), :] = (o[0] >> 16) | o[1]
        for n in range(2):
            ot = jnp.concatenate([ot_v[u, pl.ds((n * 4 + h) * HP, DH), :] for h in range(4)], axis=0)
            dst, base = (o_v, g * 2) if last is None else (last, 0)
            dst[base + n, pl.ds(j, 128, stride=NJ), :] = ot.T
        yield

    def o_cols(ref, r):
        return jnp.concatenate([_ld(ref.at[n], r) for n in range(ref.shape[0])], axis=1)

    def ln1(i):
        h = _ln_mod(x_v[rows(i, TM1), :].astype(F32), 1.0 + mod_row(1), mod_row(0))
        h_v[rows(i, TM1 // 2), :] = pltpu.bitcast(h.astype(BF16), U32)

    def ln2(i):
        r = rows(i, LB)
        y = x1_v[r, :] + _dot(o_cols(o3_v, rows(i, LB // 2)), wo_v[pl.ds((HG - 1) * GW, GW), :])
        x1 = x_v[r, :].astype(F32) + mod_row(2) * y
        x1_v[r, :] = x1
        h = _ln_mod(x1, 1.0 + mod_row(4), mod_row(3))
        h_v[rows(i, LB // 2), :] = pltpu.bitcast(h.astype(BF16), U32)

    def prefetch(g):
        nxt = [qkv_cp(g + 1, t) for t in range(3)] if g + 1 < HG else []
        for cp in nxt + [mod_cp(g + 2), w_cps[(g + 1) % HG]]:
            cp.start()

    x_cp(0).wait()
    ln1(0)
    qkv_cp(0, 0).wait()
    for t, _ in enumerate(proj(0, 0)):
        if t < 2:
            qkv_cp(0, t + 1).wait()
    x_cp(1).wait()
    ln1(1)
    prefetch(0)

    def first_body(i, carry):
        x_cp(i + 1).wait()
        _mix(proj(0, i))
        ln1(i + 1)
        return carry
    lax.fori_loop(1, nb1 - 1, first_body, 0)
    _mix(proj(0, nb1 - 1))

    half = nb1 // 2
    jpb = NJ // half

    def loads(g, i):
        for u in range(jpb):
            yield from att_load(g, i * jpb + u, u)
            yield from mod_vpu(g + 2, i * jpb + u)

    dep = [None]

    def cores(g, i, last, cfg):
        dep[0] = None
        for u in range(jpb):
            yield from att_core(g, i * jpb + u, u, last, *cfg[u])

    for g in range(1, HG):
        for t in range(3):
            qkv_cp(g, t).wait()
        mod_cp(g + 1).wait()
        prefetch(g)

        def body_a(i, c, g=g):
            _mix(proj(g, i), 3, loads(g - 1, i), 8)
            return c
        lax.fori_loop(0, half, body_a, 0)

        def body_b(i, c, g=g):
            _mix(proj(g, half + i), 3, cores(g - 1, i, None, CFG_G), 6)
            return c
        lax.fori_loop(0, half, body_b, 0)

    mod_cp(5).wait()
    w_cps[0].wait()

    def wo_part(i):
        for n in range(D // GW):
            o = o_cols(o_v, rows(i, TM1 // 2))
            cs = pl.ds(n * GW, GW)
            x1_v[rows(i, TM1), cs] = _dot(o, wo_v[pl.ds(0, (HG - 1) * GW), cs])
            yield

    def wo_a(i, c):
        _mix(wo_part(i), 4, loads(HG - 1, i), 8)
        return c
    lax.fori_loop(0, half, wo_a, 0)

    def wo_b(i, c):
        _mix(wo_part(half + i), 4, cores(HG - 1, i, o3_v, CFG_W), 6)
        return c
    lax.fori_loop(0, half, wo_b, 0)
    for cp in w_cps[1:]:
        cp.wait()

    nb, nd = S // TM, D // DC
    lax.fori_loop(0, nd, lambda n, c: ln2(n), None)

    def ffn_body(i, c):
        r = rows(i, TM)
        slot = i % 2

        def gu(f, c2):
            cs = rows(f, FC)
            h = _ld(h_v, rows(i, TM // 2))
            gate = _dot(h, wg_v[:, cs])
            up = _dot(h, wu_v[:, cs])
            a_v[:, cs] = pltpu.bitcast((gate * jax.nn.sigmoid(gate) * up).astype(BF16), U32)
            return c2
        lax.fori_loop(0, F // FC, gu, 0)

        @pl.when(i >= 2)
        def _():
            out_cp(i - 2, slot).wait()

        def dn(n, with_ln):
            if with_ln:
                ln2((i + 1) * nd + n)
            cs = rows(n, DC)
            y2 = _dot(_ld(a_v, slice(None)), wd_v[:, cs])
            ob_v[slot, :, cs] = (x1_v[r, cs] + mod_v[5, pl.ds(0, 1), cs] * y2).astype(BF16)

        @pl.when(i < nb - 1)
        def _():
            lax.fori_loop(0, nd, lambda n, c2: dn(n, True), None)

        @pl.when(i == nb - 1)
        def _():
            lax.fori_loop(0, nd, lambda n, c2: dn(n, False), None)
        out_cp(i, slot).start()
        return c
    lax.fori_loop(0, nb, ffn_body, 0)
    for i in range(nb - 2, nb):
        out_cp(i, i % 2).wait()


@jax.jit
def pallas_adaLN_cond__sliding_local_dilated__swiglu_ffn__prompt_kernel(
    A_x: jax.Array,
    A_wqkv: jax.Array,
    A_wo: jax.Array,
    B_x: jax.Array,
    B_w_gate: jax.Array,
    B_w_up: jax.Array,
    B_w_down: jax.Array,
    c: jax.Array,
    w_mod: jax.Array,
):
    del B_x
    hbm = pl.BlockSpec(memory_space=pl.ANY)
    dma = pltpu.SemaphoreType.DMA
    out = pl.pallas_call(
        _kernel,
        out_shape=jax.ShapeDtypeStruct((S, D), BF16),
        in_specs=[hbm] * 6 + [pl.BlockSpec(memory_space=pltpu.VMEM), hbm],
        out_specs=hbm,
        scratch_shapes=[
            pltpu.VMEM((S, D), BF16),
            pltpu.VMEM((HG, D, 3 * GW), BF16),
            pltpu.VMEM((D, D), BF16),
            pltpu.VMEM((D, F), BF16),
            pltpu.VMEM((D, F), BF16),
            pltpu.VMEM((F, D), BF16),
            pltpu.VMEM((6, D, D), BF16),
            pltpu.VMEM((S // 2, D), U32),
            pltpu.VMEM((6, S // 2, 128), U32),
            pltpu.VMEM((6, S // 2, 128), U32),
            pltpu.VMEM((6, 8 * HP, 128), U32),
            pltpu.VMEM((2, NJ, GW, 128), F32),
            pltpu.VMEM((2, 2 * NJ, GW, 128), F32),
            pltpu.VMEM((2, 2 * NJ, GW, 128), F32),
            pltpu.VMEM((2, 8 * HP, 128), U32),
            pltpu.VMEM((2 * HG - 2, S // 2, 128), U32),
            pltpu.VMEM((2, S // 2, 128), U32),
            pltpu.VMEM((S, D), F32),
            pltpu.VMEM((TM // 2, F), U32),
            pltpu.VMEM((2, TM, D), BF16),
            pltpu.VMEM((D, 128), F32),
            pltpu.VMEM((6, 8, D), F32),
            dma((S // TM1,)), dma((HG * 3,)), dma((6,)), dma((2 * D // MC,)), dma((4,)), dma((2,)),
        ],
        compiler_params=pltpu.CompilerParams(vmem_limit_bytes=120 * 1024 * 1024,
            flags={"XLA_TPU_EVENLY_DISTRIBUTE_CRITICAL_NODES": True}),
    )(A_x.reshape(S, D), A_wqkv, A_wo, B_w_gate, B_w_up, B_w_down, c, w_mod)
    return out.reshape(1, S, D)
```

```python
import jax
import jax.numpy as jnp
from jax import lax
from jax.experimental import pallas as pl
from jax.experimental.pallas import tpu as pltpu

S, D, F = 2048, 1024, 3584
DH, W = 32, 8
HG, GW = 4, 256
NJ = 8
TM1 = 256
TM = 512
FC = 512
DC = 256
LB = TM * DC // D
HP = 36
CFG_G = (((2, 2), 1), ((2, 2), 1))
CFG_W = (((2, 2), 1), ((2, 2), 1))
MC = 512
STAGE = (4, 4, 6, 8, 99)
PF0 = 2
LR = 64
EPS = 1e-5
F32, BF16, U32 = jnp.float32, jnp.bfloat16, jnp.uint32


def _dot(a, b):
    return jnp.dot(a, b, preferred_element_type=F32)


def _ln_mod(x, scale1, shift):
    m = jnp.mean(x, axis=-1, keepdims=True)
    xc = x - m
    v = jnp.mean(xc * xc, axis=-1, keepdims=True)
    return xc * lax.rsqrt(v + EPS) * scale1 + shift


def _unpack(w):
    lo = lax.bitcast_convert_type(w << 16, F32)
    hi = lax.bitcast_convert_type(w & jnp.uint32(0xFFFF0000), F32)
    return lo, hi


def _ld(ref, r):
    return pltpu.bitcast(ref[r, :], BF16)


def _mix(a, na=1, b=(), nb=0):
    b = iter(b)
    done = 0
    for k, _ in enumerate(a):
        while done * na < (k + 1) * nb:
            next(b)
            done += 1
    for _ in b:
        pass


def _bf16_bits(x):
    return lax.bitcast_convert_type(x.astype(BF16).astype(F32), U32)


def _kernel(x_hbm, wqkv_hbm, wo_hbm, wg_hbm, wu_hbm, wd_hbm, c_ref, wmod_hbm, out_hbm,
            x_v, wqkv_v, wo_v, wg_v, wu_v, wd_v, wmod_v, h_v, qkv0_v, qkv1_v, t_v, q_s, k_s, v_s,
            ot_v, o_v, o3_v, x1_v, x2_v, a_v, ob_v, scol_v, mod_v, sem_x, sem_qkv, sem_mod, sem_head, sem_w, sem_o):
    nb1 = S // TM1
    qkv_v = (qkv0_v, qkv1_v)

    def x_cp(i):
        r = pl.ds(i * TM1, TM1)
        return pltpu.make_async_copy(x_hbm.at[r], x_v.at[r], sem_x.at[i])

    def qkv_cp(g, t):
        return pltpu.make_async_copy(wqkv_hbm.at[:, pl.ds(t * D + g * GW, GW)],
                                     wqkv_v.at[g, :, pl.ds(t * GW, GW)], sem_qkv.at[g * 3 + t])

    def mod_cp(i):
        return pltpu.make_async_copy(wmod_hbm.at[:, pl.ds(i * D, D)], wmod_v.at[i], sem_mod.at[i])

    def mod_head_cp(i):
        return pltpu.make_async_copy(wmod_hbm.at[:, pl.ds(i * MC, MC)],
                                     wmod_v.at[i * MC // D, :, pl.ds(i * MC % D, MC)], sem_head.at[i])

    w_cps = [pltpu.make_async_copy(s, d, sem_w.at[i]) for i, (s, d) in enumerate(
        ((wo_hbm, wo_v), (wg_hbm, wg_v), (wu_hbm, wu_v), (wd_hbm, wd_v)))]

    def out_cp(i, n):
        cs = pl.ds(pl.multiple_of(n * DC, DC), DC)
        return pltpu.make_async_copy(ob_v.at[n], out_hbm.at[pl.ds(i * TM, TM), cs], sem_o.at[n])

    nm = 2 * D // MC
    head = [mod_head_cp(i) for i in range(nm)] + [x_cp(0)] + [qkv_cp(0, t) for t in range(3)]
    head += [x_cp(i) for i in range(1, nb1)]
    for cp in head[:STAGE[0]]:
        cp.start()

    cf = c_ref[...].astype(F32)
    sc = (cf * jax.nn.sigmoid(cf)).astype(BF16)
    scol_v[...] = jnp.broadcast_to(sc.astype(F32), (128, D)).T
    sc8 = jnp.broadcast_to(sc, (16, D))
    for i in range(nm):
        mod_head_cp(i).wait()
        for cp in head[STAGE[i]:STAGE[i + 1]]:
            cp.start()
        cs = pl.ds(i * MC % D, MC)
        mod_v[i * MC // D, :, cs] = _dot(sc8, wmod_v[i * MC // D, :, cs])[:8]

    def mod_vpu(i, n):
        cs = pl.ds(pl.multiple_of(n * 128, 128), 128)
        p = wmod_v[i, :, cs].astype(F32) * scol_v[...]
        mod_v[i, :, cs] = jnp.broadcast_to(jnp.sum(p, axis=0, keepdims=True), (8, 128))
        yield

    def mod_row(i):
        return mod_v[i, pl.ds(0, 1), :]

    def rows(i, n):
        return pl.ds(pl.multiple_of(i * n, n), n)

    def proj(g, i):
        for t in range(3):
            y = _dot(_ld(h_v, rows(i, TM1 // 2)), wqkv_v[g, :, pl.ds(t * GW, GW)])
            y = pltpu.bitcast(y.astype(BF16), U32)
            for n in range(2):
                qkv_v[g % 2][t * 2 + n, rows(i, TM1 // 2), :] = y[:, n * 128:(n + 1) * 128]
            yield

    def att_load(g, j, u):
        for t, dst in enumerate((q_s, k_s, v_s)):
            for n in range(2):
                w = qkv_v[g % 2][t * 2 + n, pl.ds(j, 128, stride=NJ), :]
                wt = w.T
                for h in range(4):
                    t_v[u * 3 + t, pl.ds((n * 4 + h) * HP, DH), :] = wt[h * DH:(h + 1) * DH]
            for d in range(DH):
                w = t_v[u * 3 + t, pl.ds(d, 8, stride=HP), :]
                r = pl.ds(d * 8, 8)
                if t == 0:
                    dst[0, j, r, :], dst[1, j, r, :] = _unpack(w)
                else:
                    dst[0, NJ + j, r, :], dst[1, NJ + j, r, :] = _unpack(w)
                    dst[0, j, r, :], dst[1, j, r, :] = _unpack(pltpu.roll(w, 1, 1))
            yield

    def att_core(g, j, u, last, qws, ch):
        lane0 = lax.broadcasted_iota(jnp.int32, (8, 128), 1) == 0
        probs = []
        for p in range(2):
            acc = [None] * W
            qw = qws[p]
            for w0 in range(0, W, qw):
                for d in range(DH):
                    r = pl.ds(d * 8, 8)
                    q = q_s[p, j, r, :]
                    if d == 0 and dep[0] is not None:
                        q = jnp.where(j < 0, dep[0], q)
                    for w in range(w0, w0 + qw):
                        t = q * k_s[p, j + (NJ - w), r, :]
                        acc[w] = t if d == 0 else acc[w] + t
                dep[0] = acc[w0]
            lg = [acc[0] * DH ** -0.5]
            for w in range(1, W):
                lg.append(jnp.where(jnp.logical_and(lane0, j < w), -1e9, acc[w] * DH ** -0.5))
            m = lg[0]
            for w in range(1, W):
                m = jnp.maximum(m, lg[w])
            e = [jnp.exp(l - m) for l in lg]
            den = e[0]
            for w in range(1, W):
                den = den + e[w]
            inv = 1.0 / den
            probs.append([x * inv for x in e])
            dep[0] = inv
            yield
        for d in range(DH):
            r = pl.ds(d * 8, 8)
            o = []
            for p in range(2):
                acc = probs[p][0] * v_s[p, j + NJ, r, :]
                for w in range(1, W):
                    acc = acc + probs[p][w] * v_s[p, j + (NJ - w), r, :]
                o.append(_bf16_bits(acc))
                if d % ch == ch - 1:
                    probs[p][0] = jnp.where(j < 0, acc, probs[p][0])
                    dep[0] = acc
            ot_v[u, pl.ds(d, 8, stride=HP), :] = (o[0] >> 16) | o[1]
        for n in range(2):
            ot = jnp.concatenate([ot_v[u, pl.ds((n * 4 + h) * HP, DH), :] for h in range(4)], axis=0)
            dst, base = (o_v, g * 2) if last is None else (last, 0)
            dst[base + n, pl.ds(j, 128, stride=NJ), :] = ot.T
        yield

    def o_cols(ref, r):
        return jnp.concatenate([_ld(ref.at[n], r) for n in range(ref.shape[0])], axis=1)

    def ln1(i):
        for k in range(TM1 // LR):
            b = i * (TM1 // LR) + k
            h = _ln_mod(x_v[rows(b, LR), :].astype(F32), 1.0 + mod_row(1), mod_row(0))
            h_v[rows(b, LR // 2), :] = pltpu.bitcast(h.astype(BF16), U32)

    def ln2(i):
        y = _dot(o_cols(o3_v, rows(i, LB // 2)), wo_v[pl.ds((HG - 1) * GW, GW), :])
        for k in range(LB // LR):
            b = i * (LB // LR) + k
            r = rows(b, LR)
            x1 = x_v[r, :].astype(F32) + mod_row(2) * (x1_v[r, :] + y[k * LR:(k + 1) * LR])
            x2_v[r, :] = x1
            h = _ln_mod(x1, 1.0 + mod_row(4), mod_row(3))
            h_v[rows(b, LR // 2), :] = pltpu.bitcast(h.astype(BF16), U32)

    def prefetch(g):
        nxt = [qkv_cp(g + 1, t) for t in range(3)] if g + 1 < HG else []
        for cp in nxt + [mod_cp(g + 2), w_cps[(g + 1) % HG]]:
            cp.start()

    x_cp(0).wait()
    ln1(0)
    for t in range(3):
        qkv_cp(0, t).wait()

    def first_body(i, carry):
        @pl.when(i + 1 < nb1)
        def _():
            x_cp(i + 1).wait()

        @pl.when(i == PF0)
        def _():
            prefetch(0)
        _mix(proj(0, i))
        ln1(jnp.minimum(i + 1, nb1 - 1))
        return carry
    lax.fori_loop(0, nb1, first_body, 0)

    half = nb1 // 2
    jpb = NJ // half

    def loads(g, i):
        for u in range(jpb):
            yield from att_load(g, i * jpb + u, u)
            yield from mod_vpu(g + 2, i * jpb + u)

    dep = [None]

    def cores(g, i, last, cfg):
        dep[0] = None
        for u in range(jpb):
            yield from att_core(g, i * jpb + u, u, last, *cfg[u])

    for g in range(1, HG):
        for t in range(3):
            qkv_cp(g, t).wait()
        mod_cp(g + 1).wait()
        prefetch(g)

        def body_a(i, c, g=g):
            _mix(proj(g, i), 3, loads(g - 1, i), 8)
            return c
        lax.fori_loop(0, half, body_a, 0)

        def body_b(i, c, g=g):
            _mix(proj(g, half + i), 3, cores(g - 1, i, None, CFG_G), 6)
            return c
        lax.fori_loop(0, half, body_b, 0)

    mod_cp(5).wait()
    w_cps[0].wait()

    def wo_part(i):
        for n in range(D // GW):
            o = o_cols(o_v, rows(i, TM1 // 2))
            cs = pl.ds(n * GW, GW)
            x1_v[rows(i, TM1), cs] = _dot(o, wo_v[pl.ds(0, (HG - 1) * GW), cs])
            yield

    def wo_a(i, c):
        _mix(wo_part(i), 4, loads(HG - 1, i), 8)
        return c
    lax.fori_loop(0, half, wo_a, 0)

    def wo_b(i, c):
        _mix(wo_part(half + i), 4, cores(HG - 1, i, o3_v, CFG_W), 6)
        return c
    lax.fori_loop(0, half, wo_b, 0)
    for cp in w_cps[1:]:
        cp.wait()

    nb, nd = S // TM, D // DC
    lax.fori_loop(0, nd, lambda n, c: ln2(n), None)

    def ffn_body(i, c):
        r = rows(i, TM)

        def gu(f, c2):
            cs = rows(f, FC)
            h = _ld(h_v, rows(i, TM // 2))
            gate = _dot(h, wg_v[:, cs])
            up = _dot(h, wu_v[:, cs])
            a_v[:, cs] = pltpu.bitcast((gate * jax.nn.sigmoid(gate) * up).astype(BF16), U32)
            return c2
        lax.fori_loop(0, F // FC, gu, 0)

        @pl.when(i >= 1)
        def _():
            for n in range(nd):
                out_cp(i - 1, n).wait()

        def dn(n, with_ln):
            if with_ln:
                ln2((i + 1) * nd + n)
            cs = rows(n, DC)
            y2 = _dot(_ld(a_v, slice(None)), wd_v[:, cs])
            ob_v[n] = (x2_v[r, cs] + mod_v[5, pl.ds(0, 1), cs] * y2).astype(BF16)
            out_cp(i, n).start()

        @pl.when(i < nb - 1)
        def _():
            lax.fori_loop(0, nd, lambda n, c2: dn(n, True), None)

        @pl.when(i == nb - 1)
        def _():
            lax.fori_loop(0, nd, lambda n, c2: dn(n, False), None)
        return c
    lax.fori_loop(0, nb, ffn_body, 0)
    for n in range(nd):
        out_cp(nb - 1, n).wait()


@jax.jit
def pallas_adaLN_cond__sliding_local_dilated__swiglu_ffn__prompt_kernel(
    A_x: jax.Array,
    A_wqkv: jax.Array,
    A_wo: jax.Array,
    B_x: jax.Array,
    B_w_gate: jax.Array,
    B_w_up: jax.Array,
    B_w_down: jax.Array,
    c: jax.Array,
    w_mod: jax.Array,
):
    del B_x
    hbm = pl.BlockSpec(memory_space=pl.ANY)
    dma = pltpu.SemaphoreType.DMA
    out = pl.pallas_call(
        _kernel,
        out_shape=jax.ShapeDtypeStruct((S, D), BF16),
        in_specs=[hbm] * 6 + [pl.BlockSpec(memory_space=pltpu.VMEM), hbm],
        out_specs=hbm,
        scratch_shapes=[
            pltpu.VMEM((S, D), BF16),
            pltpu.VMEM((HG, D, 3 * GW), BF16),
            pltpu.VMEM((D, D), BF16),
            pltpu.VMEM((D, F), BF16),
            pltpu.VMEM((D, F), BF16),
            pltpu.VMEM((F, D), BF16),
            pltpu.VMEM((6, D, D), BF16),
            pltpu.VMEM((S // 2, D), U32),
            pltpu.VMEM((6, S // 2, 128), U32),
            pltpu.VMEM((6, S // 2, 128), U32),
            pltpu.VMEM((6, 8 * HP, 128), U32),
            pltpu.VMEM((2, NJ, GW, 128), F32),
            pltpu.VMEM((2, 2 * NJ, GW, 128), F32),
            pltpu.VMEM((2, 2 * NJ, GW, 128), F32),
            pltpu.VMEM((2, 8 * HP, 128), U32),
            pltpu.VMEM((2 * HG - 2, S // 2, 128), U32),
            pltpu.VMEM((2, S // 2, 128), U32),
            pltpu.VMEM((S, D), F32),
            pltpu.VMEM((S, D), F32),
            pltpu.VMEM((TM // 2, F), U32),
            pltpu.VMEM((D // DC, TM, DC), BF16),
            pltpu.VMEM((D, 128), F32),
            pltpu.VMEM((6, 8, D), F32),
            dma((S // TM1,)), dma((HG * 3,)), dma((6,)), dma((2 * D // MC,)), dma((4,)), dma((D // DC,)),
        ],
        compiler_params=pltpu.CompilerParams(vmem_limit_bytes=120 * 1024 * 1024,
            flags={"XLA_TPU_EVENLY_DISTRIBUTE_CRITICAL_NODES": True}),
    )(A_x.reshape(S, D), A_wqkv, A_wo, B_w_gate, B_w_up, B_w_down, c, w_mod)
    return out.reshape(1, S, D)
```

```python
import jax
import jax.numpy as jnp
from jax import lax
from jax.experimental import pallas as pl
from jax.experimental.pallas import tpu as pltpu

S, D, F = 2048, 1024, 3584
DH, W = 32, 8
HG, GW = 4, 256
NJ = 8
TM1 = 256
TM = 512
FC = 896
DC = 256
LB = TM * DC // D
HP = 36
REP = 1
CFG = (((2, 2), 1), ((2, 2), 1))
MC = 512
STAGE = (4, 4, 6, 8, 99)
PF0 = 2
LR = 64
EPS = 1e-5
F32, BF16, U32 = jnp.float32, jnp.bfloat16, jnp.uint32


def _dot(a, b):
    return jnp.dot(a, b, preferred_element_type=F32)


def _ln_mod(x, scale1, shift):
    m = jnp.mean(x, axis=-1, keepdims=True)
    xc = x - m
    v = jnp.mean(xc * xc, axis=-1, keepdims=True)
    return xc * lax.rsqrt(v + EPS) * scale1 + shift


def _unpack(w):
    lo = lax.bitcast_convert_type(w << 16, F32)
    hi = lax.bitcast_convert_type(w & jnp.uint32(0xFFFF0000), F32)
    return lo, hi


def _ld(ref, r):
    return pltpu.bitcast(ref[r, :], BF16)


def _mix(a, na=1, b=(), nb=0):
    b = iter(b)
    done = 0
    for k, _ in enumerate(a):
        while done * na < (k + 1) * nb:
            next(b)
            done += 1
    for _ in b:
        pass


def _bf16_bits(x):
    return lax.bitcast_convert_type(x.astype(BF16).astype(F32), U32)


def _kernel(x_hbm, wqkv_hbm, wo_hbm, wg_hbm, wu_hbm, wd_hbm, c_ref, wmod_hbm, out_hbm,
            x_v, wqkv_v, wo_v, wg_v, wu_v, wd_v, wmod_v, h_v, qkv0_v, qkv1_v, t_v, q_s, k_s, v_s,
            ot_v, o_v, o3_v, x1_v, x2_v, a_v, ob_v, scol_v, mod_v, sem_x, sem_qkv, sem_mod, sem_head, sem_w, sem_o):
    nb1 = S // TM1
    qkv_v = (qkv0_v, qkv1_v)

    def x_cp(i):
        r = pl.ds(i * TM1, TM1)
        return pltpu.make_async_copy(x_hbm.at[r], x_v.at[r], sem_x.at[i])

    def qkv_cp(g, t):
        return pltpu.make_async_copy(wqkv_hbm.at[:, pl.ds(t * D + g * GW, GW)],
                                     wqkv_v.at[g, :, pl.ds(t * GW, GW)], sem_qkv.at[g * 3 + t])

    def mod_cp(i):
        return pltpu.make_async_copy(wmod_hbm.at[:, pl.ds(i * D, D)], wmod_v.at[i], sem_mod.at[i])

    def mod_head_cp(i):
        return pltpu.make_async_copy(wmod_hbm.at[:, pl.ds(i * MC, MC)],
                                     wmod_v.at[i * MC // D, :, pl.ds(i * MC % D, MC)], sem_head.at[i])

    w_cps = [pltpu.make_async_copy(s, d, sem_w.at[i]) for i, (s, d) in enumerate(
        ((wo_hbm, wo_v), (wg_hbm, wg_v), (wu_hbm, wu_v), (wd_hbm, wd_v)))]

    def out_cp(i, n):
        cs = pl.ds(pl.multiple_of(n * DC, DC), DC)
        return pltpu.make_async_copy(ob_v.at[n], out_hbm.at[pl.ds(i * TM, TM), cs], sem_o.at[n])

    nm = 2 * D // MC
    head = [mod_head_cp(i) for i in range(nm)] + [x_cp(0)] + [qkv_cp(0, t) for t in range(3)]
    head += [x_cp(i) for i in range(1, nb1)]
    for cp in head[:STAGE[0]]:
        cp.start()

    cf = c_ref[...].astype(F32)
    sc = (cf * jax.nn.sigmoid(cf)).astype(BF16)
    scol_v[...] = jnp.broadcast_to(sc.astype(F32), (128, D)).T
    sc8 = jnp.broadcast_to(sc, (16, D))
    for i in range(nm):
        mod_head_cp(i).wait()
        for cp in head[STAGE[i]:STAGE[i + 1]]:
            cp.start()
        cs = pl.ds(i * MC % D, MC)
        mod_v[i * MC // D, :, cs] = _dot(sc8, wmod_v[i * MC // D, :, cs])[:8]

    def mod_vpu(i, n):
        cs = pl.ds(pl.multiple_of(n * 128, 128), 128)
        p = wmod_v[i, :, cs].astype(F32) * scol_v[...]
        mod_v[i, :, cs] = jnp.broadcast_to(jnp.sum(p, axis=0, keepdims=True), (8, 128))
        yield

    def mod_row(i):
        return mod_v[i, pl.ds(0, 1), :]

    def rows(i, n):
        return pl.ds(pl.multiple_of(i * n, n), n)

    def proj(g, i):
        for t in range(3):
            y = _dot(_ld(h_v, rows(i, TM1 // 2)), wqkv_v[g, :, pl.ds(t * GW, GW)])
            y = pltpu.bitcast(y.astype(BF16), U32)
            for n in range(2):
                qkv_v[g % 2][t * 2 + n, rows(i, TM1 // 2), :] = y[:, n * 128:(n + 1) * 128]
            yield

    def att_load(g, j, u):
        for t, dst in enumerate((q_s, k_s, v_s)):
            for n in range(2):
                w = qkv_v[g % 2][t * 2 + n, pl.ds(j, 128, stride=NJ), :]
                wt = w.T
                for h in range(4):
                    t_v[u * 3 + t, pl.ds((n * 4 + h) * HP, DH), :] = wt[h * DH:(h + 1) * DH]
            for d in range(DH):
                w = t_v[u * 3 + t, pl.ds(d, 8, stride=HP), :]
                r = pl.ds(d * 8, 8)
                if t == 0:
                    dst[0, j, r, :], dst[1, j, r, :] = _unpack(w)
                else:
                    dst[0, NJ + j, r, :], dst[1, NJ + j, r, :] = _unpack(w)
                    dst[0, j, r, :], dst[1, j, r, :] = _unpack(pltpu.roll(w, 1, 1))
            yield

    def att_core(dst, base, j, u):
        qws, ch = CFG[u]
        lane0 = lax.broadcasted_iota(jnp.int32, (8, 128), 1) == 0
        probs = []
        for p in range(2):
            acc = [None] * W
            qw = qws[p]
            for w0 in range(0, W, qw):
                for d in range(DH):
                    r = pl.ds(d * 8, 8)
                    q = q_s[p, j, r, :]
                    if d == 0 and dep[0] is not None:
                        q = jnp.where(j < 0, dep[0], q)
                    for w in range(w0, w0 + qw):
                        t = q * k_s[p, j + (NJ - w), r, :]
                        acc[w] = t if d == 0 else acc[w] + t
                dep[0] = acc[w0]
            lg = [acc[0] * DH ** -0.5]
            for w in range(1, W):
                lg.append(jnp.where(jnp.logical_and(lane0, j < w), -1e9, acc[w] * DH ** -0.5))
            m = lg[0]
            for w in range(1, W):
                m = jnp.maximum(m, lg[w])
            e = [jnp.exp(l - m) for l in lg]
            den = e[0]
            for w in range(1, W):
                den = den + e[w]
            inv = 1.0 / den
            probs.append([x * inv for x in e])
            dep[0] = inv
            yield
        for d in range(DH):
            r = pl.ds(d * 8, 8)
            o = []
            for p in range(2):
                acc = probs[p][0] * v_s[p, j + NJ, r, :]
                for w in range(1, W):
                    acc = acc + probs[p][w] * v_s[p, j + (NJ - w), r, :]
                o.append(_bf16_bits(acc))
                if d % ch == ch - 1:
                    probs[p][0] = jnp.where(j < 0, acc, probs[p][0])
                    dep[0] = acc
            ot_v[u, pl.ds(d, 8, stride=HP), :] = (o[0] >> 16) | o[1]
        for n in range(2):
            ot = jnp.concatenate([ot_v[u, pl.ds((n * 4 + h) * HP, DH), :] for h in range(4)], axis=0)
            dst[base + n, pl.ds(j, 128, stride=NJ), :] = ot.T
        yield

    def o_cols(ref, r):
        return jnp.concatenate([_ld(ref.at[n], r) for n in range(ref.shape[0])], axis=1)

    def ln1(i):
        for k in range(TM1 // LR):
            b = i * (TM1 // LR) + k
            h = _ln_mod(x_v[rows(b, LR), :].astype(F32), 1.0 + mod_row(1), mod_row(0))
            h_v[rows(b, LR // 2), :] = pltpu.bitcast(h.astype(BF16), U32)

    def ln2(i):
        y = _dot(o_cols(o3_v, rows(i, LB // 2)), wo_v[pl.ds((HG - 1) * GW, GW), :])
        for k in range(LB // LR):
            b = i * (LB // LR) + k
            r = rows(b, LR)
            x1 = x_v[r, :].astype(F32) + mod_row(2) * (x1_v[r, :] + y[k * LR:(k + 1) * LR])
            x2_v[r, :] = x1
            h = _ln_mod(x1, 1.0 + mod_row(4), mod_row(3))
            h_v[rows(b, LR // 2), :] = pltpu.bitcast(h.astype(BF16), U32)

    def prefetch(g):
        nxt = [qkv_cp(g + 1, t) for t in range(3)] if g + 1 < HG else []
        for cp in nxt + [mod_cp(g + 2), w_cps[(g + 1) % HG]]:
            cp.start()

    x_cp(0).wait()
    ln1(0)
    for t in range(3):
        qkv_cp(0, t).wait()

    def first_body(i, carry):
        @pl.when(i + 1 < nb1)
        def _():
            x_cp(i + 1).wait()

        @pl.when(i == PF0)
        def _():
            prefetch(0)
        _mix(proj(0, i))
        ln1(jnp.minimum(i + 1, nb1 - 1))
        return carry
    lax.fori_loop(0, nb1, first_body, 0)

    half = nb1 // 2
    jpb = NJ // half

    dep = [None]

    def loads(g, i):
        for u in range(jpb):
            yield from att_load(g, i * jpb + u, u)
            yield from mod_vpu(g + 2, i * jpb + u)

    def cores(g, i):
        dst, base = (o_v, g * 2) if g + 1 < HG else (o3_v, 0)
        for u in range(jpb):
            yield from att_core(dst, base, i * jpb + u, u)

    def wo_part(i):
        for n in range(D // GW):
            cs = pl.ds(n * GW, GW)
            o = o_cols(o_v, rows(i, TM1 // 2))
            x1_v[rows(i, TM1), cs] = _dot(o, wo_v[pl.ds(0, (HG - 1) * GW), cs])
            yield

    def overlapped(g, matmul, steps):
        def body_a(i, c):
            for k in range(REP):
                _mix(matmul(i * REP + k), steps, loads(g, i * REP + k), 4 * jpb)
            return c
        lax.fori_loop(0, half // REP, body_a, 0)

        def body_b(i, c):
            dep[0] = None
            for k in range(REP):
                _mix(matmul(half + i * REP + k), steps, cores(g, i * REP + k), 3 * jpb)
            return c
        lax.fori_loop(0, half // REP, body_b, 0)

    for g in range(1, HG):
        for t in range(3):
            qkv_cp(g, t).wait()
        mod_cp(g + 1).wait()
        prefetch(g)
        overlapped(g - 1, lambda i, g=g: proj(g, i), 3)

    mod_cp(5).wait()
    w_cps[0].wait()
    overlapped(HG - 1, wo_part, D // GW)
    for cp in w_cps[1:]:
        cp.wait()

    nb, nd = S // TM, D // DC
    lax.fori_loop(0, nd, lambda n, c: ln2(n), None)

    def ffn_body(i, c):
        r = rows(i, TM)

        def gu(f, c2):
            cs = rows(f, FC)
            h = _ld(h_v, rows(i, TM // 2))
            gate = _dot(h, wg_v[:, cs])
            up = _dot(h, wu_v[:, cs])
            a_v[:, cs] = pltpu.bitcast((gate * jax.nn.sigmoid(gate) * up).astype(BF16), U32)
            return c2
        lax.fori_loop(0, F // FC, gu, 0)

        @pl.when(i >= 1)
        def _():
            for n in range(nd):
                out_cp(i - 1, n).wait()

        def dn(n, with_ln):
            if with_ln:
                ln2((i + 1) * nd + n)
            cs = rows(n, DC)
            y2 = _dot(_ld(a_v, slice(None)), wd_v[:, cs])
            ob_v[n] = (x2_v[r, cs] + mod_v[5, pl.ds(0, 1), cs] * y2).astype(BF16)
            out_cp(i, n).start()

        @pl.when(i < nb - 1)
        def _():
            lax.fori_loop(0, nd, lambda n, c2: dn(n, True), None)

        @pl.when(i == nb - 1)
        def _():
            lax.fori_loop(0, nd, lambda n, c2: dn(n, False), None)
        return c
    lax.fori_loop(0, nb, ffn_body, 0)
    for n in range(nd):
        out_cp(nb - 1, n).wait()


@jax.jit
def pallas_adaLN_cond__sliding_local_dilated__swiglu_ffn__prompt_kernel(
    A_x: jax.Array,
    A_wqkv: jax.Array,
    A_wo: jax.Array,
    B_x: jax.Array,
    B_w_gate: jax.Array,
    B_w_up: jax.Array,
    B_w_down: jax.Array,
    c: jax.Array,
    w_mod: jax.Array,
):
    del B_x
    hbm = pl.BlockSpec(memory_space=pl.ANY)
    dma = pltpu.SemaphoreType.DMA
    out = pl.pallas_call(
        _kernel,
        out_shape=jax.ShapeDtypeStruct((S, D), BF16),
        in_specs=[hbm] * 6 + [pl.BlockSpec(memory_space=pltpu.VMEM), hbm],
        out_specs=hbm,
        scratch_shapes=[
            pltpu.VMEM((S, D), BF16),
            pltpu.VMEM((HG, D, 3 * GW), BF16),
            pltpu.VMEM((D, D), BF16),
            pltpu.VMEM((D, F), BF16),
            pltpu.VMEM((D, F), BF16),
            pltpu.VMEM((F, D), BF16),
            pltpu.VMEM((6, D, D), BF16),
            pltpu.VMEM((S // 2, D), U32),
            pltpu.VMEM((6, S // 2, 128), U32),
            pltpu.VMEM((6, S // 2, 128), U32),
            pltpu.VMEM((6, 8 * HP, 128), U32),
            pltpu.VMEM((2, NJ, GW, 128), F32),
            pltpu.VMEM((2, 2 * NJ, GW, 128), F32),
            pltpu.VMEM((2, 2 * NJ, GW, 128), F32),
            pltpu.VMEM((2, 8 * HP, 128), U32),
            pltpu.VMEM((2 * HG - 2, S // 2, 128), U32),
            pltpu.VMEM((2, S // 2, 128), U32),
            pltpu.VMEM((S, D), F32),
            pltpu.VMEM((S, D), F32),
            pltpu.VMEM((TM // 2, F), U32),
            pltpu.VMEM((D // DC, TM, DC), BF16),
            pltpu.VMEM((D, 128), F32),
            pltpu.VMEM((6, 8, D), F32),
            dma((S // TM1,)), dma((HG * 3,)), dma((6,)), dma((2 * D // MC,)), dma((4,)), dma((D // DC,)),
        ],
        compiler_params=pltpu.CompilerParams(vmem_limit_bytes=120 * 1024 * 1024,
            flags={"XLA_TPU_EVENLY_DISTRIBUTE_CRITICAL_NODES": True}),
    )(A_x.reshape(S, D), A_wqkv, A_wo, B_w_gate, B_w_up, B_w_down, c, w_mod)
    return out.reshape(1, S, D)
```

```python
import jax
import jax.numpy as jnp
from jax import lax
from jax.experimental import pallas as pl
from jax.experimental.pallas import tpu as pltpu

S, D, F = 2048, 1024, 3584
DH, W = 32, 8
HG, GW = 4, 256
NJ = 8
TM1 = 256
TM = 512
FC = 896
DC = 256
LB = TM * DC // D
HP = 36
CFG = (((2, 2), 1), ((2, 2), 1))
MC = 512
STAGE = (4, 4, 6, 8, 99)
PF0 = 2
LR = 128
EPS = 1e-5
F32, BF16, U32 = jnp.float32, jnp.bfloat16, jnp.uint32


def _dot(a, b):
    return jnp.dot(a, b, preferred_element_type=F32)


def _ln_mod(x, scale1, shift):
    m = jnp.mean(x, axis=-1, keepdims=True)
    xc = x - m
    v = jnp.mean(xc * xc, axis=-1, keepdims=True)
    return xc * lax.rsqrt(v + EPS) * scale1 + shift


def _unpack(w):
    lo = lax.bitcast_convert_type(w << 16, F32)
    hi = lax.bitcast_convert_type(w & jnp.uint32(0xFFFF0000), F32)
    return lo, hi


def _ld(ref, r):
    return pltpu.bitcast(ref[r, :], BF16)


def _mix(a, na=1, b=(), nb=0):
    b = iter(b)
    done = 0
    for k, _ in enumerate(a):
        while done * na < (k + 1) * nb:
            next(b)
            done += 1
    for _ in b:
        pass


def _bf16_bits(x):
    return lax.bitcast_convert_type(x.astype(BF16).astype(F32), U32)


def _kernel(x_hbm, wqkv_hbm, wo_hbm, wg_hbm, wu_hbm, wd_hbm, c_ref, wmod_hbm, out_hbm,
            x_v, wqkv_v, wo_v, wg_v, wu_v, wd_v, wmod_v, h_v, qkv0_v, qkv1_v, t_v, q_s, k_s, v_s,
            ot_v, o_v, o3_v, x1_v, x2_v, a_v, ob_v, scol_v, mod_v, sem_x, sem_qkv, sem_mod, sem_head, sem_w, sem_o):
    nb1 = S // TM1
    qkv_v = (qkv0_v, qkv1_v)

    def x_cp(i):
        r = pl.ds(i * TM1, TM1)
        return pltpu.make_async_copy(x_hbm.at[r], x_v.at[r], sem_x.at[i])

    def qkv_cp(g, t):
        return pltpu.make_async_copy(wqkv_hbm.at[:, pl.ds(t * D + g * GW, GW)],
                                     wqkv_v.at[g, :, pl.ds(t * GW, GW)], sem_qkv.at[g * 3 + t])

    def mod_cp(i):
        return pltpu.make_async_copy(wmod_hbm.at[:, pl.ds(i * D, D)], wmod_v.at[i], sem_mod.at[i])

    def mod_head_cp(i):
        return pltpu.make_async_copy(wmod_hbm.at[:, pl.ds(i * MC, MC)],
                                     wmod_v.at[i * MC // D, :, pl.ds(i * MC % D, MC)], sem_head.at[i])

    w_cps = [pltpu.make_async_copy(s, d, sem_w.at[i]) for i, (s, d) in enumerate(
        ((wo_hbm, wo_v), (wg_hbm, wg_v), (wu_hbm, wu_v), (wd_hbm, wd_v)))]

    def out_cp(i, n):
        cs = pl.ds(pl.multiple_of(n * DC, DC), DC)
        return pltpu.make_async_copy(ob_v.at[n], out_hbm.at[pl.ds(i * TM, TM), cs], sem_o.at[n])

    nm = 2 * D // MC
    head = [mod_head_cp(i) for i in range(nm)] + [x_cp(0)] + [qkv_cp(0, t) for t in range(3)]
    head += [x_cp(i) for i in range(1, nb1)]
    for cp in head[:STAGE[0]]:
        cp.start()

    cf = c_ref[...].astype(F32)
    sc = (cf * jax.nn.sigmoid(cf)).astype(BF16)
    scol_v[...] = jnp.broadcast_to(sc.astype(F32), (128, D)).T
    sc8 = jnp.broadcast_to(sc, (16, D))
    for i in range(nm):
        mod_head_cp(i).wait()
        for cp in head[STAGE[i]:STAGE[i + 1]]:
            cp.start()
        cs = pl.ds(i * MC % D, MC)
        mod_v[i * MC // D, :, cs] = _dot(sc8, wmod_v[i * MC // D, :, cs])[:8]

    def mod_vpu(i, n):
        cs = pl.ds(pl.multiple_of(n * 128, 128), 128)
        p = wmod_v[i, :, cs].astype(F32) * scol_v[...]
        mod_v[i, :, cs] = jnp.broadcast_to(jnp.sum(p, axis=0, keepdims=True), (8, 128))
        yield

    def mod_row(i):
        return mod_v[i, pl.ds(0, 1), :]

    def rows(i, n):
        return pl.ds(pl.multiple_of(i * n, n), n)

    def proj(g, i):
        for t in range(3):
            y = _dot(_ld(h_v, rows(i, TM1 // 2)), wqkv_v[g, :, pl.ds(t * GW, GW)])
            y = pltpu.bitcast(y.astype(BF16), U32)
            for n in range(2):
                qkv_v[g % 2][t * 2 + n, rows(i, TM1 // 2), :] = y[:, n * 128:(n + 1) * 128]
            yield

    def att_load(g, j, u):
        for t, dst in enumerate((q_s, k_s, v_s)):
            for n in range(2):
                w = qkv_v[g % 2][t * 2 + n, pl.ds(j, 128, stride=NJ), :]
                wt = w.T
                for h in range(4):
                    t_v[u * 3 + t, pl.ds((n * 4 + h) * HP, DH), :] = wt[h * DH:(h + 1) * DH]
            for d in range(DH):
                w = t_v[u * 3 + t, pl.ds(d, 8, stride=HP), :]
                r = pl.ds(d * 8, 8)
                if t == 0:
                    dst[0, j, r, :], dst[1, j, r, :] = _unpack(w)
                else:
                    dst[0, NJ + j, r, :], dst[1, NJ + j, r, :] = _unpack(w)
                    dst[0, j, r, :], dst[1, j, r, :] = _unpack(pltpu.roll(w, 1, 1))
            yield

    def att_core(dst, base, j, u):
        qws, ch = CFG[u]
        lane0 = lax.broadcasted_iota(jnp.int32, (8, 128), 1) == 0
        probs = []
        for p in range(2):
            acc = [None] * W
            qw = qws[p]
            for w0 in range(0, W, qw):
                for d in range(DH):
                    r = pl.ds(d * 8, 8)
                    q = q_s[p, j, r, :]
                    if d == 0 and dep[0] is not None:
                        q = jnp.where(j < 0, dep[0], q)
                    for w in range(w0, w0 + qw):
                        t = q * k_s[p, j + (NJ - w), r, :]
                        acc[w] = t if d == 0 else acc[w] + t
                dep[0] = acc[w0]
            lg = [acc[0] * DH ** -0.5]
            for w in range(1, W):
                lg.append(jnp.where(jnp.logical_and(lane0, j < w), -1e9, acc[w] * DH ** -0.5))
            m = lg[0]
            for w in range(1, W):
                m = jnp.maximum(m, lg[w])
            e = [jnp.exp(l - m) for l in lg]
            den = e[0]
            for w in range(1, W):
                den = den + e[w]
            inv = 1.0 / den
            probs.append([x * inv for x in e])
            dep[0] = inv
            yield
        for d in range(DH):
            r = pl.ds(d * 8, 8)
            o = []
            for p in range(2):
                acc = probs[p][0] * v_s[p, j + NJ, r, :]
                for w in range(1, W):
                    acc = acc + probs[p][w] * v_s[p, j + (NJ - w), r, :]
                o.append(_bf16_bits(acc))
                if d % ch == ch - 1:
                    probs[p][0] = jnp.where(j < 0, acc, probs[p][0])
                    dep[0] = acc
            ot_v[u, pl.ds(d, 8, stride=HP), :] = (o[0] >> 16) | o[1]
        for n in range(2):
            ot = jnp.concatenate([ot_v[u, pl.ds((n * 4 + h) * HP, DH), :] for h in range(4)], axis=0)
            dst[base + n, pl.ds(j, 128, stride=NJ), :] = ot.T
        yield

    def o_cols(ref, r):
        return jnp.concatenate([_ld(ref.at[n], r) for n in range(ref.shape[0])], axis=1)

    def ln1(i):
        for k in range(TM1 // LR):
            b = i * (TM1 // LR) + k
            h = _ln_mod(x_v[rows(b, LR), :].astype(F32), 1.0 + mod_row(1), mod_row(0))
            h_v[rows(b, LR // 2), :] = pltpu.bitcast(h.astype(BF16), U32)

    def ln2(i):
        y = _dot(o_cols(o3_v, rows(i, LB // 2)), wo_v[pl.ds((HG - 1) * GW, GW), :])
        for k in range(LB // LR):
            b = i * (LB // LR) + k
            r = rows(b, LR)
            x1 = x_v[r, :].astype(F32) + mod_row(2) * (x1_v[r, :] + y[k * LR:(k + 1) * LR])
            x2_v[r, :] = x1
            h = _ln_mod(x1, 1.0 + mod_row(4), mod_row(3))
            h_v[rows(b, LR // 2), :] = pltpu.bitcast(h.astype(BF16), U32)

    def prefetch(g):
        nxt = [qkv_cp(g + 1, t) for t in range(3)] if g + 1 < HG else []
        for cp in nxt + [mod_cp(g + 2), w_cps[(g + 1) % HG]]:
            cp.start()

    x_cp(0).wait()
    ln1(0)
    for t in range(3):
        qkv_cp(0, t).wait()

    def first_body(i, carry):
        @pl.when(i + 1 < nb1)
        def _():
            x_cp(i + 1).wait()

        @pl.when(i == PF0)
        def _():
            prefetch(0)
        _mix(proj(0, i))
        ln1(jnp.minimum(i + 1, nb1 - 1))
        return carry
    lax.fori_loop(0, nb1, first_body, 0)

    half = nb1 // 2
    jpb = NJ // half

    dep = [None]

    def loads(g, j0, nj):
        for u in range(nj):
            yield from att_load(g, j0 + u, u)
            yield from mod_vpu(g + 2, j0 + u)

    def cores(g, i):
        dst, base = (o_v, g * 2) if g + 1 < HG else (o3_v, 0)
        for u in range(jpb):
            yield from att_core(dst, base, i * jpb + u, u)

    def wo_part(i):
        for n in range(D // GW):
            cs = pl.ds(n * GW, GW)
            o = o_cols(o_v, rows(i, TM1 // 2))
            x1_v[rows(i, TM1), cs] = _dot(o, wo_v[pl.ds(0, (HG - 1) * GW), cs])
            yield

    def overlapped(g, matmul, steps, na):
        nj = NJ // na

        def body_a(i, c):
            _mix(matmul(i), steps, loads(g, i * nj, nj), 4 * nj)
            return c
        lax.fori_loop(0, na, body_a, 0)

        def body_b(i, c):
            dep[0] = None
            _mix(matmul(na + i), steps, cores(g, i), 3 * jpb)
            return c
        lax.fori_loop(0, half, body_b, 0)

    for g in range(1, HG):
        for t in range(3):
            qkv_cp(g, t).wait()
        mod_cp(g + 1).wait()
        prefetch(g)
        overlapped(g - 1, lambda i, g=g: proj(g, i), 3, half)

    mod_cp(5).wait()
    w_cps[0].wait()
    nd = D // DC
    nlate = TM // TM1
    overlapped(HG - 1, wo_part, D // GW, half - nlate)

    def late_body(i, c):
        for k in range(nd // nlate):
            ln2(i * (nd // nlate) + k)
        _mix(wo_part(nb1 - nlate + i))
        return c
    lax.fori_loop(0, nlate, late_body, 0)
    for cp in w_cps[1:]:
        cp.wait()

    nb = S // TM

    def ffn_body(i, c):
        r = rows(i, TM)

        def gu(f, c2):
            cs = rows(f, FC)
            h = _ld(h_v, rows(i, TM // 2))
            gate = _dot(h, wg_v[:, cs])
            up = _dot(h, wu_v[:, cs])
            a_v[:, cs] = pltpu.bitcast((gate * jax.nn.sigmoid(gate) * up).astype(BF16), U32)
            return c2
        lax.fori_loop(0, F // FC, gu, 0)

        @pl.when(i >= 1)
        def _():
            for n in range(nd):
                out_cp(i - 1, n).wait()

        def dn(n, with_ln):
            if with_ln:
                ln2((i + 1) * nd + n)
            cs = rows(n, DC)
            y2 = _dot(_ld(a_v, slice(None)), wd_v[:, cs])
            ob_v[n] = (x2_v[r, cs] + mod_v[5, pl.ds(0, 1), cs] * y2).astype(BF16)
            out_cp(i, n).start()

        @pl.when(i < nb - 1)
        def _():
            lax.fori_loop(0, nd, lambda n, c2: dn(n, True), None)

        @pl.when(i == nb - 1)
        def _():
            lax.fori_loop(0, nd, lambda n, c2: dn(n, False), None)
        return c
    lax.fori_loop(0, nb, ffn_body, 0)
    for n in range(nd):
        out_cp(nb - 1, n).wait()


@jax.jit
def pallas_adaLN_cond__sliding_local_dilated__swiglu_ffn__prompt_kernel(
    A_x: jax.Array,
    A_wqkv: jax.Array,
    A_wo: jax.Array,
    B_x: jax.Array,
    B_w_gate: jax.Array,
    B_w_up: jax.Array,
    B_w_down: jax.Array,
    c: jax.Array,
    w_mod: jax.Array,
):
    del B_x
    hbm = pl.BlockSpec(memory_space=pl.ANY)
    dma = pltpu.SemaphoreType.DMA
    out = pl.pallas_call(
        _kernel,
        out_shape=jax.ShapeDtypeStruct((S, D), BF16),
        in_specs=[hbm] * 6 + [pl.BlockSpec(memory_space=pltpu.VMEM), hbm],
        out_specs=hbm,
        scratch_shapes=[
            pltpu.VMEM((S, D), BF16),
            pltpu.VMEM((HG, D, 3 * GW), BF16),
            pltpu.VMEM((D, D), BF16),
            pltpu.VMEM((D, F), BF16),
            pltpu.VMEM((D, F), BF16),
            pltpu.VMEM((F, D), BF16),
            pltpu.VMEM((6, D, D), BF16),
            pltpu.VMEM((S // 2, D), U32),
            pltpu.VMEM((6, S // 2, 128), U32),
            pltpu.VMEM((6, S // 2, 128), U32),
            pltpu.VMEM((12, 8 * HP, 128), U32),
            pltpu.VMEM((2, NJ, GW, 128), F32),
            pltpu.VMEM((2, 2 * NJ, GW, 128), F32),
            pltpu.VMEM((2, 2 * NJ, GW, 128), F32),
            pltpu.VMEM((2, 8 * HP, 128), U32),
            pltpu.VMEM((2 * HG - 2, S // 2, 128), U32),
            pltpu.VMEM((2, S // 2, 128), U32),
            pltpu.VMEM((S, D), F32),
            pltpu.VMEM((S, D), F32),
            pltpu.VMEM((TM // 2, F), U32),
            pltpu.VMEM((D // DC, TM, DC), BF16),
            pltpu.VMEM((D, 128), F32),
            pltpu.VMEM((6, 8, D), F32),
            dma((S // TM1,)), dma((HG * 3,)), dma((6,)), dma((2 * D // MC,)), dma((4,)), dma((D // DC,)),
        ],
        compiler_params=pltpu.CompilerParams(vmem_limit_bytes=120 * 1024 * 1024,
            flags={"XLA_TPU_EVENLY_DISTRIBUTE_CRITICAL_NODES": True}),
    )(A_x.reshape(S, D), A_wqkv, A_wo, B_w_gate, B_w_up, B_w_down, c, w_mod)
    return out.reshape(1, S, D)
```

```python
import jax
import jax.numpy as jnp
from jax import lax
from jax.experimental import pallas as pl
from jax.experimental.pallas import tpu as pltpu

S, D, F = 2048, 1024, 3584
DH, W = 32, 8
HG, GW = 4, 256
NJ = 8
TM1 = 256
TM = 512
FC = 896
DC = 256
LB = TM * DC // D
HP = 36
CFG = (((2, 4), 1), ((2, 4), 1))
MC = 512
STAGE = (4, 4, 6, 8, 99)
PF0 = 2
LR = 128
TIE, TIW = 512, 768
EPS = 1e-5
F32, BF16, U32 = jnp.float32, jnp.bfloat16, jnp.uint32


def _dot(a, b):
    return jnp.dot(a, b, preferred_element_type=F32)


def _ln_mod(x, scale1, shift):
    m = jnp.mean(x, axis=-1, keepdims=True)
    xc = x - m
    v = jnp.mean(xc * xc, axis=-1, keepdims=True)
    return xc * lax.rsqrt(v + EPS) * scale1 + shift


def _unpack(w):
    lo = lax.bitcast_convert_type(w << 16, F32)
    hi = lax.bitcast_convert_type(w & jnp.uint32(0xFFFF0000), F32)
    return lo, hi


def _ld(ref, r):
    return pltpu.bitcast(ref[r, :], BF16)


def _mix(a, na=1, b=(), nb=0):
    b = iter(b)
    done = 0
    for k, _ in enumerate(a):
        while done * na < (k + 1) * nb:
            next(b)
            done += 1
    for _ in b:
        pass


def _bf16_bits(x):
    return lax.bitcast_convert_type(x.astype(BF16).astype(F32), U32)


def _kernel(x_hbm, wqkv_hbm, wo_hbm, wg_hbm, wu_hbm, wd_hbm, c_ref, wmod_hbm, out_hbm,
            x_v, wqkv_v, wo_v, wg_v, wu_v, wd_v, wmod_v, h_v, qkv0_v, qkv1_v, t_v, q_s, k_s, v_s,
            ot_v, o_v, o3_v, x1_v, x2_v, a_v, ob_v, scol_v, mod_v, sem_x, sem_qkv, sem_mod, sem_head, sem_w, sem_o):
    nb1 = S // TM1
    qkv_v = (qkv0_v, qkv1_v)

    def x_cp(i):
        r = pl.ds(i * TM1, TM1)
        return pltpu.make_async_copy(x_hbm.at[r], x_v.at[r], sem_x.at[i])

    def qkv_cp(g, t):
        return pltpu.make_async_copy(wqkv_hbm.at[:, pl.ds(t * D + g * GW, GW)],
                                     wqkv_v.at[g, :, pl.ds(t * GW, GW)], sem_qkv.at[g * 3 + t])

    def mod_cp(i):
        return pltpu.make_async_copy(wmod_hbm.at[:, pl.ds(i * D, D)], wmod_v.at[i], sem_mod.at[i])

    def mod_head_cp(i):
        return pltpu.make_async_copy(wmod_hbm.at[:, pl.ds(i * MC, MC)],
                                     wmod_v.at[i * MC // D, :, pl.ds(i * MC % D, MC)], sem_head.at[i])

    w_cps = [pltpu.make_async_copy(s, d, sem_w.at[i]) for i, (s, d) in enumerate(
        ((wo_hbm, wo_v), (wg_hbm, wg_v), (wu_hbm, wu_v), (wd_hbm, wd_v)))]

    def out_cp(i, n):
        cs = pl.ds(pl.multiple_of(n * DC, DC), DC)
        return pltpu.make_async_copy(ob_v.at[n], out_hbm.at[pl.ds(i * TM, TM), cs], sem_o.at[n])

    nm = 2 * D // MC
    head = [mod_head_cp(i) for i in range(nm)] + [x_cp(0)] + [qkv_cp(0, t) for t in range(3)]
    head += [x_cp(i) for i in range(1, nb1)]
    for cp in head[:STAGE[0]]:
        cp.start()

    cf = c_ref[...].astype(F32)
    sc = (cf * jax.nn.sigmoid(cf)).astype(BF16)
    scol_v[...] = jnp.broadcast_to(sc.astype(F32), (128, D)).T
    sc8 = jnp.broadcast_to(sc, (16, D))
    for i in range(nm):
        mod_head_cp(i).wait()
        for cp in head[STAGE[i]:STAGE[i + 1]]:
            cp.start()
        cs = pl.ds(i * MC % D, MC)
        mod_v[i * MC // D, :, cs] = _dot(sc8, wmod_v[i * MC // D, :, cs])[:8]

    def mod_vpu(i, n):
        cs = pl.ds(pl.multiple_of(n * 128, 128), 128)
        p = wmod_v[i, :, cs].astype(F32) * scol_v[...]
        mod_v[i, :, cs] = jnp.broadcast_to(jnp.sum(p, axis=0, keepdims=True), (8, 128))
        yield

    def mod_row(i):
        return mod_v[i, pl.ds(0, 1), :]

    dep = [None]

    def rows(i, n):
        return pl.ds(pl.multiple_of(i * n, n), n)

    def tied(h, i, n):
        k0 = h.shape[1] - n
        late = jnp.tile(lax.bitcast_convert_type(dep[0], U32), (h.shape[0] // 8, n // 128))
        late = jnp.where(i < 0, late, h[:, k0:])
        return jnp.concatenate([h[:, :k0], late], axis=1) if k0 else late

    def proj(g, i, tie=False):
        for t in range(3):
            h = h_v[rows(i, TM1 // 2), :]
            if tie and t == 2:
                h = tied(h, i, TIE)
            y = _dot(pltpu.bitcast(h, BF16), wqkv_v[g, :, pl.ds(t * GW, GW)])
            y = pltpu.bitcast(y.astype(BF16), U32)
            for n in range(2):
                qkv_v[g % 2][t * 2 + n, rows(i, TM1 // 2), :] = y[:, n * 128:(n + 1) * 128]
            yield

    def att_load(g, j, u):
        for t, dst in enumerate((q_s, k_s, v_s)):
            for n in range(2):
                w = qkv_v[g % 2][t * 2 + n, pl.ds(j, 128, stride=NJ), :]
                wt = w.T
                for h in range(4):
                    t_v[u * 3 + t, pl.ds((n * 4 + h) * HP, DH), :] = wt[h * DH:(h + 1) * DH]
            for d in range(DH):
                w = t_v[u * 3 + t, pl.ds(d, 8, stride=HP), :]
                r = pl.ds(d * 8, 8)
                if t == 0:
                    dst[0, j, r, :], dst[1, j, r, :] = _unpack(w)
                else:
                    dst[0, NJ + j, r, :], dst[1, NJ + j, r, :] = _unpack(w)
                    dst[0, j, r, :], dst[1, j, r, :] = _unpack(pltpu.roll(w, 1, 1))
            yield

    def att_core(dst, base, j, u):
        qws, ch = CFG[u]
        lane0 = lax.broadcasted_iota(jnp.int32, (8, 128), 1) == 0
        probs = []
        for p in range(2):
            acc = [None] * W
            qw = qws[p]
            for w0 in range(0, W, qw):
                for d in range(DH):
                    r = pl.ds(d * 8, 8)
                    q = q_s[p, j, r, :]
                    if d == 0 and dep[0] is not None:
                        q = jnp.where(j < 0, dep[0], q)
                    for w in range(w0, w0 + qw):
                        t = q * k_s[p, j + (NJ - w), r, :]
                        acc[w] = t if d == 0 else acc[w] + t
                dep[0] = acc[w0]
            lg = [acc[0] * DH ** -0.5]
            for w in range(1, W):
                lg.append(jnp.where(jnp.logical_and(lane0, j < w), -1e9, acc[w] * DH ** -0.5))
            m = lg[0]
            for w in range(1, W):
                m = jnp.maximum(m, lg[w])
            e = [jnp.exp(l - m) for l in lg]
            den = e[0]
            for w in range(1, W):
                den = den + e[w]
            inv = 1.0 / den
            probs.append([x * inv for x in e])
            dep[0] = inv
            yield
        for d in range(DH):
            r = pl.ds(d * 8, 8)
            o = []
            for p in range(2):
                acc = probs[p][0] * v_s[p, j + NJ, r, :]
                for w in range(1, W):
                    acc = acc + probs[p][w] * v_s[p, j + (NJ - w), r, :]
                o.append(_bf16_bits(acc))
                if d % ch == ch - 1:
                    probs[p][0] = jnp.where(j < 0, acc, probs[p][0])
                    dep[0] = acc
            ot_v[u, pl.ds(d, 8, stride=HP), :] = (o[0] >> 16) | o[1]
        for n in range(2):
            ot = jnp.concatenate([ot_v[u, pl.ds((n * 4 + h) * HP, DH), :] for h in range(4)], axis=0)
            dst[base + n, pl.ds(j, 128, stride=NJ), :] = ot.T
        yield

    def o_cols(ref, r):
        return jnp.concatenate([ref[n, r, :] for n in range(ref.shape[0])], axis=1)

    def ln1(i):
        for k in range(TM1 // LR):
            b = i * (TM1 // LR) + k
            h = _ln_mod(x_v[rows(b, LR), :].astype(F32), 1.0 + mod_row(1), mod_row(0))
            h_v[rows(b, LR // 2), :] = pltpu.bitcast(h.astype(BF16), U32)

    def ln2(i):
        y = _dot(pltpu.bitcast(o_cols(o3_v, rows(i, LB // 2)), BF16), wo_v[pl.ds((HG - 1) * GW, GW), :])
        for k in range(LB // LR):
            b = i * (LB // LR) + k
            r = rows(b, LR)
            x1 = x_v[r, :].astype(F32) + mod_row(2) * (x1_v[r, :] + y[k * LR:(k + 1) * LR])
            x2_v[r, :] = x1
            h = _ln_mod(x1, 1.0 + mod_row(4), mod_row(3))
            dep[0] = h[-8:, -128:]
            h_v[rows(b, LR // 2), :] = pltpu.bitcast(h.astype(BF16), U32)

    def prefetch(g):
        nxt = [qkv_cp(g + 1, t) for t in range(3)] if g + 1 < HG else []
        for cp in nxt + [mod_cp(g + 2), w_cps[(g + 1) % HG]]:
            cp.start()

    x_cp(0).wait()
    ln1(0)
    for t in range(3):
        qkv_cp(0, t).wait()

    def first_body(i, carry):
        @pl.when(i + 1 < nb1)
        def _():
            x_cp(i + 1).wait()

        @pl.when(i == PF0)
        def _():
            prefetch(0)
        _mix(proj(0, i))
        ln1(jnp.minimum(i + 1, nb1 - 1))
        return carry
    lax.fori_loop(0, nb1, first_body, 0)

    half = nb1 // 2
    jpb = NJ // half

    def loads(g, j0, nj):
        for u in range(nj):
            yield from att_load(g, j0 + u, u)
            yield from mod_vpu(g + 2, j0 + u)

    def cores(g, i):
        dst, base = (o_v, g * 2) if g + 1 < HG else (o3_v, 0)
        for u in range(jpb):
            yield from att_core(dst, base, i * jpb + u, u)

    def wo_part(i, tie=False):
        for n in range(D // GW):
            cs = pl.ds(n * GW, GW)
            o = o_cols(o_v, rows(i, TM1 // 2))
            if tie and n == D // GW - 1:
                o = tied(o, i, TIW)
            x1_v[rows(i, TM1), cs] = _dot(pltpu.bitcast(o, BF16), wo_v[pl.ds(0, (HG - 1) * GW), cs])
            yield

    def overlapped(g, matmul, steps, na):
        nj = NJ // na

        def body_a(i, c):
            _mix(matmul(i), steps, loads(g, i * nj, nj), 4 * nj)
            return c
        lax.fori_loop(0, na, body_a, 0)

        def body_b(i, carry):
            dep[0] = None
            _mix(cores(g, i))
            _mix(matmul(na + i, True))
            return carry
        lax.fori_loop(0, half, body_b, 0)

    for g in range(1, HG):
        for t in range(3):
            qkv_cp(g, t).wait()
        mod_cp(g + 1).wait()
        prefetch(g)
        overlapped(g - 1, lambda i, tie=False, g=g: proj(g, i, tie), 3, half)

    mod_cp(5).wait()
    w_cps[0].wait()
    nd = D // DC
    nlate = TM // TM1
    overlapped(HG - 1, wo_part, D // GW, half - nlate)

    def late_body(i, c):
        for k in range(nd // nlate):
            ln2(i * (nd // nlate) + k)
        _mix(wo_part(nb1 - nlate + i, True))
        return c
    lax.fori_loop(0, nlate, late_body, 0)
    for cp in w_cps[1:]:
        cp.wait()

    nb = S // TM

    def ffn_body(i, c):
        r = rows(i, TM)

        def gu(f, c2):
            cs = rows(f, FC)
            h = _ld(h_v, rows(i, TM // 2))
            gate = _dot(h, wg_v[:, cs])
            up = _dot(h, wu_v[:, cs])
            a_v[:, cs] = pltpu.bitcast((gate * jax.nn.sigmoid(gate) * up).astype(BF16), U32)
            return c2
        lax.fori_loop(0, F // FC, gu, 0)

        @pl.when(i >= 1)
        def _():
            for n in range(nd):
                out_cp(i - 1, n).wait()

        def dn(n, with_ln):
            if with_ln:
                ln2((i + 1) * nd + n)
            cs = rows(n, DC)
            y2 = _dot(_ld(a_v, slice(None)), wd_v[:, cs])
            ob_v[n] = (x2_v[r, cs] + mod_v[5, pl.ds(0, 1), cs] * y2).astype(BF16)
            out_cp(i, n).start()

        @pl.when(i < nb - 1)
        def _():
            lax.fori_loop(0, nd, lambda n, c2: dn(n, True), None)

        @pl.when(i == nb - 1)
        def _():
            lax.fori_loop(0, nd, lambda n, c2: dn(n, False), None)
        return c
    lax.fori_loop(0, nb, ffn_body, 0)
    for n in range(nd):
        out_cp(nb - 1, n).wait()


@jax.jit
def pallas_adaLN_cond__sliding_local_dilated__swiglu_ffn__prompt_kernel(
    A_x: jax.Array,
    A_wqkv: jax.Array,
    A_wo: jax.Array,
    B_x: jax.Array,
    B_w_gate: jax.Array,
    B_w_up: jax.Array,
    B_w_down: jax.Array,
    c: jax.Array,
    w_mod: jax.Array,
):
    del B_x
    hbm = pl.BlockSpec(memory_space=pl.ANY)
    dma = pltpu.SemaphoreType.DMA
    out = pl.pallas_call(
        _kernel,
        out_shape=jax.ShapeDtypeStruct((S, D), BF16),
        in_specs=[hbm] * 6 + [pl.BlockSpec(memory_space=pltpu.VMEM), hbm],
        out_specs=hbm,
        scratch_shapes=[
            pltpu.VMEM((S, D), BF16),
            pltpu.VMEM((HG, D, 3 * GW), BF16),
            pltpu.VMEM((D, D), BF16),
            pltpu.VMEM((D, F), BF16),
            pltpu.VMEM((D, F), BF16),
            pltpu.VMEM((F, D), BF16),
            pltpu.VMEM((6, D, D), BF16),
            pltpu.VMEM((S // 2, D), U32),
            pltpu.VMEM((6, S // 2, 128), U32),
            pltpu.VMEM((6, S // 2, 128), U32),
            pltpu.VMEM((12, 8 * HP, 128), U32),
            pltpu.VMEM((2, NJ, GW, 128), F32),
            pltpu.VMEM((2, 2 * NJ, GW, 128), F32),
            pltpu.VMEM((2, 2 * NJ, GW, 128), F32),
            pltpu.VMEM((2, 8 * HP, 128), U32),
            pltpu.VMEM((2 * HG - 2, S // 2, 128), U32),
            pltpu.VMEM((2, S // 2, 128), U32),
            pltpu.VMEM((S, D), F32),
            pltpu.VMEM((S, D), F32),
            pltpu.VMEM((TM // 2, F), U32),
            pltpu.VMEM((D // DC, TM, DC), BF16),
            pltpu.VMEM((D, 128), F32),
            pltpu.VMEM((6, 8, D), F32),
            dma((S // TM1,)), dma((HG * 3,)), dma((6,)), dma((2 * D // MC,)), dma((4,)), dma((D // DC,)),
        ],
        compiler_params=pltpu.CompilerParams(vmem_limit_bytes=120 * 1024 * 1024,
            flags={"XLA_TPU_EVENLY_DISTRIBUTE_CRITICAL_NODES": True}),
    )(A_x.reshape(S, D), A_wqkv, A_wo, B_w_gate, B_w_up, B_w_down, c, w_mod)
    return out.reshape(1, S, D)
```

```python
import jax
import jax.numpy as jnp
from jax import lax
from jax.experimental import pallas as pl
from jax.experimental.pallas import tpu as pltpu

S, D, F = 2048, 1024, 3584
DH, W = 32, 8
HG, GW = 4, 256
NJ = 8
TM1 = 256
TM = 512
FC = 896
DC = 256
LB = TM * DC // D
HP = 36
CFG = (((2, 4), 1), ((2, 4), 1))
MC = 512
STAGE = (4, 4, 6, 8, 99)
PF0 = 2
LR = 128
TIE, TIW = 512, 768
EPS = 1e-5
F32, BF16, U32 = jnp.float32, jnp.bfloat16, jnp.uint32


def _dot(a, b):
    return jnp.dot(a, b, preferred_element_type=F32)


def _ln_mod(x, scale1, shift):
    m = jnp.mean(x, axis=-1, keepdims=True)
    xc = x - m
    v = jnp.mean(xc * xc, axis=-1, keepdims=True)
    return xc * lax.rsqrt(v + EPS) * scale1 + shift


def _unpack(w):
    lo = lax.bitcast_convert_type(w << 16, F32)
    hi = lax.bitcast_convert_type(w & jnp.uint32(0xFFFF0000), F32)
    return lo, hi


def _ld(ref, r):
    return pltpu.bitcast(ref[r, :], BF16)


def _mix(a, na=1, b=(), nb=0):
    b = iter(b)
    done = 0
    for k, _ in enumerate(a):
        while done * na < (k + 1) * nb:
            next(b)
            done += 1
    for _ in b:
        pass


def _bf16_bits(x):
    return lax.bitcast_convert_type(x.astype(BF16).astype(F32), U32)


def _kernel(x_hbm, wqkv_hbm, wo_hbm, wg_hbm, wu_hbm, wd_hbm, c_ref, wmod_hbm, out_hbm,
            x_v, wqkv_v, wo_v, wg_v, wu_v, wd_v, wmod_v, h_v, qkv0_v, qkv1_v, t_v, q_s, k_s, v_s,
            ot_v, o_v, o3_v, x1_v, x2_v, a_v, ob_v, scol_v, mod_v, sem_x, sem_qkv, sem_mod, sem_head, sem_w, sem_o):
    nb1 = S // TM1
    qkv_v = (qkv0_v, qkv1_v)

    def x_cp(i):
        r = pl.ds(i * TM1, TM1)
        return pltpu.make_async_copy(x_hbm.at[r], x_v.at[r], sem_x.at[i])

    def qkv_cp(g, t):
        return pltpu.make_async_copy(wqkv_hbm.at[:, pl.ds(t * D + g * GW, GW)],
                                     wqkv_v.at[g, :, pl.ds(t * GW, GW)], sem_qkv.at[g * 3 + t])

    def mod_cp(i):
        return pltpu.make_async_copy(wmod_hbm.at[:, pl.ds(i * D, D)], wmod_v.at[i], sem_mod.at[i])

    def mod_head_cp(i):
        return pltpu.make_async_copy(wmod_hbm.at[:, pl.ds(i * MC, MC)],
                                     wmod_v.at[i * MC // D, :, pl.ds(i * MC % D, MC)], sem_head.at[i])

    w_cps = [pltpu.make_async_copy(s, d, sem_w.at[i]) for i, (s, d) in enumerate(
        ((wo_hbm, wo_v), (wg_hbm, wg_v), (wu_hbm, wu_v), (wd_hbm, wd_v)))]

    def out_cp(i, n):
        cs = pl.ds(pl.multiple_of(n * DC, DC), DC)
        return pltpu.make_async_copy(ob_v.at[n], out_hbm.at[pl.ds(i * TM, TM), cs], sem_o.at[n])

    nm = 2 * D // MC
    head = [mod_head_cp(i) for i in range(nm)] + [x_cp(0)] + [qkv_cp(0, t) for t in range(3)]
    head += [x_cp(i) for i in range(1, nb1)]
    for cp in head[:STAGE[0]]:
        cp.start()

    cf = c_ref[...].astype(F32)
    sc = (cf * jax.nn.sigmoid(cf)).astype(BF16)
    scol_v[...] = jnp.broadcast_to(sc.astype(F32), (128, D)).T
    sc8 = jnp.broadcast_to(sc, (16, D))
    for i in range(nm):
        mod_head_cp(i).wait()
        for cp in head[STAGE[i]:STAGE[i + 1]]:
            cp.start()
        cs = pl.ds(i * MC % D, MC)
        mod_v[i * MC // D, :, cs] = _dot(sc8, wmod_v[i * MC // D, :, cs])[:8]

    def mod_vpu(i, n):
        cs = pl.ds(pl.multiple_of(n * 128, 128), 128)
        p = wmod_v[i, :, cs].astype(F32) * scol_v[...]
        mod_v[i, :, cs] = jnp.broadcast_to(jnp.sum(p, axis=0, keepdims=True), (8, 128))
        yield

    def mod_row(i):
        return mod_v[i, pl.ds(0, 1), :]

    dep = [None]

    def rows(i, n):
        return pl.ds(pl.multiple_of(i * n, n), n)

    def tied(h, i, n):
        k0 = h.shape[1] - n
        late = jnp.tile(lax.bitcast_convert_type(dep[0], U32), (h.shape[0] // 8, n // 128))
        late = jnp.where(i < 0, late, h[:, k0:])
        return jnp.concatenate([h[:, :k0], late], axis=1) if k0 else late

    def proj(g, i, tie=False):
        for t in range(3):
            h = h_v[rows(i, TM1 // 2), :]
            if tie and t == 2:
                h = tied(h, i, TIE)
            y = _dot(pltpu.bitcast(h, BF16), wqkv_v[g, :, pl.ds(t * GW, GW)])
            y = pltpu.bitcast(y.astype(BF16), U32)
            for n in range(2):
                qkv_v[g % 2][t * 2 + n, rows(i, TM1 // 2), :] = y[:, n * 128:(n + 1) * 128]
            yield

    def att_load(g, j, u):
        for t, dst in enumerate((q_s, k_s, v_s)):
            for n in range(2):
                w = qkv_v[g % 2][t * 2 + n, pl.ds(j, 128, stride=NJ), :]
                wt = w.T
                for h in range(4):
                    t_v[u * 3 + t, pl.ds((n * 4 + h) * HP, DH), :] = wt[h * DH:(h + 1) * DH]
            for d in range(DH):
                w = t_v[u * 3 + t, pl.ds(d, 8, stride=HP), :]
                r = pl.ds(d * 8, 8)
                if t == 0:
                    dst[0, j, r, :], dst[1, j, r, :] = _unpack(w)
                else:
                    dst[0, NJ + j, r, :], dst[1, NJ + j, r, :] = _unpack(w)
                    dst[0, j, r, :], dst[1, j, r, :] = _unpack(pltpu.roll(w, 1, 1))
            yield

    def att_core(dst, base, j, u):
        qws, ch = CFG[u]
        lane0 = lax.broadcasted_iota(jnp.int32, (8, 128), 1) == 0
        probs = []
        for p in range(2):
            acc = [None] * W
            qw = qws[p]
            for w0 in range(0, W, qw):
                for d in range(DH):
                    r = pl.ds(d * 8, 8)
                    q = q_s[p, j, r, :]
                    if d == 0 and dep[0] is not None:
                        q = jnp.where(j < 0, dep[0], q)
                    for w in range(w0, w0 + qw):
                        t = q * k_s[p, j + (NJ - w), r, :]
                        acc[w] = t if d == 0 else acc[w] + t
                dep[0] = acc[w0]
            lg = [acc[0] * DH ** -0.5]
            for w in range(1, W):
                lg.append(jnp.where(jnp.logical_and(lane0, j < w), -1e9, acc[w] * DH ** -0.5))
            m = lg[0]
            for w in range(1, W):
                m = jnp.maximum(m, lg[w])
            e = [jnp.exp(l - m) for l in lg]
            den = e[0]
            for w in range(1, W):
                den = den + e[w]
            inv = 1.0 / den
            probs.append([x * inv for x in e])
            dep[0] = inv
            yield
        for d in range(DH):
            r = pl.ds(d * 8, 8)
            o = []
            for p in range(2):
                acc = probs[p][0] * v_s[p, j + NJ, r, :]
                for w in range(1, W):
                    acc = acc + probs[p][w] * v_s[p, j + (NJ - w), r, :]
                o.append(_bf16_bits(acc))
                if d % ch == ch - 1:
                    probs[p][0] = jnp.where(j < 0, acc, probs[p][0])
                    dep[0] = acc
            ot_v[u, pl.ds(d, 8, stride=HP), :] = (o[0] >> 16) | o[1]
        for n in range(2):
            ot = jnp.concatenate([ot_v[u, pl.ds((n * 4 + h) * HP, DH), :] for h in range(4)], axis=0)
            dst[base + n, pl.ds(j, 128, stride=NJ), :] = ot.T
        yield

    def o_cols(ref, r):
        return jnp.concatenate([ref[n, r, :] for n in range(ref.shape[0])], axis=1)

    def ln1(i):
        for k in range(TM1 // LR):
            b = i * (TM1 // LR) + k
            h = _ln_mod(x_v[rows(b, LR), :].astype(F32), 1.0 + mod_row(1), mod_row(0))
            h_v[rows(b, LR // 2), :] = pltpu.bitcast(h.astype(BF16), U32)

    def ln2(i):
        y = _dot(pltpu.bitcast(o_cols(o3_v, rows(i, LB // 2)), BF16), wo_v[pl.ds((HG - 1) * GW, GW), :])
        for k in range(LB // LR):
            b = i * (LB // LR) + k
            r = rows(b, LR)
            x1 = x_v[r, :].astype(F32) + mod_row(2) * (x1_v[r, :] + y[k * LR:(k + 1) * LR])
            x2_v[r, :] = x1
            h = _ln_mod(x1, 1.0 + mod_row(4), mod_row(3))
            dep[0] = h[-8:, -128:]
            h_v[rows(b, LR // 2), :] = pltpu.bitcast(h.astype(BF16), U32)

    def prefetch(g):
        nxt = [qkv_cp(g + 1, t) for t in range(3)] if g + 1 < HG else []
        for cp in nxt + [mod_cp(g + 2)] + ([w_cps[0]] if g == 3 else []):
            cp.start()

    x_cp(0).wait()
    ln1(0)
    for t in range(3):
        qkv_cp(0, t).wait()

    def first_body(i, carry):
        @pl.when(i + 1 < nb1)
        def _():
            x_cp(i + 1).wait()

        @pl.when(i == PF0)
        def _():
            prefetch(0)
        _mix(proj(0, i))
        ln1(jnp.minimum(i + 1, nb1 - 1))
        return carry
    lax.fori_loop(0, nb1, first_body, 0)

    half = nb1 // 2
    jpb = NJ // half

    def loads(g, j0, nj):
        for u in range(nj):
            yield from att_load(g, j0 + u, u)
            if g + 1 < HG:
                yield from mod_vpu(g + 2, j0 + u)

    def cores(g, i):
        dst, base = (o_v, g * 2) if g + 1 < HG else (o3_v, 0)
        for u in range(jpb):
            yield from att_core(dst, base, i * jpb + u, u)

    def wo_part(i, tie=False):
        for n in range(D // GW):
            cs = pl.ds(n * GW, GW)
            o = o_cols(o_v, rows(i, TM1 // 2))
            if tie and n == D // GW - 1:
                o = tied(o, i, TIW)
            x1_v[rows(i, TM1), cs] = _dot(pltpu.bitcast(o, BF16), wo_v[pl.ds(0, (HG - 1) * GW), cs])
            yield

    def overlapped(g, matmul, steps, na):
        nj = NJ // na

        def body_a(i, c):
            _mix(matmul(i), steps, loads(g, i * nj, nj), (4 if g + 1 < HG else 3) * nj)
            return c
        lax.fori_loop(0, na, body_a, 0)
        if g < 3:
            w_cps[g + 1].start()

        def body_b(i, carry):
            dep[0] = None
            _mix(cores(g, i))
            _mix(matmul(na + i, True))
            return carry
        lax.fori_loop(0, half, body_b, 0)

    for g in range(1, HG):
        for t in range(3):
            qkv_cp(g, t).wait()
        mod_cp(g + 1).wait()
        prefetch(g)
        overlapped(g - 1, lambda i, tie=False, g=g: proj(g, i, tie), 3, half)

    mod_cp(5).wait()
    w_cps[0].wait()
    nd = D // DC
    nlate = TM // TM1
    overlapped(HG - 1, wo_part, D // GW, half - nlate)

    def late_body(i, c):
        for k in range(nd // nlate):
            ln2(i * (nd // nlate) + k)
        _mix(wo_part(nb1 - nlate + i))
        for k in range(NJ // nlate):
            _mix(mod_vpu(5, i * (NJ // nlate) + k))
        return c
    lax.fori_loop(0, nlate, late_body, 0)
    for cp in w_cps[1:]:
        cp.wait()

    nb = S // TM

    def ffn_body(i, c):
        r = rows(i, TM)

        def gu(f, c2):
            cs = rows(f, FC)
            h = _ld(h_v, rows(i, TM // 2))
            gate = _dot(h, wg_v[:, cs])
            up = _dot(h, wu_v[:, cs])
            a_v[:, cs] = pltpu.bitcast((gate * jax.nn.sigmoid(gate) * up).astype(BF16), U32)
            return c2
        lax.fori_loop(0, F // FC, gu, 0)

        @pl.when(i >= 1)
        def _():
            for n in range(nd):
                out_cp(i - 1, n).wait()

        def dn(n, with_ln):
            if with_ln:
                ln2((i + 1) * nd + n)
            cs = rows(n, DC)
            y2 = _dot(_ld(a_v, slice(None)), wd_v[:, cs])
            ob_v[n] = (x2_v[r, cs] + mod_v[5, pl.ds(0, 1), cs] * y2).astype(BF16)
            out_cp(i, n).start()

        @pl.when(i < nb - 1)
        def _():
            lax.fori_loop(0, nd, lambda n, c2: dn(n, True), None)

        @pl.when(i == nb - 1)
        def _():
            lax.fori_loop(0, nd, lambda n, c2: dn(n, False), None)
        return c
    lax.fori_loop(0, nb, ffn_body, 0)
    for n in range(nd):
        out_cp(nb - 1, n).wait()


@jax.jit
def pallas_adaLN_cond__sliding_local_dilated__swiglu_ffn__prompt_kernel(
    A_x: jax.Array,
    A_wqkv: jax.Array,
    A_wo: jax.Array,
    B_x: jax.Array,
    B_w_gate: jax.Array,
    B_w_up: jax.Array,
    B_w_down: jax.Array,
    c: jax.Array,
    w_mod: jax.Array,
):
    del B_x
    hbm = pl.BlockSpec(memory_space=pl.ANY)
    dma = pltpu.SemaphoreType.DMA
    out = pl.pallas_call(
        _kernel,
        out_shape=jax.ShapeDtypeStruct((S, D), BF16),
        in_specs=[hbm] * 6 + [pl.BlockSpec(memory_space=pltpu.VMEM), hbm],
        out_specs=hbm,
        scratch_shapes=[
            pltpu.VMEM((S, D), BF16),
            pltpu.VMEM((HG, D, 3 * GW), BF16),
            pltpu.VMEM((D, D), BF16),
            pltpu.VMEM((D, F), BF16),
            pltpu.VMEM((D, F), BF16),
            pltpu.VMEM((F, D), BF16),
            pltpu.VMEM((6, D, D), BF16),
            pltpu.VMEM((S // 2, D), U32),
            pltpu.VMEM((6, S // 2, 128), U32),
            pltpu.VMEM((6, S // 2, 128), U32),
            pltpu.VMEM((12, 8 * HP, 128), U32),
            pltpu.VMEM((2, NJ, GW, 128), F32),
            pltpu.VMEM((2, 2 * NJ, GW, 128), F32),
            pltpu.VMEM((2, 2 * NJ, GW, 128), F32),
            pltpu.VMEM((2, 8 * HP, 128), U32),
            pltpu.VMEM((2 * HG - 2, S // 2, 128), U32),
            pltpu.VMEM((2, S // 2, 128), U32),
            pltpu.VMEM((S, D), F32),
            pltpu.VMEM((S, D), F32),
            pltpu.VMEM((TM // 2, F), U32),
            pltpu.VMEM((D // DC, TM, DC), BF16),
            pltpu.VMEM((D, 128), F32),
            pltpu.VMEM((6, 8, D), F32),
            dma((S // TM1,)), dma((HG * 3,)), dma((6,)), dma((2 * D // MC,)), dma((4,)), dma((D // DC,)),
        ],
        compiler_params=pltpu.CompilerParams(vmem_limit_bytes=120 * 1024 * 1024,
            flags={"XLA_TPU_EVENLY_DISTRIBUTE_CRITICAL_NODES": True}),
    )(A_x.reshape(S, D), A_wqkv, A_wo, B_w_gate, B_w_up, B_w_down, c, w_mod)
    return out.reshape(1, S, D)
```

```python
import jax
import jax.numpy as jnp
from jax import lax
from jax.experimental import pallas as pl
from jax.experimental.pallas import tpu as pltpu

S, D, F = 2048, 1024, 3584
DH, W = 32, 8
HG, GW = 4, 256
NJ = 8
TM1 = 256
TM = 512
FC = 256
DC = 256
HM, HD, HF = TM // 2, D // 2, F // 2
LB = 64
HP = 36
CFG = (((2, 4), 1), ((2, 4), 1))
MC = 512
STAGE = (4, 4, 6, 8, 99)
PF0 = 2
LR = 128
TIE, TIW = 512, 768
PC = 128
EPS = 1e-5
F32, BF16, U32 = jnp.float32, jnp.bfloat16, jnp.uint32


def _dot(a, b):
    return jnp.dot(a, b, preferred_element_type=F32)


def _ln_mod(x, scale1, shift):
    m = jnp.mean(x, axis=-1, keepdims=True)
    xc = x - m
    v = jnp.mean(xc * xc, axis=-1, keepdims=True)
    return xc * lax.rsqrt(v + EPS) * scale1 + shift


def _unpack(w):
    lo = lax.bitcast_convert_type(w << 16, F32)
    hi = lax.bitcast_convert_type(w & jnp.uint32(0xFFFF0000), F32)
    return lo, hi


def _ld(ref, r):
    return pltpu.bitcast(ref[r, :], BF16)


def _mix(a, na=1, b=(), nb=0):
    b = iter(b)
    done = 0
    for k, _ in enumerate(a):
        while done * na < (k + 1) * nb:
            next(b)
            done += 1
    for _ in b:
        pass


def _lhs_terms(a11, a12, a21, a22):
    terms = (a11 + a22, a21 + a22, a11, a22, a11 + a12, a21 - a11, a12 - a22)
    return [pltpu.bitcast(t.astype(BF16), U32) for t in terms]


def _rhs_terms(b11, b12, b21, b22):
    halves = [(b11 + b22, b12 - b22, b21 - b11, b11 + b12, b21 + b22)
              for b11, b12, b21, b22 in zip(*(_unpack(b) for b in (b11, b12, b21, b22)))]
    return [pltpu.pack_elementwise([lo, hi], packed_dtype=BF16) for lo, hi in zip(*halves)]


def _strassen(lhs, rhs):
    p1, p2, p3, p4, p5, p6, p7 = (_dot(pltpu.bitcast(a, BF16), pltpu.bitcast(b, BF16)) for a, b in zip(lhs, rhs))
    return p1 + p4 - p5 + p7, p3 + p5, p2 + p4, p1 - p2 + p3 + p6


def _bf16_bits(x):
    return lax.bitcast_convert_type(x.astype(BF16).astype(F32), U32)


def _kernel(x_hbm, wqkv_hbm, wo_hbm, wg_hbm, wu_hbm, wd_hbm, c_ref, wmod_hbm, out_hbm,
            x_v, wqkv_v, wo_v, wg_v, wu_v, wd_v, wmod_v, h_v, qkv0_v, qkv1_v, t_v, q_s, k_s, v_s,
            ot_v, o_v, o3_v, x1_v, x2_v, hs_v, as_v, sg_v, sd_v, ob_v, scol_v, mod_v, sem_x, sem_qkv, sem_mod, sem_head, sem_w, sem_o):
    nb1 = S // TM1
    qkv_v = (qkv0_v, qkv1_v)

    def x_cp(i):
        r = pl.ds(i * TM1, TM1)
        return pltpu.make_async_copy(x_hbm.at[r], x_v.at[r], sem_x.at[i])

    def qkv_cp(g, t):
        return pltpu.make_async_copy(wqkv_hbm.at[:, pl.ds(t * D + g * GW, GW)],
                                     wqkv_v.at[g, :, pl.ds(t * GW, GW)], sem_qkv.at[g * 3 + t])

    def mod_cp(i):
        return pltpu.make_async_copy(wmod_hbm.at[:, pl.ds(i * D, D)], wmod_v.at[i], sem_mod.at[i])

    def mod_head_cp(i):
        return pltpu.make_async_copy(wmod_hbm.at[:, pl.ds(i * MC, MC)],
                                     wmod_v.at[i * MC // D, :, pl.ds(i * MC % D, MC)], sem_head.at[i])

    w_cps = [pltpu.make_async_copy(s, d, sem_w.at[i]) for i, (s, d) in enumerate(
        ((wo_hbm, wo_v), (wg_hbm, wg_v.bitcast(BF16)), (wu_hbm, wu_v.bitcast(BF16)), (wd_hbm, wd_v.bitcast(BF16))))]

    def out_cp(i, n):
        cs = pl.ds(pl.multiple_of(n * DC, DC), DC)
        return pltpu.make_async_copy(ob_v.at[n], out_hbm.at[pl.ds(i * TM, TM), cs], sem_o.at[n])

    nm = 2 * D // MC
    head = [mod_head_cp(i) for i in range(nm)] + [x_cp(0)] + [qkv_cp(0, t) for t in range(3)]
    head += [x_cp(i) for i in range(1, nb1)]
    for cp in head[:STAGE[0]]:
        cp.start()

    cf = c_ref[...].astype(F32)
    sc = (cf * jax.nn.sigmoid(cf)).astype(BF16)
    scol_v[...] = jnp.broadcast_to(sc.astype(F32), (128, D)).T
    sc8 = jnp.broadcast_to(sc, (16, D))
    for i in range(nm):
        mod_head_cp(i).wait()
        for cp in head[STAGE[i]:STAGE[i + 1]]:
            cp.start()
        cs = pl.ds(i * MC % D, MC)
        mod_v[i * MC // D, :, cs] = _dot(sc8, wmod_v[i * MC // D, :, cs])[:8]

    def mod_vpu(i, n):
        cs = pl.ds(pl.multiple_of(n * 128, 128), 128)
        p = wmod_v[i, :, cs].astype(F32) * scol_v[...]
        mod_v[i, :, cs] = jnp.broadcast_to(jnp.sum(p, axis=0, keepdims=True), (8, 128))
        yield

    def mod_row(i):
        return mod_v[i, pl.ds(0, 1), :]

    dep = [None]

    def rows(i, n):
        return pl.ds(pl.multiple_of(i * n, n), n)

    def tied(h, i, n):
        k0 = h.shape[1] - n
        late = jnp.tile(lax.bitcast_convert_type(dep[0], U32), (h.shape[0] // 8, n // 128))
        late = jnp.where(i < 0, late, h[:, k0:])
        return jnp.concatenate([h[:, :k0], late], axis=1) if k0 else late

    def proj(g, i, tie=False):
        for t in range(3):
            h = h_v[rows(i, TM1 // 2), :]
            if tie and t == 2:
                h = tied(h, i, TIE)
            y = _dot(pltpu.bitcast(h, BF16), wqkv_v[g, :, pl.ds(t * GW, GW)])
            y = pltpu.bitcast(y.astype(BF16), U32)
            for n in range(2):
                qkv_v[g % 2][t * 2 + n, rows(i, TM1 // 2), :] = y[:, n * 128:(n + 1) * 128]
            yield

    def att_load(g, j, u):
        for t, dst in enumerate((q_s, k_s, v_s)):
            for n in range(2):
                w = qkv_v[g % 2][t * 2 + n, pl.ds(j, 128, stride=NJ), :]
                wt = w.T
                for h in range(4):
                    t_v[u * 3 + t, pl.ds((n * 4 + h) * HP, DH), :] = wt[h * DH:(h + 1) * DH]
            for d in range(DH):
                w = t_v[u * 3 + t, pl.ds(d, 8, stride=HP), :]
                r = pl.ds(d * 8, 8)
                if t == 0:
                    dst[0, j, r, :], dst[1, j, r, :] = _unpack(w)
                else:
                    dst[0, NJ + j, r, :], dst[1, NJ + j, r, :] = _unpack(w)
                    dst[0, j, r, :], dst[1, j, r, :] = _unpack(pltpu.roll(w, 1, 1))
            yield

    def att_core(dst, base, j, u):
        qws, ch = CFG[u]
        lane0 = lax.broadcasted_iota(jnp.int32, (8, 128), 1) == 0
        probs = []
        for p in range(2):
            acc = [None] * W
            qw = qws[p]
            for w0 in range(0, W, qw):
                for d in range(DH):
                    r = pl.ds(d * 8, 8)
                    q = q_s[p, j, r, :]
                    if d == 0 and dep[0] is not None:
                        q = jnp.where(j < 0, dep[0], q)
                    for w in range(w0, w0 + qw):
                        t = q * k_s[p, j + (NJ - w), r, :]
                        acc[w] = t if d == 0 else acc[w] + t
                dep[0] = acc[w0]
            lg = [acc[0] * DH ** -0.5]
            for w in range(1, W):
                lg.append(jnp.where(jnp.logical_and(lane0, j < w), -1e9, acc[w] * DH ** -0.5))
            m = lg[0]
            for w in range(1, W):
                m = jnp.maximum(m, lg[w])
            e = [jnp.exp(l - m) for l in lg]
            den = e[0]
            for w in range(1, W):
                den = den + e[w]
            inv = 1.0 / den
            probs.append([x * inv for x in e])
            dep[0] = inv
            yield
        for d in range(DH):
            r = pl.ds(d * 8, 8)
            o = []
            for p in range(2):
                acc = probs[p][0] * v_s[p, j + NJ, r, :]
                for w in range(1, W):
                    acc = acc + probs[p][w] * v_s[p, j + (NJ - w), r, :]
                o.append(acc)
                if d % ch == ch - 1:
                    probs[p][0] = jnp.where(j < 0, acc, probs[p][0])
                    dep[0] = acc
            ot_v[u, pl.ds(d, 8, stride=HP), :] = pltpu.pack_elementwise(o, packed_dtype=BF16)
        for n in range(2):
            ot = jnp.concatenate([ot_v[u, pl.ds((n * 4 + h) * HP, DH), :] for h in range(4)], axis=0)
            dst[base + n, pl.ds(j, 128, stride=NJ), :] = ot.T
        yield

    def o_cols(ref, r):
        return jnp.concatenate([ref[n, r, :] for n in range(ref.shape[0])], axis=1)

    def ln1(i):
        for k in range(TM1 // LR):
            b = i * (TM1 // LR) + k
            h = _ln_mod(x_v[rows(b, LR), :].astype(F32), 1.0 + mod_row(1), mod_row(0))
            h_v[rows(b, LR // 2), :] = pltpu.bitcast(h.astype(BF16), U32)

    def ln2(blk, n):
        starts = [blk * (TM // LB) + half_ * (HM // LB) + n for half_ in range(2)]
        o = jnp.concatenate([o_cols(o3_v, rows(b, LB // 2)) for b in starts], axis=0)
        y = _dot(pltpu.bitcast(o, BF16), wo_v[pl.ds((HG - 1) * GW, GW), :])
        hs = []
        for k, b in enumerate(starts):
            r = rows(b, LB)
            x1 = x_v[r, :].astype(F32) + mod_row(2) * (x1_v[r, :] + y[k * LB:(k + 1) * LB])
            x2_v[blk % 2, rows(k * (HM // LB) + n, LB), :] = x1
            hs.append(_ln_mod(x1, 1.0 + mod_row(4), mod_row(3)))
        terms = _lhs_terms(hs[0][:, :HD], hs[0][:, HD:], hs[1][:, :HD], hs[1][:, HD:])
        for k, t in enumerate(terms):
            hs_v[k, rows(n, LB // 2), :] = t

    def prep_gate_up(step):
        n = HD // 16
        top, bot = rows(step, n), rows(8 + step, n)
        for k in range(F // PC):
            cs = pl.ds(k * PC, PC)
            s1, s3, s4, s6, s7 = _rhs_terms(wg_v[top, cs], wu_v[top, cs], wg_v[bot, cs], wu_v[bot, cs])
            wu_v[top, cs], wg_v[bot, cs] = s3, s4
            sg_v[0, top, cs], sg_v[1, top, cs], sg_v[2, top, cs] = s1, s6, s7
            dep[0] = lax.bitcast_convert_type(s7[:8], F32)

    def prep_down(step):
        n = HF // 8
        top, bot = rows(step, n), rows(4 + step, n)
        for k in range(HD // 128):
            lo, hi = pl.ds(k * 128, 128), pl.ds(HD + k * 128, 128)
            s1, s3, s4, s6, s7 = _rhs_terms(wd_v[top, lo], wd_v[top, hi], wd_v[bot, lo], wd_v[bot, hi])
            wd_v[top, hi], wd_v[bot, lo] = s3, s4
            sd_v[0, top, lo], sd_v[1, top, lo], sd_v[2, top, lo] = s1, s6, s7
            dep[0] = lax.bitcast_convert_type(s7[:8], F32)

    def prefetch(g):
        nxt = [qkv_cp(g + 1, t) for t in range(3)] if g + 1 < HG else []
        for cp in nxt + [mod_cp(g + 2)] + [w_cps[k] for k in ((), (3,), (2,), (0,))[g]]:
            cp.start()

    x_cp(0).wait()
    ln1(0)
    for t in range(3):
        qkv_cp(0, t).wait()

    def first_body(i, carry):
        @pl.when(i + 1 < nb1)
        def _():
            x_cp(i + 1).wait()

        @pl.when(i == PF0)
        def _():
            prefetch(0)
        _mix(proj(0, i))
        ln1(jnp.minimum(i + 1, nb1 - 1))
        return carry
    lax.fori_loop(0, nb1, first_body, 0)

    half = nb1 // 2
    jpb = NJ // half

    def loads(g, j0, nj):
        for u in range(nj):
            yield from att_load(g, j0 + u, u)
            if g + 1 < HG:
                yield from mod_vpu(g + 2, j0 + u)

    def cores(g, i):
        dst, base = (o_v, g * 2) if g + 1 < HG else (o3_v, 0)
        for u in range(jpb):
            yield from att_core(dst, base, i * jpb + u, u)

    def wo_part(i, tie=False):
        for n in range(D // GW):
            cs = pl.ds(n * GW, GW)
            o = o_cols(o_v, rows(i, TM1 // 2))
            if tie and n == D // GW - 1:
                o = tied(o, i, TIW)
            x1_v[rows(i, TM1), cs] = _dot(pltpu.bitcast(o, BF16), wo_v[pl.ds(0, (HG - 1) * GW), cs])
            yield

    def overlapped(g, matmul, steps, na, prep):
        nj = NJ // na

        def body_a(i, c):
            if prep is not None:
                prep(i)
            _mix(matmul(i, prep is not None), steps, loads(g, i * nj, nj), (4 if g + 1 < HG else 3) * nj)
            return c
        lax.fori_loop(0, na, body_a, 0)
        if g == 0:
            w_cps[1].start()

        def body_b(i, carry):
            dep[0] = None
            _mix(cores(g, i))
            _mix(matmul(na + i, True))
            return carry
        lax.fori_loop(0, half, body_b, 0)

    for g in range(1, HG):
        for t in range(3):
            qkv_cp(g, t).wait()
        mod_cp(g + 1).wait()
        prefetch(g)
        for k in ((), (), (3,), (1, 2))[g]:
            w_cps[k].wait()
        overlapped(g - 1, lambda i, tie=False, g=g: proj(g, i, tie), 3, half,
                   (None, None, prep_down, prep_gate_up)[g])

    mod_cp(5).wait()
    w_cps[0].wait()
    nd = HD // DC
    nln = HM // LB
    nlate = TM // TM1
    overlapped(HG - 1, wo_part, D // GW, half - nlate, lambda i: prep_gate_up(half + i))

    def late_body(i, c):
        for k in range(nln // nlate):
            ln2(0, i * (nln // nlate) + k)
        prep_gate_up(nb1 - nlate + i)
        _mix(wo_part(nb1 - nlate + i))
        for k in range(NJ // nlate):
            _mix(mod_vpu(5, i * (NJ // nlate) + k))
        return c
    lax.fori_loop(0, nlate, late_body, 0)

    nb = S // TM

    def ffn_body(i, c):
        def gu(f, c2):
            act = []
            for half_ in range(2):
                cs = rows(half_ * (HF // FC) + f, FC)
                top, bot = pl.ds(0, HD // 2), pl.ds(HD // 2, HD // 2)
                rhs = (sg_v[0, :, cs], wg_v[top, cs], wu_v[top, cs], wg_v[bot, cs], wu_v[bot, cs],
                       sg_v[1, :, cs], sg_v[2, :, cs])
                g_top, u_top, g_bot, u_bot = _strassen([hs_v[k] for k in range(7)], rhs)
                act.append((g_top * jax.nn.sigmoid(g_top) * u_top, g_bot * jax.nn.sigmoid(g_bot) * u_bot))
            for k, t in enumerate(_lhs_terms(act[0][0], act[1][0], act[0][1], act[1][1])):
                as_v[k, :, rows(f, FC)] = t
            return c2
        lax.fori_loop(0, HF // FC, gu, 0)

        @pl.when(i >= 1)
        def _():
            for n in range(2 * nd):
                out_cp(i - 1, n).wait()

        def dn(n, with_ln):
            if with_ln:
                for k in range(nln // nd):
                    ln2(i + 1, n * (nln // nd) + k)
            lo, hi = rows(n, DC), rows(nd + n, DC)
            top, bot = pl.ds(0, HF // 2), pl.ds(HF // 2, HF // 2)
            rhs = (sd_v[0, :, lo], wd_v[top, lo], wd_v[top, hi], wd_v[bot, lo], wd_v[bot, hi],
                   sd_v[1, :, lo], sd_v[2, :, lo])
            c11, c12, c21, c22 = _strassen([as_v[k] for k in range(7)], rhs)
            for m, cs, y_top, y_bot in ((n, lo, c11, c21), (nd + n, hi, c12, c22)):
                gate = mod_v[5, pl.ds(0, 1), cs]
                for r, y in ((pl.ds(0, HM), y_top), (pl.ds(HM, HM), y_bot)):
                    ob_v[m, r, :] = (x2_v[i % 2, r, cs] + gate * y).astype(BF16)
            out_cp(i, n).start()
            out_cp(i, nd + n).start()

        @pl.when(i < nb - 1)
        def _():
            lax.fori_loop(0, nd, lambda n, c2: dn(n, True), None)

        @pl.when(i == nb - 1)
        def _():
            lax.fori_loop(0, nd, lambda n, c2: dn(n, False), None)
        return c
    lax.fori_loop(0, nb, ffn_body, 0)
    for n in range(2 * nd):
        out_cp(nb - 1, n).wait()


@jax.jit
def pallas_adaLN_cond__sliding_local_dilated__swiglu_ffn__prompt_kernel(
    A_x: jax.Array,
    A_wqkv: jax.Array,
    A_wo: jax.Array,
    B_x: jax.Array,
    B_w_gate: jax.Array,
    B_w_up: jax.Array,
    B_w_down: jax.Array,
    c: jax.Array,
    w_mod: jax.Array,
):
    del B_x
    hbm = pl.BlockSpec(memory_space=pl.ANY)
    dma = pltpu.SemaphoreType.DMA
    out = pl.pallas_call(
        _kernel,
        out_shape=jax.ShapeDtypeStruct((S, D), BF16),
        in_specs=[hbm] * 6 + [pl.BlockSpec(memory_space=pltpu.VMEM), hbm],
        out_specs=hbm,
        scratch_shapes=[
            pltpu.VMEM((S, D), BF16),
            pltpu.VMEM((HG, D, 3 * GW), BF16),
            pltpu.VMEM((D, D), BF16),
            pltpu.VMEM((D // 2, F), U32),
            pltpu.VMEM((D // 2, F), U32),
            pltpu.VMEM((F // 2, D), U32),
            pltpu.VMEM((6, D, D), BF16),
            pltpu.VMEM((S // 2, D), U32),
            pltpu.VMEM((6, S // 2, 128), U32),
            pltpu.VMEM((6, S // 2, 128), U32),
            pltpu.VMEM((12, 8 * HP, 128), U32),
            pltpu.VMEM((2, NJ, GW, 128), F32),
            pltpu.VMEM((2, 2 * NJ, GW, 128), F32),
            pltpu.VMEM((2, 2 * NJ, GW, 128), F32),
            pltpu.VMEM((2, 8 * HP, 128), U32),
            pltpu.VMEM((2 * HG - 2, S // 2, 128), U32),
            pltpu.VMEM((2, S // 2, 128), U32),
            pltpu.VMEM((S, D), F32),
            pltpu.VMEM((2, TM, D), F32),
            pltpu.VMEM((7, HM // 2, HD), U32),
            pltpu.VMEM((7, HM // 2, HF), U32),
            pltpu.VMEM((3, HD // 2, F), U32),
            pltpu.VMEM((3, HF // 2, HD), U32),
            pltpu.VMEM((D // DC, TM, DC), BF16),
            pltpu.VMEM((D, 128), F32),
            pltpu.VMEM((6, 8, D), F32),
            dma((S // TM1,)), dma((HG * 3,)), dma((6,)), dma((2 * D // MC,)), dma((4,)), dma((D // DC,)),
        ],
        compiler_params=pltpu.CompilerParams(vmem_limit_bytes=120 * 1024 * 1024,
            flags={"XLA_TPU_EVENLY_DISTRIBUTE_CRITICAL_NODES": True}),
    )(A_x.reshape(S, D), A_wqkv, A_wo, B_w_gate, B_w_up, B_w_down, c, w_mod)
    return out.reshape(1, S, D)
```

```python
import jax
import jax.numpy as jnp
from jax import lax
from jax.experimental import pallas as pl
from jax.experimental.pallas import tpu as pltpu

S, D, F = 2048, 1024, 3584
DH, W = 32, 8
HG, GW = 4, 256
NJ = 8
TM1 = 256
TM = 512
FC = 256
DC = 128
HM, HD, HF = TM // 2, D // 2, F // 2
LB = 64
HP = 36
CFG = (((2, 4), 1), ((2, 4), 1))
MC = 512
STAGE = (4, 4, 6, 8, 99)
PF0 = 2
LR = 128
TIE, TIW = 512, 768
PC = 128
EPS = 1e-5
F32, BF16, U32 = jnp.float32, jnp.bfloat16, jnp.uint32


def _dot(a, b):
    return jnp.dot(a, b, preferred_element_type=F32)


def _ln_mod(x, scale1, shift):
    m = jnp.mean(x, axis=-1, keepdims=True)
    xc = x - m
    v = jnp.mean(xc * xc, axis=-1, keepdims=True)
    return xc * lax.rsqrt(v + EPS) * scale1 + shift


def _unpack(w):
    lo = lax.bitcast_convert_type(w << 16, F32)
    hi = lax.bitcast_convert_type(w & jnp.uint32(0xFFFF0000), F32)
    return lo, hi


def _ld(ref, r):
    return pltpu.bitcast(ref[r, :], BF16)


def _mix(a, na=1, b=(), nb=0):
    b = iter(b)
    done = 0
    for k, _ in enumerate(a):
        while done * na < (k + 1) * nb:
            next(b)
            done += 1
    for _ in b:
        pass


def _lhs_terms(a11, a12, a21, a22):
    terms = (a11 + a22, a21 + a22, a11, a22, a11 + a12, a21 - a11, a12 - a22)
    return [pltpu.bitcast(t.astype(BF16), U32) for t in terms]


def _rhs_terms(b11, b12, b21, b22):
    halves = [(b11 + b22, b12 - b22, b21 - b11, b11 + b12, b21 + b22)
              for b11, b12, b21, b22 in zip(*(_unpack(b) for b in (b11, b12, b21, b22)))]
    return [pltpu.pack_elementwise([lo, hi], packed_dtype=BF16) for lo, hi in zip(*halves)]


def _strassen(lhs, rhs):
    p1, p2, p3, p4, p5, p6, p7 = (_dot(pltpu.bitcast(a, BF16), pltpu.bitcast(b, BF16)) for a, b in zip(lhs, rhs))
    return p1 + p4 - p5 + p7, p3 + p5, p2 + p4, p1 - p2 + p3 + p6


def _bf16_bits(x):
    return lax.bitcast_convert_type(x.astype(BF16).astype(F32), U32)


def _kernel(x_hbm, wqkv_hbm, wo_hbm, wg_hbm, wu_hbm, wd_hbm, c_ref, wmod_hbm, out_hbm,
            x_v, wqkv_v, wo_v, wg_v, wu_v, wd_v, wmod_v, h_v, qkv0_v, qkv1_v, t_v, q_s, k_s, v_s,
            ot_v, o_v, o3_v, x1_v, x2_v, hs_v, as_v, sg_v, sd_v, ob_v, scol_v, mod_v, sem_x, sem_qkv, sem_mod, sem_head, sem_w, sem_o):
    nb1 = S // TM1
    qkv_v = (qkv0_v, qkv1_v)

    def x_cp(i):
        r = pl.ds(i * TM1, TM1)
        return pltpu.make_async_copy(x_hbm.at[r], x_v.at[r], sem_x.at[i])

    def qkv_cp(g, t):
        return pltpu.make_async_copy(wqkv_hbm.at[:, pl.ds(t * D + g * GW, GW)],
                                     wqkv_v.at[g, :, pl.ds(t * GW, GW)], sem_qkv.at[g * 3 + t])

    def mod_cp(i):
        return pltpu.make_async_copy(wmod_hbm.at[:, pl.ds(i * D, D)], wmod_v.at[i], sem_mod.at[i])

    def mod_head_cp(i):
        return pltpu.make_async_copy(wmod_hbm.at[:, pl.ds(i * MC, MC)],
                                     wmod_v.at[i * MC // D, :, pl.ds(i * MC % D, MC)], sem_head.at[i])

    w_cps = [pltpu.make_async_copy(s, d, sem_w.at[i]) for i, (s, d) in enumerate(
        ((wo_hbm, wo_v), (wg_hbm, wg_v.bitcast(BF16)), (wu_hbm, wu_v.bitcast(BF16)), (wd_hbm, wd_v.bitcast(BF16))))]

    def out_cp(i, n):
        cs = pl.ds(pl.multiple_of(n * DC, DC), DC)
        return pltpu.make_async_copy(ob_v.at[n], out_hbm.at[pl.ds(i * TM, TM), cs], sem_o.at[n])

    nm = 2 * D // MC
    head = [mod_head_cp(i) for i in range(nm)] + [x_cp(0)] + [qkv_cp(0, t) for t in range(3)]
    head += [x_cp(i) for i in range(1, nb1)]
    for cp in head[:STAGE[0]]:
        cp.start()

    cf = c_ref[...].astype(F32)
    sc = (cf * jax.nn.sigmoid(cf)).astype(BF16)
    scol_v[...] = jnp.broadcast_to(sc.astype(F32), (128, D)).T
    sc8 = jnp.broadcast_to(sc, (16, D))
    for i in range(nm):
        mod_head_cp(i).wait()
        for cp in head[STAGE[i]:STAGE[i + 1]]:
            cp.start()
        cs = pl.ds(i * MC % D, MC)
        mod_v[i * MC // D, :, cs] = _dot(sc8, wmod_v[i * MC // D, :, cs])[:8]

    def mod_vpu(i, n):
        cs = pl.ds(pl.multiple_of(n * 128, 128), 128)
        p = wmod_v[i, :, cs].astype(F32) * scol_v[...]
        mod_v[i, :, cs] = jnp.broadcast_to(jnp.sum(p, axis=0, keepdims=True), (8, 128))
        yield

    def mod_row(i):
        return mod_v[i, pl.ds(0, 1), :]

    dep = [None]

    def rows(i, n):
        return pl.ds(pl.multiple_of(i * n, n), n)

    def tied(h, i, n):
        k0 = h.shape[1] - n
        late = jnp.tile(lax.bitcast_convert_type(dep[0], U32), (h.shape[0] // 8, n // 128))
        late = jnp.where(i < 0, late, h[:, k0:])
        return jnp.concatenate([h[:, :k0], late], axis=1) if k0 else late

    def proj(g, i, tie=False):
        for t in range(3):
            h = h_v[rows(i, TM1 // 2), :]
            if tie and t == 2:
                h = tied(h, i, TIE)
            y = _dot(pltpu.bitcast(h, BF16), wqkv_v[g, :, pl.ds(t * GW, GW)])
            y = pltpu.bitcast(y.astype(BF16), U32)
            for n in range(2):
                qkv_v[g % 2][t * 2 + n, rows(i, TM1 // 2), :] = y[:, n * 128:(n + 1) * 128]
            yield

    def att_load(g, j, u):
        for t, dst in enumerate((q_s, k_s, v_s)):
            for n in range(2):
                w = qkv_v[g % 2][t * 2 + n, pl.ds(j, 128, stride=NJ), :]
                wt = w.T
                for h in range(4):
                    t_v[u * 3 + t, pl.ds((n * 4 + h) * HP, DH), :] = wt[h * DH:(h + 1) * DH]
            for d in range(DH):
                w = t_v[u * 3 + t, pl.ds(d, 8, stride=HP), :]
                r = pl.ds(d * 8, 8)
                if t == 0:
                    dst[0, j, r, :], dst[1, j, r, :] = _unpack(w)
                else:
                    dst[0, NJ + j, r, :], dst[1, NJ + j, r, :] = _unpack(w)
                    dst[0, j, r, :], dst[1, j, r, :] = _unpack(pltpu.roll(w, 1, 1))
            yield

    def att_core(dst, base, j, u):
        qws, ch = CFG[u]
        lane0 = lax.broadcasted_iota(jnp.int32, (8, 128), 1) == 0
        probs = []
        for p in range(2):
            acc = [None] * W
            qw = qws[p]
            for w0 in range(0, W, qw):
                for d in range(DH):
                    r = pl.ds(d * 8, 8)
                    q = q_s[p, j, r, :]
                    if d == 0 and dep[0] is not None:
                        q = jnp.where(j < 0, dep[0], q)
                    for w in range(w0, w0 + qw):
                        t = q * k_s[p, j + (NJ - w), r, :]
                        acc[w] = t if d == 0 else acc[w] + t
                dep[0] = acc[w0]
            lg = [acc[0] * DH ** -0.5]
            for w in range(1, W):
                lg.append(jnp.where(jnp.logical_and(lane0, j < w), -1e9, acc[w] * DH ** -0.5))
            m = lg[0]
            for w in range(1, W):
                m = jnp.maximum(m, lg[w])
            e = [jnp.exp(l - m) for l in lg]
            den = e[0]
            for w in range(1, W):
                den = den + e[w]
            inv = 1.0 / den
            probs.append([x * inv for x in e])
            dep[0] = inv
            yield
        for d in range(DH):
            r = pl.ds(d * 8, 8)
            o = []
            for p in range(2):
                acc = probs[p][0] * v_s[p, j + NJ, r, :]
                for w in range(1, W):
                    acc = acc + probs[p][w] * v_s[p, j + (NJ - w), r, :]
                o.append(acc)
                if d % ch == ch - 1:
                    probs[p][0] = jnp.where(j < 0, acc, probs[p][0])
                    dep[0] = acc
            ot_v[u, pl.ds(d, 8, stride=HP), :] = pltpu.pack_elementwise(o, packed_dtype=BF16)
        for n in range(2):
            ot = jnp.concatenate([ot_v[u, pl.ds((n * 4 + h) * HP, DH), :] for h in range(4)], axis=0)
            dst[base + n, pl.ds(j, 128, stride=NJ), :] = ot.T
        yield

    def o_cols(ref, r):
        return jnp.concatenate([ref[n, r, :] for n in range(ref.shape[0])], axis=1)

    def ln1(i):
        for k in range(TM1 // LR):
            b = i * (TM1 // LR) + k
            h = _ln_mod(x_v[rows(b, LR), :].astype(F32), 1.0 + mod_row(1), mod_row(0))
            h_v[rows(b, LR // 2), :] = pltpu.bitcast(h.astype(BF16), U32)

    def ln2(blk, n):
        starts = [blk * (TM // LB) + half_ * (HM // LB) + n for half_ in range(2)]
        o = jnp.concatenate([o_cols(o3_v, rows(b, LB // 2)) for b in starts], axis=0)
        y = _dot(pltpu.bitcast(o, BF16), wo_v[pl.ds((HG - 1) * GW, GW), :])
        hs = []
        for k, b in enumerate(starts):
            r = rows(b, LB)
            x1 = x_v[r, :].astype(F32) + mod_row(2) * (x1_v[r, :] + y[k * LB:(k + 1) * LB])
            x2_v[blk % 2, rows(k * (HM // LB) + n, LB), :] = x1
            hs.append(_ln_mod(x1, 1.0 + mod_row(4), mod_row(3)))
        terms = _lhs_terms(hs[0][:, :HD], hs[0][:, HD:], hs[1][:, :HD], hs[1][:, HD:])
        for k, t in enumerate(terms):
            hs_v[k, rows(n, LB // 2), :] = t

    def prep_gate_up(step):
        n = HD // 16
        top, bot = rows(step, n), rows(8 + step, n)
        for k in range(F // PC):
            cs = pl.ds(k * PC, PC)
            s1, s3, s4, s6, s7 = _rhs_terms(wg_v[top, cs], wu_v[top, cs], wg_v[bot, cs], wu_v[bot, cs])
            wu_v[top, cs], wg_v[bot, cs] = s3, s4
            sg_v[0, top, cs], sg_v[1, top, cs], sg_v[2, top, cs] = s1, s6, s7
            dep[0] = lax.bitcast_convert_type(s7[:8, :128], F32)

    def prep_down(step):
        n = HF // 64
        lo, hi = pl.ds(0, HD), pl.ds(HD, HD)
        for k in range(n):
            top, bot = rows(step * n + k, 8), rows((4 + step) * n + k, 8)
            s1, s3, s4, s6, s7 = _rhs_terms(wd_v[top, lo], wd_v[top, hi], wd_v[bot, lo], wd_v[bot, hi])
            wd_v[top, hi], wd_v[bot, lo] = s3, s4
            sd_v[0, top, lo], sd_v[1, top, lo], sd_v[2, top, lo] = s1, s6, s7
            dep[0] = lax.bitcast_convert_type(s7[:8, :128], F32)

    def prefetch(g):
        nxt = [qkv_cp(g + 1, t) for t in range(3)] if g + 1 < HG else []
        for cp in nxt + [mod_cp(g + 2)] + [w_cps[k] for k in ((), (3,), (2,), (0,))[g]]:
            cp.start()

    x_cp(0).wait()
    ln1(0)
    for t in range(3):
        qkv_cp(0, t).wait()

    def first_body(i, carry):
        @pl.when(i + 1 < nb1)
        def _():
            x_cp(i + 1).wait()

        @pl.when(i == PF0)
        def _():
            prefetch(0)
        _mix(proj(0, i))
        ln1(jnp.minimum(i + 1, nb1 - 1))
        return carry
    lax.fori_loop(0, nb1, first_body, 0)

    half = nb1 // 2
    jpb = NJ // half

    def loads(g, j0, nj):
        for u in range(nj):
            yield from att_load(g, j0 + u, u)
            if g + 1 < HG:
                yield from mod_vpu(g + 2, j0 + u)

    def cores(g, i):
        dst, base = (o_v, g * 2) if g + 1 < HG else (o3_v, 0)
        for u in range(jpb):
            yield from att_core(dst, base, i * jpb + u, u)

    def wo_part(i, tie=False):
        for n in range(D // GW):
            cs = pl.ds(n * GW, GW)
            o = o_cols(o_v, rows(i, TM1 // 2))
            if tie and n == D // GW - 1:
                o = tied(o, i, TIW)
            x1_v[rows(i, TM1), cs] = _dot(pltpu.bitcast(o, BF16), wo_v[pl.ds(0, (HG - 1) * GW), cs])
            yield

    def overlapped(g, matmul, steps, na, prep):
        nj = NJ // na

        def body_a(i, c):
            if prep is not None:
                prep(i)
            _mix(matmul(i, prep is not None), steps, loads(g, i * nj, nj), (4 if g + 1 < HG else 3) * nj)
            return c
        lax.fori_loop(0, na, body_a, 0)
        if g == 0:
            w_cps[1].start()

        def body_b(i, carry):
            dep[0] = None
            _mix(cores(g, i))
            _mix(matmul(na + i, True))
            return carry
        lax.fori_loop(0, half, body_b, 0)

    for g in range(1, HG):
        for t in range(3):
            qkv_cp(g, t).wait()
        mod_cp(g + 1).wait()
        prefetch(g)
        for k in ((), (), (3,), (1, 2))[g]:
            w_cps[k].wait()
        overlapped(g - 1, lambda i, tie=False, g=g: proj(g, i, tie), 3, half,
                   (None, None, prep_down, prep_gate_up)[g])

    mod_cp(5).wait()
    w_cps[0].wait()
    nd = HD // DC
    nln = HM // LB
    nlate = TM // TM1
    overlapped(HG - 1, wo_part, D // GW, half - nlate, lambda i: prep_gate_up(half + i))

    def late_body(i, c):
        for k in range(nln // nlate):
            ln2(0, i * (nln // nlate) + k)
        prep_gate_up(nb1 - nlate + i)
        _mix(wo_part(nb1 - nlate + i))
        for k in range(NJ // nlate):
            _mix(mod_vpu(5, i * (NJ // nlate) + k))
        return c
    lax.fori_loop(0, nlate, late_body, 0)

    nb = S // TM

    def ffn_body(i, c):
        def gu(f, c2):
            act = []
            for half_ in range(2):
                cs = rows(half_ * (HF // FC) + f, FC)
                top, bot = pl.ds(0, HD // 2), pl.ds(HD // 2, HD // 2)
                rhs = (sg_v[0, :, cs], wg_v[top, cs], wu_v[top, cs], wg_v[bot, cs], wu_v[bot, cs],
                       sg_v[1, :, cs], sg_v[2, :, cs])
                g_top, u_top, g_bot, u_bot = _strassen([hs_v[k] for k in range(7)], rhs)
                act.append((g_top * jax.nn.sigmoid(g_top) * u_top, g_bot * jax.nn.sigmoid(g_bot) * u_bot))
            for k, t in enumerate(_lhs_terms(act[0][0], act[1][0], act[0][1], act[1][1])):
                as_v[k, :, rows(f, FC)] = t
            return c2
        lax.fori_loop(0, HF // FC, gu, 0)

        @pl.when(i >= 1)
        def _():
            for n in range(2 * nd):
                out_cp(i - 1, n).wait()

        def dn(n, with_ln):
            if with_ln:
                for k in range(nln // nd):
                    ln2(i + 1, n * (nln // nd) + k)
            lo, hi = rows(n, DC), rows(nd + n, DC)
            top, bot = pl.ds(0, HF // 2), pl.ds(HF // 2, HF // 2)
            rhs = (sd_v[0, :, lo], wd_v[top, lo], wd_v[top, hi], wd_v[bot, lo], wd_v[bot, hi],
                   sd_v[1, :, lo], sd_v[2, :, lo])
            c11, c12, c21, c22 = _strassen([as_v[k] for k in range(7)], rhs)
            for m, cs, y_top, y_bot in ((n, lo, c11, c21), (nd + n, hi, c12, c22)):
                gate = mod_v[5, pl.ds(0, 1), cs]
                for r, y in ((pl.ds(0, HM), y_top), (pl.ds(HM, HM), y_bot)):
                    ob_v[m, r, :] = (x2_v[i % 2, r, cs] + gate * y).astype(BF16)
            out_cp(i, n).start()
            out_cp(i, nd + n).start()

        @pl.when(i < nb - 1)
        def _():
            lax.fori_loop(0, nd, lambda n, c2: dn(n, True), None)

        @pl.when(i == nb - 1)
        def _():
            lax.fori_loop(0, nd, lambda n, c2: dn(n, False), None)
        return c
    lax.fori_loop(0, nb, ffn_body, 0)
    for n in range(2 * nd):
        out_cp(nb - 1, n).wait()


@jax.jit
def pallas_adaLN_cond__sliding_local_dilated__swiglu_ffn__prompt_kernel(
    A_x: jax.Array,
    A_wqkv: jax.Array,
    A_wo: jax.Array,
    B_x: jax.Array,
    B_w_gate: jax.Array,
    B_w_up: jax.Array,
    B_w_down: jax.Array,
    c: jax.Array,
    w_mod: jax.Array,
):
    del B_x
    hbm = pl.BlockSpec(memory_space=pl.ANY)
    dma = pltpu.SemaphoreType.DMA
    out = pl.pallas_call(
        _kernel,
        out_shape=jax.ShapeDtypeStruct((S, D), BF16),
        in_specs=[hbm] * 6 + [pl.BlockSpec(memory_space=pltpu.VMEM), hbm],
        out_specs=hbm,
        scratch_shapes=[
            pltpu.VMEM((S, D), BF16),
            pltpu.VMEM((HG, D, 3 * GW), BF16),
            pltpu.VMEM((D, D), BF16),
            pltpu.VMEM((D // 2, F), U32),
            pltpu.VMEM((D // 2, F), U32),
            pltpu.VMEM((F // 2, D), U32),
            pltpu.VMEM((6, D, D), BF16),
            pltpu.VMEM((S // 2, D), U32),
            pltpu.VMEM((6, S // 2, 128), U32),
            pltpu.VMEM((6, S // 2, 128), U32),
            pltpu.VMEM((12, 8 * HP, 128), U32),
            pltpu.VMEM((2, NJ, GW, 128), F32),
            pltpu.VMEM((2, 2 * NJ, GW, 128), F32),
            pltpu.VMEM((2, 2 * NJ, GW, 128), F32),
            pltpu.VMEM((2, 8 * HP, 128), U32),
            pltpu.VMEM((2 * HG - 2, S // 2, 128), U32),
            pltpu.VMEM((2, S // 2, 128), U32),
            pltpu.VMEM((S, D), F32),
            pltpu.VMEM((2, TM, D), F32),
            pltpu.VMEM((7, HM // 2, HD), U32),
            pltpu.VMEM((7, HM // 2, HF), U32),
            pltpu.VMEM((3, HD // 2, F), U32),
            pltpu.VMEM((3, HF // 2, HD), U32),
            pltpu.VMEM((D // DC, TM, DC), BF16),
            pltpu.VMEM((D, 128), F32),
            pltpu.VMEM((6, 8, D), F32),
            dma((S // TM1,)), dma((HG * 3,)), dma((6,)), dma((2 * D // MC,)), dma((4,)), dma((D // DC,)),
        ],
        compiler_params=pltpu.CompilerParams(vmem_limit_bytes=120 * 1024 * 1024,
            flags={"XLA_TPU_EVENLY_DISTRIBUTE_CRITICAL_NODES": True}),
    )(A_x.reshape(S, D), A_wqkv, A_wo, B_w_gate, B_w_up, B_w_down, c, w_mod)
    return out.reshape(1, S, D)
```

```python
import jax
import jax.numpy as jnp
from jax import lax
from jax.experimental import pallas as pl
from jax.experimental.pallas import tpu as pltpu

S, D, F = 2048, 1024, 3584
DH, W = 32, 8
HG, GW = 4, 256
NJ = 8
TM1 = 256
TM = 512
FC = 256
DC = 128
HM, HD, HF = TM // 2, D // 2, F // 2
LB = 64
HP = 36
CFG = (((2, 4), 1), ((2, 4), 1))
MC = 512
STAGE = (4, 4, 6, 8, 99)
PF0 = 2
LR = 128
TIE, TIW = 512, 768
PC = 128
EPS = 1e-5
F32, BF16, U32 = jnp.float32, jnp.bfloat16, jnp.uint32


def _dot(a, b):
    return jnp.dot(a, b, preferred_element_type=F32)


def _ln_mod(x, scale1, shift):
    m = jnp.mean(x, axis=-1, keepdims=True)
    xc = x - m
    v = jnp.mean(xc * xc, axis=-1, keepdims=True)
    return xc * lax.rsqrt(v + EPS) * scale1 + shift


def _unpack(w):
    lo = lax.bitcast_convert_type(w << 16, F32)
    hi = lax.bitcast_convert_type(w & jnp.uint32(0xFFFF0000), F32)
    return lo, hi


def _ld(ref, r):
    return pltpu.bitcast(ref[r, :], BF16)


def _mix(a, na=1, b=(), nb=0):
    b = iter(b)
    done = 0
    for k, _ in enumerate(a):
        while done * na < (k + 1) * nb:
            next(b)
            done += 1
    for _ in b:
        pass


def _lhs_terms(a11, a12, a21, a22):
    terms = (a11 + a22, a21 + a22, a11, a22, a11 + a12, a21 - a11, a12 - a22)
    return [pltpu.bitcast(t.astype(BF16), U32) for t in terms]


def _rhs_terms(b11, b12, b21, b22):
    halves = [(b11 + b22, b12 - b22, b21 - b11, b11 + b12, b21 + b22)
              for b11, b12, b21, b22 in zip(*(_unpack(b) for b in (b11, b12, b21, b22)))]
    return [pltpu.pack_elementwise([lo, hi], packed_dtype=BF16) for lo, hi in zip(*halves)]


def _strassen(lhs, rhs):
    p1, p2, p3, p4, p5, p6, p7 = (_dot(pltpu.bitcast(a, BF16), pltpu.bitcast(b, BF16)) for a, b in zip(lhs, rhs))
    return p1 + p4 - p5 + p7, p3 + p5, p2 + p4, p1 - p2 + p3 + p6


def _bf16_bits(x):
    return lax.bitcast_convert_type(x.astype(BF16).astype(F32), U32)


def _kernel(x_hbm, wqkv_hbm, wo_hbm, wg_hbm, wu_hbm, wd_hbm, c_ref, wmod_hbm, out_hbm,
            x_v, wqkv_v, wo_v, wg_v, wu_v, wd_v, wmod_v, h_v, qkv0_v, qkv1_v, t_v, q_s, k_s, v_s,
            ot_v, o_v, o3_v, x1_v, x2_v, hs_v, as_v, sg_v, sd_v, ob_v, scol_v, mod_v, sem_x, sem_qkv, sem_mod, sem_head, sem_w, sem_o):
    nb1 = S // TM1
    qkv_v = (qkv0_v, qkv1_v)

    def x_cp(i):
        r = pl.ds(i * TM1, TM1)
        return pltpu.make_async_copy(x_hbm.at[r], x_v.at[r], sem_x.at[i])

    def qkv_cp(g, t):
        return pltpu.make_async_copy(wqkv_hbm.at[:, pl.ds(t * D + g * GW, GW)],
                                     wqkv_v.at[g].bitcast(BF16).at[:, pl.ds(t * GW, GW)], sem_qkv.at[g * 3 + t])

    def mod_cp(i):
        return pltpu.make_async_copy(wmod_hbm.at[:, pl.ds(i * D, D)], wmod_v.at[i], sem_mod.at[i])

    def mod_head_cp(i):
        return pltpu.make_async_copy(wmod_hbm.at[:, pl.ds(i * MC, MC)],
                                     wmod_v.at[i * MC // D, :, pl.ds(i * MC % D, MC)], sem_head.at[i])

    w_cps = [pltpu.make_async_copy(s, d, sem_w.at[i]) for i, (s, d) in enumerate(
        ((wo_hbm, wo_v.bitcast(BF16)), (wg_hbm, wg_v.bitcast(BF16)), (wu_hbm, wu_v.bitcast(BF16)), (wd_hbm, wd_v.bitcast(BF16))))]

    def out_cp(i, n):
        cs = pl.ds(pl.multiple_of(n * DC, DC), DC)
        return pltpu.make_async_copy(ob_v.at[n], out_hbm.at[pl.ds(i * TM, TM), cs], sem_o.at[n])

    nm = 2 * D // MC
    head = [mod_head_cp(i) for i in range(nm)] + [x_cp(0)] + [qkv_cp(0, t) for t in range(3)]
    head += [x_cp(i) for i in range(1, nb1)]
    for cp in head[:STAGE[0]]:
        cp.start()

    cf = c_ref[...].astype(F32)
    sc = (cf * jax.nn.sigmoid(cf)).astype(BF16)
    scol_v[...] = jnp.broadcast_to(sc.astype(F32), (128, D)).T
    sc8 = jnp.broadcast_to(sc, (16, D))
    for i in range(nm):
        mod_head_cp(i).wait()
        for cp in head[STAGE[i]:STAGE[i + 1]]:
            cp.start()
        cs = pl.ds(i * MC % D, MC)
        mod_v[i * MC // D, :, cs] = _dot(sc8, wmod_v[i * MC // D, :, cs])[:8]

    def mod_vpu(i, n):
        cs = pl.ds(pl.multiple_of(n * 128, 128), 128)
        p = wmod_v[i, :, cs].astype(F32) * scol_v[...]
        mod_v[i, :, cs] = jnp.broadcast_to(jnp.sum(p, axis=0, keepdims=True), (8, 128))
        yield

    def mod_row(i):
        return mod_v[i, pl.ds(0, 1), :]

    dep = [None]

    def rows(i, n):
        return pl.ds(pl.multiple_of(i * n, n), n)

    def tied(h, i, n):
        k0 = h.shape[1] - n
        late = jnp.tile(lax.bitcast_convert_type(dep[0], U32), (h.shape[0] // 8, n // 128))
        late = jnp.where(i < 0, late, h[:, k0:])
        return jnp.concatenate([h[:, :k0], late], axis=1) if k0 else late

    def proj(g, i, tie=False):
        for t in range(3):
            h = h_v[rows(i, TM1 // 2), :]
            if tie and t == 2:
                h = tied(h, i, TIE)
            y = _dot(pltpu.bitcast(h, BF16), pltpu.bitcast(wqkv_v[g, :, pl.ds(t * GW, GW)], BF16))
            y = pltpu.bitcast(y.astype(BF16), U32)
            for n in range(2):
                qkv_v[g % 2][t * 2 + n, rows(i, TM1 // 2), :] = y[:, n * 128:(n + 1) * 128]
            yield

    def att_load(g, j, u):
        for t, dst in enumerate((q_s, k_s, v_s)):
            for n in range(2):
                w = qkv_v[g % 2][t * 2 + n, pl.ds(j, 128, stride=NJ), :]
                wt = w.T
                for h in range(4):
                    t_v[u * 3 + t, pl.ds((n * 4 + h) * HP, DH), :] = wt[h * DH:(h + 1) * DH]
            for d in range(DH):
                w = t_v[u * 3 + t, pl.ds(d, 8, stride=HP), :]
                r = pl.ds(d * 8, 8)
                if t == 0:
                    dst[0, j, r, :], dst[1, j, r, :] = _unpack(w)
                else:
                    dst[0, NJ + j, r, :], dst[1, NJ + j, r, :] = _unpack(w)
                    dst[0, j, r, :], dst[1, j, r, :] = _unpack(pltpu.roll(w, 1, 1))
            yield

    def att_core(dst, base, j, u):
        qws, ch = CFG[u]
        lane0 = lax.broadcasted_iota(jnp.int32, (8, 128), 1) == 0
        probs = []
        for p in range(2):
            acc = [None] * W
            qw = qws[p]
            for w0 in range(0, W, qw):
                for d in range(DH):
                    r = pl.ds(d * 8, 8)
                    q = q_s[p, j, r, :]
                    if d == 0 and dep[0] is not None:
                        q = jnp.where(j < 0, dep[0], q)
                    for w in range(w0, w0 + qw):
                        t = q * k_s[p, j + (NJ - w), r, :]
                        acc[w] = t if d == 0 else acc[w] + t
                dep[0] = acc[w0]
            lg = [acc[0] * DH ** -0.5]
            for w in range(1, W):
                lg.append(jnp.where(jnp.logical_and(lane0, j < w), -1e9, acc[w] * DH ** -0.5))
            m = lg[0]
            for w in range(1, W):
                m = jnp.maximum(m, lg[w])
            e = [jnp.exp(l - m) for l in lg]
            den = e[0]
            for w in range(1, W):
                den = den + e[w]
            inv = 1.0 / den
            probs.append([x * inv for x in e])
            dep[0] = inv
            yield
        for d in range(DH):
            r = pl.ds(d * 8, 8)
            o = []
            for p in range(2):
                acc = probs[p][0] * v_s[p, j + NJ, r, :]
                for w in range(1, W):
                    acc = acc + probs[p][w] * v_s[p, j + (NJ - w), r, :]
                o.append(acc)
                if d % ch == ch - 1:
                    probs[p][0] = jnp.where(j < 0, acc, probs[p][0])
                    dep[0] = acc
            ot_v[u, pl.ds(d, 8, stride=HP), :] = pltpu.pack_elementwise(o, packed_dtype=BF16)
        for n in range(2):
            ot = jnp.concatenate([ot_v[u, pl.ds((n * 4 + h) * HP, DH), :] for h in range(4)], axis=0)
            dst[base + n, pl.ds(j, 128, stride=NJ), :] = ot.T
        yield

    def o_cols(ref, r):
        return jnp.concatenate([ref[n, r, :] for n in range(ref.shape[0])], axis=1)

    def ln1(i):
        for k in range(TM1 // LR):
            b = i * (TM1 // LR) + k
            h = _ln_mod(x_v[rows(b, LR), :].astype(F32), 1.0 + mod_row(1), mod_row(0))
            h_v[rows(b, LR // 2), :] = pltpu.bitcast(h.astype(BF16), U32)

    def ln2(blk, n):
        starts = [blk * (TM // LB) + half_ * (HM // LB) + n for half_ in range(2)]
        o = jnp.concatenate([o_cols(o3_v, rows(b, LB // 2)) for b in starts], axis=0)
        y = _dot(pltpu.bitcast(o, BF16), _ld(wo_v, pl.ds((HG - 1) * GW // 2, GW // 2)))
        hs = []
        for k, b in enumerate(starts):
            r = rows(b, LB)
            x1 = x_v[r, :].astype(F32) + mod_row(2) * (x1_v[r, :] + y[k * LB:(k + 1) * LB])
            x2_v[blk % 2, rows(k * (HM // LB) + n, LB), :] = x1
            hs.append(_ln_mod(x1, 1.0 + mod_row(4), mod_row(3)))
        terms = _lhs_terms(hs[0][:, :HD], hs[0][:, HD:], hs[1][:, :HD], hs[1][:, HD:])
        for k, t in enumerate(terms):
            hs_v[k, rows(n, LB // 2), :] = t

    def prep_gate_up(step):
        n = HD // 16
        top, bot = rows(step, n), rows(8 + step, n)
        for k in range(F // PC):
            cs = pl.ds(k * PC, PC)
            s1, s3, s4, s6, s7 = _rhs_terms(wg_v[top, cs], wu_v[top, cs], wg_v[bot, cs], wu_v[bot, cs])
            wu_v[top, cs], wg_v[bot, cs] = s3, s4
            sg_v[0, top, cs], sg_v[1, top, cs], sg_v[2, top, cs] = s1, s6, s7
            dep[0] = lax.bitcast_convert_type(s7[:8, :128], F32)

    def prep_down(step):
        steps = HF // FC
        n = HF // 16 // steps
        lo, hi = pl.ds(0, HD), pl.ds(HD, HD)
        for k in range(n):
            top, bot = rows(step * n + k, 8), rows((steps + step) * n + k, 8)
            s1, s3, s4, s6, s7 = _rhs_terms(wd_v[top, lo], wd_v[top, hi], wd_v[bot, lo], wd_v[bot, hi])
            wd_v[top, hi], wd_v[bot, lo] = s3, s4
            sd_v[0, top, lo], sd_v[1, top, lo], sd_v[2, top, lo] = s1, s6, s7

    def prefetch(g):
        nxt = [qkv_cp(g + 1, t) for t in range(3)] if g + 1 < HG else []
        for cp in nxt + [mod_cp(g + 2)] + [w_cps[k] for k in ((), (1,), (), (0,))[g]]:
            cp.start()

    x_cp(0).wait()
    ln1(0)
    for t in range(3):
        qkv_cp(0, t).wait()

    def first_body(i, carry):
        @pl.when(i + 1 < nb1)
        def _():
            x_cp(i + 1).wait()

        @pl.when(i == PF0)
        def _():
            prefetch(0)
        _mix(proj(0, i))
        ln1(jnp.minimum(i + 1, nb1 - 1))
        return carry
    lax.fori_loop(0, nb1, first_body, 0)

    half = nb1 // 2
    jpb = NJ // half

    def loads(g, j0, nj):
        for u in range(nj):
            yield from att_load(g, j0 + u, u)
            if g + 1 < HG:
                yield from mod_vpu(g + 2, j0 + u)

    def cores(g, i):
        dst, base = (o_v, g * 2) if g + 1 < HG else (o3_v, 0)
        for u in range(jpb):
            yield from att_core(dst, base, i * jpb + u, u)

    def wo_part(i, tie=False):
        for n in range(D // GW):
            cs = pl.ds(n * GW, GW)
            o = o_cols(o_v, rows(i, TM1 // 2))
            if tie and n == D // GW - 1:
                o = tied(o, i, TIW)
            x1_v[rows(i, TM1), cs] = _dot(pltpu.bitcast(o, BF16), pltpu.bitcast(wo_v[pl.ds(0, (HG - 1) * GW // 2), cs], BF16))
            yield

    def overlapped(g, matmul, steps, na, prep):
        nj = NJ // na

        def body_a(i, c):
            if prep is not None:
                prep(i)
            _mix(matmul(i), steps, loads(g, i * nj, nj), (4 if g + 1 < HG else 3) * nj)
            return c
        lax.fori_loop(0, na, body_a, 0)
        if g < 2:
            w_cps[g + 2].start()

        def body_b(i, carry):
            dep[0] = None
            _mix(cores(g, i))
            _mix(matmul(na + i, True))
            return carry
        lax.fori_loop(0, half, body_b, 0)

    for g in range(1, HG):
        for t in range(3):
            qkv_cp(g, t).wait()
        mod_cp(g + 1).wait()
        prefetch(g)
        for k in ((), (), (), (1, 2))[g]:
            w_cps[k].wait()
        overlapped(g - 1, lambda i, tie=False, g=g: proj(g, i, tie), 3, half,
                   (None, None, None, prep_gate_up)[g])

    mod_cp(5).wait()
    w_cps[0].wait()
    nd = HD // DC
    nln = HM // LB
    nlate = TM // TM1
    overlapped(HG - 1, wo_part, D // GW, half - nlate, lambda i: prep_gate_up(half + i))

    def late_body(i, c):
        for k in range(nln // nlate):
            ln2(0, i * (nln // nlate) + k)
        prep_gate_up(nb1 - nlate + i)
        _mix(wo_part(nb1 - nlate + i))
        for k in range(NJ // nlate):
            _mix(mod_vpu(5, i * (NJ // nlate) + k))
        return c
    lax.fori_loop(0, nlate, late_body, 0)

    nb = S // TM
    w_cps[3].wait()

    def ffn_body(i, c):
        def gu(f, with_prep):
            if with_prep:
                prep_down(f)
            act = []
            for half_ in range(2):
                cs = rows(half_ * (HF // FC) + f, FC)
                top, bot = pl.ds(0, HD // 2), pl.ds(HD // 2, HD // 2)
                rhs = (sg_v[0, :, cs], wg_v[top, cs], wu_v[top, cs], wg_v[bot, cs], wu_v[bot, cs],
                       sg_v[1, :, cs], sg_v[2, :, cs])
                g_top, u_top, g_bot, u_bot = _strassen([hs_v[k] for k in range(7)], rhs)
                act.append((g_top * jax.nn.sigmoid(g_top) * u_top, g_bot * jax.nn.sigmoid(g_bot) * u_bot))
            for k, t in enumerate(_lhs_terms(act[0][0], act[1][0], act[0][1], act[1][1])):
                as_v[k, :, rows(f, FC)] = t

        @pl.when(i == 0)
        def _():
            lax.fori_loop(0, HF // FC, lambda f, c2: gu(f, True), None)

        @pl.when(i > 0)
        def _():
            lax.fori_loop(0, HF // FC, lambda f, c2: gu(f, False), None)

        @pl.when(i >= 1)
        def _():
            for n in range(2 * nd):
                out_cp(i - 1, n).wait()

        def dn(n, with_ln):
            if with_ln:
                for k in range(nln // nd):
                    ln2(i + 1, n * (nln // nd) + k)
            lo, hi = rows(n, DC), rows(nd + n, DC)
            top, bot = pl.ds(0, HF // 2), pl.ds(HF // 2, HF // 2)
            rhs = (sd_v[0, :, lo], wd_v[top, lo], wd_v[top, hi], wd_v[bot, lo], wd_v[bot, hi],
                   sd_v[1, :, lo], sd_v[2, :, lo])
            c11, c12, c21, c22 = _strassen([as_v[k] for k in range(7)], rhs)
            for m, cs, y_top, y_bot in ((n, lo, c11, c21), (nd + n, hi, c12, c22)):
                gate = mod_v[5, pl.ds(0, 1), cs]
                for r, y in ((pl.ds(0, HM), y_top), (pl.ds(HM, HM), y_bot)):
                    ob_v[m, r, :] = (x2_v[i % 2, r, cs] + gate * y).astype(BF16)
            out_cp(i, n).start()
            out_cp(i, nd + n).start()

        @pl.when(i < nb - 1)
        def _():
            lax.fori_loop(0, nd, lambda n, c2: dn(n, True), None)

        @pl.when(i == nb - 1)
        def _():
            lax.fori_loop(0, nd, lambda n, c2: dn(n, False), None)
        return c
    lax.fori_loop(0, nb, ffn_body, 0)
    for n in range(2 * nd):
        out_cp(nb - 1, n).wait()


@jax.jit
def pallas_adaLN_cond__sliding_local_dilated__swiglu_ffn__prompt_kernel(
    A_x: jax.Array,
    A_wqkv: jax.Array,
    A_wo: jax.Array,
    B_x: jax.Array,
    B_w_gate: jax.Array,
    B_w_up: jax.Array,
    B_w_down: jax.Array,
    c: jax.Array,
    w_mod: jax.Array,
):
    del B_x
    hbm = pl.BlockSpec(memory_space=pl.ANY)
    dma = pltpu.SemaphoreType.DMA
    out = pl.pallas_call(
        _kernel,
        out_shape=jax.ShapeDtypeStruct((S, D), BF16),
        in_specs=[hbm] * 6 + [pl.BlockSpec(memory_space=pltpu.VMEM), hbm],
        out_specs=hbm,
        scratch_shapes=[
            pltpu.VMEM((S, D), BF16),
            pltpu.VMEM((HG, D // 2, 3 * GW), U32),
            pltpu.VMEM((D // 2, D), U32),
            pltpu.VMEM((D // 2, F), U32),
            pltpu.VMEM((D // 2, F), U32),
            pltpu.VMEM((F // 2, D), U32),
            pltpu.VMEM((6, D, D), BF16),
            pltpu.VMEM((S // 2, D), U32),
            pltpu.VMEM((6, S // 2, 128), U32),
            pltpu.VMEM((6, S // 2, 128), U32),
            pltpu.VMEM((12, 8 * HP, 128), U32),
            pltpu.VMEM((2, NJ, GW, 128), F32),
            pltpu.VMEM((2, 2 * NJ, GW, 128), F32),
            pltpu.VMEM((2, 2 * NJ, GW, 128), F32),
            pltpu.VMEM((2, 8 * HP, 128), U32),
            pltpu.VMEM((2 * HG - 2, S // 2, 128), U32),
            pltpu.VMEM((2, S // 2, 128), U32),
            pltpu.VMEM((S, D), F32),
            pltpu.VMEM((2, TM, D), F32),
            pltpu.VMEM((7, HM // 2, HD), U32),
            pltpu.VMEM((7, HM // 2, HF), U32),
            pltpu.VMEM((3, HD // 2, F), U32),
            pltpu.VMEM((3, HF // 2, HD), U32),
            pltpu.VMEM((D // DC, TM, DC), BF16),
            pltpu.VMEM((D, 128), F32),
            pltpu.VMEM((6, 8, D), F32),
            dma((S // TM1,)), dma((HG * 3,)), dma((6,)), dma((2 * D // MC,)), dma((4,)), dma((D // DC,)),
        ],
        compiler_params=pltpu.CompilerParams(vmem_limit_bytes=120 * 1024 * 1024,
            flags={"XLA_TPU_EVENLY_DISTRIBUTE_CRITICAL_NODES": True}),
    )(A_x.reshape(S, D), A_wqkv, A_wo, B_w_gate, B_w_up, B_w_down, c, w_mod)
    return out.reshape(1, S, D)
```

```python
import jax
import jax.numpy as jnp
from jax import lax
from jax.experimental import pallas as pl
from jax.experimental.pallas import tpu as pltpu

S, D, F = 2048, 1024, 3584
DH, W = 32, 8
HG, GW = 4, 256
NJ = 8
TM1 = 256
TM = 512
FC = 256
DC = 128
HM, HD, HF = TM // 2, D // 2, F // 2
LB = 64
HP = 36
CFG = (((2, 4), 1), ((2, 4), 1))
MC = 512
STAGE = (4, 4, 6, 8, 99)
PF0 = 0
LR = 128
TIE, TIW = 512, 768
PC = 128
EPS = 1e-5
F32, BF16, U32 = jnp.float32, jnp.bfloat16, jnp.uint32


def _dot(a, b):
    return jnp.dot(a, b, preferred_element_type=F32)


def _ln_mod(x, scale1, shift):
    m = jnp.mean(x, axis=-1, keepdims=True)
    xc = x - m
    v = jnp.mean(xc * xc, axis=-1, keepdims=True)
    return xc * lax.rsqrt(v + EPS) * scale1 + shift


def _unpack(w):
    lo = lax.bitcast_convert_type(w << 16, F32)
    hi = lax.bitcast_convert_type(w & jnp.uint32(0xFFFF0000), F32)
    return lo, hi


def _ld(ref, r):
    return pltpu.bitcast(ref[r, :], BF16)


def _mix(a, na=1, b=(), nb=0):
    b = iter(b)
    done = 0
    for k, _ in enumerate(a):
        while done * na < (k + 1) * nb:
            next(b)
            done += 1
    for _ in b:
        pass


def _lhs_terms(a11, a12, a21, a22):
    terms = (a11 + a22, a21 + a22, a11, a22, a11 + a12, a21 - a11, a12 - a22)
    return [pltpu.bitcast(t.astype(BF16), U32) for t in terms]


def _rhs_terms(b11, b12, b21, b22):
    halves = [(b11 + b22, b12 - b22, b21 - b11, b11 + b12, b21 + b22)
              for b11, b12, b21, b22 in zip(*(_unpack(b) for b in (b11, b12, b21, b22)))]
    return [pltpu.pack_elementwise([lo, hi], packed_dtype=BF16) for lo, hi in zip(*halves)]


def _strassen(lhs, rhs):
    p1, p2, p3, p4, p5, p6, p7 = (_dot(pltpu.bitcast(a, BF16), pltpu.bitcast(b, BF16)) for a, b in zip(lhs, rhs))
    return p1 + p4 - p5 + p7, p3 + p5, p2 + p4, p1 - p2 + p3 + p6


def _bf16_bits(x):
    return lax.bitcast_convert_type(x.astype(BF16).astype(F32), U32)


def _kernel(x_hbm, wqkv_hbm, wo_hbm, wg_hbm, wu_hbm, wd_hbm, c_ref, wmod_hbm, out_hbm,
            x_v, wqkv_v, wo_v, wg_v, wu_v, wd_v, wmod_v, h_v, qkv0_v, qkv1_v, t_v, q_s, k_s, v_s,
            ot_v, o_v, o3_v, x1_v, x2_v, hs_v, as_v, sg_v, sd_v, ob_v, scol_v, mod_v, sem_x, sem_qkv, sem_mod, sem_head, sem_w, sem_o):
    nb1 = S // TM1
    qkv_v = (qkv0_v, qkv1_v)

    def x_cp(i):
        r = pl.ds(i * TM1, TM1)
        return pltpu.make_async_copy(x_hbm.at[r], x_v.at[r], sem_x.at[i])

    def qkv_cp(g, t):
        return pltpu.make_async_copy(wqkv_hbm.at[:, pl.ds(t * D + g * GW, GW)],
                                     wqkv_v.at[g].bitcast(BF16).at[:, pl.ds(t * GW, GW)], sem_qkv.at[g * 3 + t])

    def mod_cp(i):
        return pltpu.make_async_copy(wmod_hbm.at[:, pl.ds(i * D, D)], wmod_v.at[i], sem_mod.at[i])

    def mod_head_cp(i):
        return pltpu.make_async_copy(wmod_hbm.at[:, pl.ds(i * MC, MC)],
                                     wmod_v.at[i * MC // D, :, pl.ds(i * MC % D, MC)], sem_head.at[i])

    w_cps = [pltpu.make_async_copy(s, d, sem_w.at[i]) for i, (s, d) in enumerate(
        ((wo_hbm, wo_v.bitcast(BF16)), (wg_hbm, wg_v.bitcast(BF16)), (wu_hbm, wu_v.bitcast(BF16)), (wd_hbm, wd_v.bitcast(BF16))))]

    def out_cp(i, n):
        cs = pl.ds(pl.multiple_of(n * DC, DC), DC)
        return pltpu.make_async_copy(ob_v.at[n], out_hbm.at[pl.ds(i * TM, TM), cs], sem_o.at[n])

    nm = 2 * D // MC
    head = [mod_head_cp(i) for i in range(nm)] + [x_cp(0)] + [qkv_cp(0, t) for t in range(3)]
    head += [x_cp(i) for i in range(1, nb1)]
    for cp in head[:STAGE[0]]:
        cp.start()

    cf = c_ref[...].astype(F32)
    sc = (cf * jax.nn.sigmoid(cf)).astype(BF16)
    scol_v[...] = jnp.broadcast_to(sc.astype(F32), (128, D)).T
    sc8 = jnp.broadcast_to(sc, (16, D))
    for i in range(nm):
        mod_head_cp(i).wait()
        for cp in head[STAGE[i]:STAGE[i + 1]]:
            cp.start()
        cs = pl.ds(i * MC % D, MC)
        mod_v[i * MC // D, :, cs] = _dot(sc8, wmod_v[i * MC // D, :, cs])[:8]

    def mod_vpu(i, n):
        cs = pl.ds(pl.multiple_of(n * 128, 128), 128)
        p = wmod_v[i, :, cs].astype(F32) * scol_v[...]
        mod_v[i, :, cs] = jnp.broadcast_to(jnp.sum(p, axis=0, keepdims=True), (8, 128))
        yield

    def mod_row(i):
        return mod_v[i, pl.ds(0, 1), :]

    dep = [None]

    def rows(i, n):
        return pl.ds(pl.multiple_of(i * n, n), n)

    def tied(h, i, n):
        k0 = h.shape[1] - n
        late = jnp.tile(lax.bitcast_convert_type(dep[0], U32), (h.shape[0] // 8, n // 128))
        late = jnp.where(i < 0, late, h[:, k0:])
        return jnp.concatenate([h[:, :k0], late], axis=1) if k0 else late

    def proj(g, i, tie=False):
        for t in range(3):
            h = h_v[rows(i, TM1 // 2), :]
            if tie and t == 2:
                h = tied(h, i, TIE)
            y = _dot(pltpu.bitcast(h, BF16), pltpu.bitcast(wqkv_v[g, :, pl.ds(t * GW, GW)], BF16))
            y = pltpu.bitcast(y.astype(BF16), U32)
            for n in range(2):
                qkv_v[g % 2][t * 2 + n, rows(i, TM1 // 2), :] = y[:, n * 128:(n + 1) * 128]
            yield

    def att_load(g, j, u):
        for t, dst in enumerate((q_s, k_s, v_s)):
            for n in range(2):
                w = qkv_v[g % 2][t * 2 + n, pl.ds(j, 128, stride=NJ), :]
                wt = w.T
                for h in range(4):
                    t_v[u * 3 + t, pl.ds((n * 4 + h) * HP, DH), :] = wt[h * DH:(h + 1) * DH]
            for d in range(DH):
                w = t_v[u * 3 + t, pl.ds(d, 8, stride=HP), :]
                r = pl.ds(d * 8, 8)
                if t == 0:
                    dst[0, j, r, :], dst[1, j, r, :] = _unpack(w)
                else:
                    dst[0, NJ + j, r, :], dst[1, NJ + j, r, :] = _unpack(w)
                    dst[0, j, r, :], dst[1, j, r, :] = _unpack(pltpu.roll(w, 1, 1))
            yield

    def att_core(dst, base, j, u):
        qws, ch = CFG[u]
        lane0 = lax.broadcasted_iota(jnp.int32, (8, 128), 1) == 0
        probs = []
        for p in range(2):
            acc = [None] * W
            qw = qws[p]
            for w0 in range(0, W, qw):
                for d in range(DH):
                    r = pl.ds(d * 8, 8)
                    q = q_s[p, j, r, :]
                    if d == 0 and dep[0] is not None:
                        q = jnp.where(j < 0, dep[0], q)
                    for w in range(w0, w0 + qw):
                        t = q * k_s[p, j + (NJ - w), r, :]
                        acc[w] = t if d == 0 else acc[w] + t
                dep[0] = acc[w0]
            lg = [acc[0] * DH ** -0.5]
            for w in range(1, W):
                lg.append(jnp.where(jnp.logical_and(lane0, j < w), -1e9, acc[w] * DH ** -0.5))
            m = lg[0]
            for w in range(1, W):
                m = jnp.maximum(m, lg[w])
            e = [jnp.exp(l - m) for l in lg]
            den = e[0]
            for w in range(1, W):
                den = den + e[w]
            inv = 1.0 / den
            probs.append([x * inv for x in e])
            dep[0] = inv
            yield
        for d in range(DH):
            r = pl.ds(d * 8, 8)
            o = []
            for p in range(2):
                acc = probs[p][0] * v_s[p, j + NJ, r, :]
                for w in range(1, W):
                    acc = acc + probs[p][w] * v_s[p, j + (NJ - w), r, :]
                o.append(acc)
                if d % ch == ch - 1:
                    probs[p][0] = jnp.where(j < 0, acc, probs[p][0])
                    dep[0] = acc
            ot_v[u, pl.ds(d, 8, stride=HP), :] = pltpu.pack_elementwise(o, packed_dtype=BF16)
        for n in range(2):
            ot = jnp.concatenate([ot_v[u, pl.ds((n * 4 + h) * HP, DH), :] for h in range(4)], axis=0)
            dst[base + n, pl.ds(j, 128, stride=NJ), :] = ot.T
        yield

    def o_cols(ref, r):
        return jnp.concatenate([ref[n, r, :] for n in range(ref.shape[0])], axis=1)

    def ln1(i):
        for k in range(TM1 // LR):
            b = i * (TM1 // LR) + k
            h = _ln_mod(x_v[rows(b, LR), :].astype(F32), 1.0 + mod_row(1), mod_row(0))
            h_v[rows(b, LR // 2), :] = pltpu.bitcast(h.astype(BF16), U32)

    def ln2(blk, n):
        starts = [blk * (TM // LB) + half_ * (HM // LB) + n for half_ in range(2)]
        o = jnp.concatenate([o_cols(o3_v, rows(b, LB // 2)) for b in starts], axis=0)
        y = _dot(pltpu.bitcast(o, BF16), _ld(wo_v, pl.ds((HG - 1) * GW // 2, GW // 2)))
        hs = []
        for k, b in enumerate(starts):
            r = rows(b, LB)
            x1 = x_v[r, :].astype(F32) + mod_row(2) * (x1_v[r, :] + y[k * LB:(k + 1) * LB])
            x2_v[blk % 2, rows(k * (HM // LB) + n, LB), :] = x1
            hs.append(_ln_mod(x1, 1.0 + mod_row(4), mod_row(3)))
        terms = _lhs_terms(hs[0][:, :HD], hs[0][:, HD:], hs[1][:, :HD], hs[1][:, HD:])
        for k, t in enumerate(terms):
            hs_v[k, rows(n, LB // 2), :] = t

    def prep_gate_up(step):
        n = HD // 16
        top, bot = rows(step, n), rows(8 + step, n)
        for k in range(F // PC):
            cs = pl.ds(k * PC, PC)
            s1, s3, s4, s6, s7 = _rhs_terms(wg_v[top, cs], wu_v[top, cs], wg_v[bot, cs], wu_v[bot, cs])
            wu_v[top, cs], wg_v[bot, cs] = s3, s4
            sg_v[0, top, cs], sg_v[1, top, cs], sg_v[2, top, cs] = s1, s6, s7

    def prep_down(step):
        steps = HF // FC
        n = HF // 16 // steps
        lo, hi = pl.ds(0, HD), pl.ds(HD, HD)
        for k in range(n):
            top, bot = rows(step * n + k, 8), rows((steps + step) * n + k, 8)
            s1, s3, s4, s6, s7 = _rhs_terms(wd_v[top, lo], wd_v[top, hi], wd_v[bot, lo], wd_v[bot, hi])
            wd_v[top, hi], wd_v[bot, lo] = s3, s4
            sd_v[0, top, lo], sd_v[1, top, lo], sd_v[2, top, lo] = s1, s6, s7

    def prefetch(g):
        nxt = [qkv_cp(g + 1, t) for t in range(3)] if g + 1 < HG else []
        for cp in nxt + [mod_cp(g + 2)] + [w_cps[k] for k in ((1,), (2,), (3,), (0,))[g]]:
            cp.start()

    x_cp(0).wait()
    ln1(0)
    for t in range(3):
        qkv_cp(0, t).wait()

    def first_body(i, carry):
        @pl.when(i + 1 < nb1)
        def _():
            x_cp(i + 1).wait()

        @pl.when(i == PF0)
        def _():
            prefetch(0)
        _mix(proj(0, i))
        ln1(jnp.minimum(i + 1, nb1 - 1))
        return carry
    lax.fori_loop(0, nb1, first_body, 0)

    half = nb1 // 2
    jpb = NJ // half

    def loads(g, j0, nj):
        for u in range(nj):
            yield from att_load(g, j0 + u, u)
            if g + 1 < HG:
                yield from mod_vpu(g + 2, j0 + u)

    def cores(g, i):
        dst, base = (o_v, g * 2) if g + 1 < HG else (o3_v, 0)
        for u in range(jpb):
            yield from att_core(dst, base, i * jpb + u, u)

    def wo_part(i, tie=False):
        for n in range(D // GW):
            cs = pl.ds(n * GW, GW)
            o = o_cols(o_v, rows(i, TM1 // 2))
            if tie and n == D // GW - 1:
                o = tied(o, i, TIW)
            x1_v[rows(i, TM1), cs] = _dot(pltpu.bitcast(o, BF16), pltpu.bitcast(wo_v[pl.ds(0, (HG - 1) * GW // 2), cs], BF16))
            yield

    def overlapped(g, matmul, steps, na, prep):
        nj = NJ // na

        def body_a(i, c):
            if prep is not None:
                prep(i)
            _mix(matmul(i), steps, loads(g, i * nj, nj), (4 if g + 1 < HG else 3) * nj)
            return c
        lax.fori_loop(0, na, body_a, 0)

        def body_b(i, carry):
            dep[0] = None
            _mix(cores(g, i))
            _mix(matmul(na + i, True))
            return carry
        lax.fori_loop(0, half, body_b, 0)

    for g in range(1, HG):
        for t in range(3):
            qkv_cp(g, t).wait()
        mod_cp(g + 1).wait()
        prefetch(g)
        for k in ((), (), (1, 2), ())[g]:
            w_cps[k].wait()
        overlapped(g - 1, lambda i, tie=False, g=g: proj(g, i, tie), 3, half,
                   (None, None, prep_gate_up, lambda i: prep_gate_up(half + i))[g])

    mod_cp(5).wait()
    w_cps[0].wait()
    nd = HD // DC
    nln = HM // LB
    nlate = TM // TM1
    overlapped(HG - 1, wo_part, D // GW, half - nlate, None)

    def late_body(i, c):
        for k in range(nln // nlate):
            ln2(0, i * (nln // nlate) + k)
        _mix(wo_part(nb1 - nlate + i))
        for k in range(NJ // nlate):
            _mix(mod_vpu(5, i * (NJ // nlate) + k))
        return c
    lax.fori_loop(0, nlate, late_body, 0)

    nb = S // TM
    w_cps[3].wait()

    def ffn_body(i, c):
        def gu(f, with_prep):
            if with_prep:
                prep_down(f)
            act = []
            for half_ in range(2):
                cs = rows(half_ * (HF // FC) + f, FC)
                top, bot = pl.ds(0, HD // 2), pl.ds(HD // 2, HD // 2)
                rhs = (sg_v[0, :, cs], wg_v[top, cs], wu_v[top, cs], wg_v[bot, cs], wu_v[bot, cs],
                       sg_v[1, :, cs], sg_v[2, :, cs])
                g_top, u_top, g_bot, u_bot = _strassen([hs_v[k] for k in range(7)], rhs)
                act.append((g_top * jax.nn.sigmoid(g_top) * u_top, g_bot * jax.nn.sigmoid(g_bot) * u_bot))
            for k, t in enumerate(_lhs_terms(act[0][0], act[1][0], act[0][1], act[1][1])):
                as_v[k, :, rows(f, FC)] = t

        @pl.when(i == 0)
        def _():
            lax.fori_loop(0, HF // FC, lambda f, c2: gu(f, True), None)

        @pl.when(i > 0)
        def _():
            lax.fori_loop(0, HF // FC, lambda f, c2: gu(f, False), None)

        @pl.when(i >= 1)
        def _():
            for n in range(2 * nd):
                out_cp(i - 1, n).wait()

        def dn(n, with_ln):
            if with_ln:
                for k in range(nln // nd):
                    ln2(i + 1, n * (nln // nd) + k)
            lo, hi = rows(n, DC), rows(nd + n, DC)
            top, bot = pl.ds(0, HF // 2), pl.ds(HF // 2, HF // 2)
            rhs = (sd_v[0, :, lo], wd_v[top, lo], wd_v[top, hi], wd_v[bot, lo], wd_v[bot, hi],
                   sd_v[1, :, lo], sd_v[2, :, lo])
            c11, c12, c21, c22 = _strassen([as_v[k] for k in range(7)], rhs)
            for m, cs, y_top, y_bot in ((n, lo, c11, c21), (nd + n, hi, c12, c22)):
                gate = mod_v[5, pl.ds(0, 1), cs]
                for r, y in ((pl.ds(0, HM), y_top), (pl.ds(HM, HM), y_bot)):
                    ob_v[m, r, :] = (x2_v[i % 2, r, cs] + gate * y).astype(BF16)
            out_cp(i, n).start()
            out_cp(i, nd + n).start()

        @pl.when(i < nb - 1)
        def _():
            lax.fori_loop(0, nd, lambda n, c2: dn(n, True), None)

        @pl.when(i == nb - 1)
        def _():
            lax.fori_loop(0, nd, lambda n, c2: dn(n, False), None)
        return c
    lax.fori_loop(0, nb, ffn_body, 0)
    for n in range(2 * nd):
        out_cp(nb - 1, n).wait()


@jax.jit
def pallas_adaLN_cond__sliding_local_dilated__swiglu_ffn__prompt_kernel(
    A_x: jax.Array,
    A_wqkv: jax.Array,
    A_wo: jax.Array,
    B_x: jax.Array,
    B_w_gate: jax.Array,
    B_w_up: jax.Array,
    B_w_down: jax.Array,
    c: jax.Array,
    w_mod: jax.Array,
):
    del B_x
    hbm = pl.BlockSpec(memory_space=pl.ANY)
    dma = pltpu.SemaphoreType.DMA
    out = pl.pallas_call(
        _kernel,
        out_shape=jax.ShapeDtypeStruct((S, D), BF16),
        in_specs=[hbm] * 6 + [pl.BlockSpec(memory_space=pltpu.VMEM), hbm],
        out_specs=hbm,
        scratch_shapes=[
            pltpu.VMEM((S, D), BF16),
            pltpu.VMEM((HG, D // 2, 3 * GW), U32),
            pltpu.VMEM((D // 2, D), U32),
            pltpu.VMEM((D // 2, F), U32),
            pltpu.VMEM((D // 2, F), U32),
            pltpu.VMEM((F // 2, D), U32),
            pltpu.VMEM((6, D, D), BF16),
            pltpu.VMEM((S // 2, D), U32),
            pltpu.VMEM((6, S // 2, 128), U32),
            pltpu.VMEM((6, S // 2, 128), U32),
            pltpu.VMEM((12, 8 * HP, 128), U32),
            pltpu.VMEM((2, NJ, GW, 128), F32),
            pltpu.VMEM((2, 2 * NJ, GW, 128), F32),
            pltpu.VMEM((2, 2 * NJ, GW, 128), F32),
            pltpu.VMEM((2, 8 * HP, 128), U32),
            pltpu.VMEM((2 * HG - 2, S // 2, 128), U32),
            pltpu.VMEM((2, S // 2, 128), U32),
            pltpu.VMEM((S, D), F32),
            pltpu.VMEM((2, TM, D), F32),
            pltpu.VMEM((7, HM // 2, HD), U32),
            pltpu.VMEM((7, HM // 2, HF), U32),
            pltpu.VMEM((3, HD // 2, F), U32),
            pltpu.VMEM((3, HF // 2, HD), U32),
            pltpu.VMEM((D // DC, TM, DC), BF16),
            pltpu.VMEM((D, 128), F32),
            pltpu.VMEM((6, 8, D), F32),
            dma((S // TM1,)), dma((HG * 3,)), dma((6,)), dma((2 * D // MC,)), dma((4,)), dma((D // DC,)),
        ],
        compiler_params=pltpu.CompilerParams(vmem_limit_bytes=120 * 1024 * 1024,
            flags={"XLA_TPU_EVENLY_DISTRIBUTE_CRITICAL_NODES": True}),
    )(A_x.reshape(S, D), A_wqkv, A_wo, B_w_gate, B_w_up, B_w_down, c, w_mod)
    return out.reshape(1, S, D)
```

```python
import jax
import jax.numpy as jnp
from jax import lax
from jax.experimental import pallas as pl
from jax.experimental.pallas import tpu as pltpu

S, D, F = 2048, 1024, 3584
DH, W = 32, 8
HG, GW = 4, 256
NJ = 8
TM1 = 256
TM = 512
FC = 256
DC = 128
HM, HD, HF = TM // 2, D // 2, F // 2
HQ = TM1 // 2
LB = 64
HP = 36
CFG = (((2, 4), 1), ((2, 4), 1))
MC = 512
STAGE = (4, 4, 6, 8, 99)
PF0 = 0
LR = 128
TIE, TIW = 4, 768
PC = 128
EPS = 1e-5
F32, BF16, U32 = jnp.float32, jnp.bfloat16, jnp.uint32


def _dot(a, b):
    return jnp.dot(a, b, preferred_element_type=F32)


def _ln_mod(x, scale1, shift):
    m = jnp.mean(x, axis=-1, keepdims=True)
    xc = x - m
    v = jnp.mean(xc * xc, axis=-1, keepdims=True)
    return xc * lax.rsqrt(v + EPS) * scale1 + shift


def _unpack(w):
    lo = lax.bitcast_convert_type(w << 16, F32)
    hi = lax.bitcast_convert_type(w & jnp.uint32(0xFFFF0000), F32)
    return lo, hi


def _ld(ref, r):
    return pltpu.bitcast(ref[r, :], BF16)


def _mix(a, na=1, b=(), nb=0):
    b = iter(b)
    done = 0
    for k, _ in enumerate(a):
        while done * na < (k + 1) * nb:
            next(b)
            done += 1
    for _ in b:
        pass


def _lhs_terms(a11, a12, a21, a22):
    terms = (a11 + a22, a21 + a22, a11, a22, a11 + a12, a21 - a11, a12 - a22)
    return [pltpu.bitcast(t.astype(BF16), U32) for t in terms]


def _rhs_terms(b11, b12, b21, b22):
    halves = [(b11 + b22, b12 - b22, b21 - b11, b11 + b12, b21 + b22)
              for b11, b12, b21, b22 in zip(*(_unpack(b) for b in (b11, b12, b21, b22)))]
    return [pltpu.pack_elementwise([lo, hi], packed_dtype=BF16) for lo, hi in zip(*halves)]


def _strassen(lhs, rhs):
    p1, p2, p3, p4, p5, p6, p7 = (_dot(pltpu.bitcast(a, BF16), pltpu.bitcast(b, BF16)) for a, b in zip(lhs, rhs))
    return p1 + p4 - p5 + p7, p3 + p5, p2 + p4, p1 - p2 + p3 + p6


def _bf16_bits(x):
    return lax.bitcast_convert_type(x.astype(BF16).astype(F32), U32)


def _kernel(x_hbm, wqkv_hbm, wo_hbm, wg_hbm, wu_hbm, wd_hbm, c_ref, wmod_hbm, out_hbm,
            x_v, wqkv_v, wo_v, wg_v, wu_v, wd_v, wmod_v, h_v, sq_v, qkv0_v, qkv1_v, t_v, q_s, k_s, v_s,
            ot_v, o_v, o3_v, x1_v, x2_v, hs_v, as_v, sg_v, sd_v, ob_v, scol_v, mod_v, sem_x, sem_qkv, sem_mod, sem_head, sem_w, sem_o):
    nb1 = S // TM1
    qkv_v = (qkv0_v, qkv1_v)

    def x_cp(i):
        r = pl.ds(i * TM1, TM1)
        return pltpu.make_async_copy(x_hbm.at[r], x_v.at[r], sem_x.at[i])

    def qkv_cp(g, t):
        return pltpu.make_async_copy(wqkv_hbm.at[:, pl.ds(t * D + g * GW, GW)],
                                     wqkv_v.at[g].bitcast(BF16).at[:, pl.ds(t * GW, GW)], sem_qkv.at[g * 3 + t])

    def mod_cp(i):
        return pltpu.make_async_copy(wmod_hbm.at[:, pl.ds(i * D, D)], wmod_v.at[i], sem_mod.at[i])

    def mod_head_cp(i):
        return pltpu.make_async_copy(wmod_hbm.at[:, pl.ds(i * MC, MC)],
                                     wmod_v.at[i * MC // D, :, pl.ds(i * MC % D, MC)], sem_head.at[i])

    w_cps = [pltpu.make_async_copy(s, d, sem_w.at[i]) for i, (s, d) in enumerate(
        ((wo_hbm, wo_v.bitcast(BF16)), (wg_hbm, wg_v.bitcast(BF16)), (wu_hbm, wu_v.bitcast(BF16)), (wd_hbm, wd_v.bitcast(BF16))))]

    def out_cp(i, n):
        cs = pl.ds(pl.multiple_of(n * DC, DC), DC)
        return pltpu.make_async_copy(ob_v.at[n], out_hbm.at[pl.ds(i * TM, TM), cs], sem_o.at[n])

    nm = 2 * D // MC
    head = [mod_head_cp(i) for i in range(nm)] + [x_cp(0)] + [qkv_cp(0, t) for t in range(3)]
    head += [x_cp(i) for i in range(1, nb1)]
    for cp in head[:STAGE[0]]:
        cp.start()

    cf = c_ref[...].astype(F32)
    sc = (cf * jax.nn.sigmoid(cf)).astype(BF16)
    scol_v[...] = jnp.broadcast_to(sc.astype(F32), (128, D)).T
    sc8 = jnp.broadcast_to(sc, (16, D))
    for i in range(nm):
        mod_head_cp(i).wait()
        for cp in head[STAGE[i]:STAGE[i + 1]]:
            cp.start()
        cs = pl.ds(i * MC % D, MC)
        mod_v[i * MC // D, :, cs] = _dot(sc8, wmod_v[i * MC // D, :, cs])[:8]

    def mod_vpu(i, n):
        cs = pl.ds(pl.multiple_of(n * 128, 128), 128)
        p = wmod_v[i, :, cs].astype(F32) * scol_v[...]
        mod_v[i, :, cs] = jnp.broadcast_to(jnp.sum(p, axis=0, keepdims=True), (8, 128))
        yield

    def mod_row(i):
        return mod_v[i, pl.ds(0, 1), :]

    dep = [None]

    def rows(i, n):
        return pl.ds(pl.multiple_of(i * n, n), n)

    def tied(h, i, n):
        k0 = h.shape[1] - n
        late = jnp.tile(lax.bitcast_convert_type(dep[0], U32), (h.shape[0] // 8, n // 128))
        late = jnp.where(i < 0, late, h[:, k0:])
        return jnp.concatenate([h[:, :k0], late], axis=1) if k0 else late

    def proj(g, i, tie=False):
        top, bot = pl.ds(0, HD // 2), pl.ds(HD // 2, HD // 2)
        for t in range(3):
            lhs = [h_v[k, rows(i, HQ // 2), :] for k in range(7)]
            if tie and t == 2:
                lhs = lhs[:TIE] + [tied(h, i, HD) for h in lhs[TIE:]]
            lo, hi = pl.ds(t * 128, 128), pl.ds((3 + t) * 128, 128)
            rhs = (sq_v[g, 0, :, lo], wqkv_v[g, top, lo], wqkv_v[g, top, hi], wqkv_v[g, bot, lo],
                   wqkv_v[g, bot, hi], sq_v[g, 1, :, lo], sq_v[g, 2, :, lo])
            c11, c12, c21, c22 = _strassen(lhs, rhs)
            for n, m, y in ((t, 0, c11), (3 + t, 0, c12), (t, 1, c21), (3 + t, 1, c22)):
                qkv_v[g % 2][n, rows(2 * i + m, HQ // 2), :] = pltpu.bitcast(y.astype(BF16), U32)
            yield

    def prep_qkv(g):
        def step(k, c):
            top, bot = rows(k, 32), rows(HD // 64 + k, 32)
            for t in range(3):
                lo, hi = pl.ds(t * 128, 128), pl.ds((3 + t) * 128, 128)
                s1, s3, s4, s6, s7 = _rhs_terms(wqkv_v[g, top, lo], wqkv_v[g, top, hi],
                                                wqkv_v[g, bot, lo], wqkv_v[g, bot, hi])
                wqkv_v[g, top, hi], wqkv_v[g, bot, lo] = s3, s4
                sq_v[g, 0, top, lo], sq_v[g, 1, top, lo], sq_v[g, 2, top, lo] = s1, s6, s7
            return c
        for t in range(3):
            qkv_cp(g, t).wait()
        lax.fori_loop(0, HD // 64, step, 0)

    def att_load(g, j, u):
        for t, dst in enumerate((q_s, k_s, v_s)):
            for n in range(2):
                w = qkv_v[g % 2][t * 2 + n, pl.ds(j, 128, stride=NJ), :]
                wt = w.T
                for h in range(4):
                    t_v[u * 3 + t, pl.ds((n * 4 + h) * HP, DH), :] = wt[h * DH:(h + 1) * DH]
            for d in range(DH):
                w = t_v[u * 3 + t, pl.ds(d, 8, stride=HP), :]
                r = pl.ds(d * 8, 8)
                if t == 0:
                    dst[0, j, r, :], dst[1, j, r, :] = _unpack(w)
                else:
                    dst[0, NJ + j, r, :], dst[1, NJ + j, r, :] = _unpack(w)
                    dst[0, j, r, :], dst[1, j, r, :] = _unpack(pltpu.roll(w, 1, 1))
            yield

    def att_core(dst, base, j, u):
        qws, ch = CFG[u]
        lane0 = lax.broadcasted_iota(jnp.int32, (8, 128), 1) == 0
        probs = []
        for p in range(2):
            acc = [None] * W
            qw = qws[p]
            for w0 in range(0, W, qw):
                for d in range(DH):
                    r = pl.ds(d * 8, 8)
                    q = q_s[p, j, r, :]
                    if d == 0 and dep[0] is not None:
                        q = jnp.where(j < 0, dep[0], q)
                    for w in range(w0, w0 + qw):
                        t = q * k_s[p, j + (NJ - w), r, :]
                        acc[w] = t if d == 0 else acc[w] + t
                dep[0] = acc[w0]
            lg = [acc[0] * DH ** -0.5]
            for w in range(1, W):
                lg.append(jnp.where(jnp.logical_and(lane0, j < w), -1e9, acc[w] * DH ** -0.5))
            m = lg[0]
            for w in range(1, W):
                m = jnp.maximum(m, lg[w])
            e = [jnp.exp(l - m) for l in lg]
            den = e[0]
            for w in range(1, W):
                den = den + e[w]
            inv = 1.0 / den
            probs.append([x * inv for x in e])
            dep[0] = inv
            yield
        for d in range(DH):
            r = pl.ds(d * 8, 8)
            o = []
            for p in range(2):
                acc = probs[p][0] * v_s[p, j + NJ, r, :]
                for w in range(1, W):
                    acc = acc + probs[p][w] * v_s[p, j + (NJ - w), r, :]
                o.append(acc)
                if d % ch == ch - 1:
                    probs[p][0] = jnp.where(j < 0, acc, probs[p][0])
                    dep[0] = acc
            ot_v[u, pl.ds(d, 8, stride=HP), :] = pltpu.pack_elementwise(o, packed_dtype=BF16)
        for n in range(2):
            ot = jnp.concatenate([ot_v[u, pl.ds((n * 4 + h) * HP, DH), :] for h in range(4)], axis=0)
            dst[base + n, pl.ds(j, 128, stride=NJ), :] = ot.T
        yield

    def o_cols(ref, r):
        return jnp.concatenate([ref[n, r, :] for n in range(ref.shape[0])], axis=1)

    def ln1(i):
        top, bot = (_ln_mod(x_v[rows(2 * i + m, HQ), :].astype(F32), 1.0 + mod_row(1), mod_row(0))
                    for m in range(2))
        for k, t in enumerate(_lhs_terms(top[:, :HD], top[:, HD:], bot[:, :HD], bot[:, HD:])):
            h_v[k, rows(i, HQ // 2), :] = t

    def ln2(blk, n):
        starts = [blk * (TM // LB) + half_ * (HM // LB) + n for half_ in range(2)]
        o = jnp.concatenate([o_cols(o3_v, rows(b, LB // 2)) for b in starts], axis=0)
        y = _dot(pltpu.bitcast(o, BF16), _ld(wo_v, pl.ds((HG - 1) * GW // 2, GW // 2)))
        hs = []
        for k, b in enumerate(starts):
            r = rows(b, LB)
            x1 = x_v[r, :].astype(F32) + mod_row(2) * (x1_v[r, :] + y[k * LB:(k + 1) * LB])
            x2_v[blk % 2, rows(k * (HM // LB) + n, LB), :] = x1
            hs.append(_ln_mod(x1, 1.0 + mod_row(4), mod_row(3)))
        terms = _lhs_terms(hs[0][:, :HD], hs[0][:, HD:], hs[1][:, :HD], hs[1][:, HD:])
        for k, t in enumerate(terms):
            hs_v[k, rows(n, LB // 2), :] = t

    def prep_gate_up(step):
        n = HD // 16
        top, bot = rows(step, n), rows(8 + step, n)
        for k in range(F // PC):
            cs = pl.ds(k * PC, PC)
            s1, s3, s4, s6, s7 = _rhs_terms(wg_v[top, cs], wu_v[top, cs], wg_v[bot, cs], wu_v[bot, cs])
            wu_v[top, cs], wg_v[bot, cs] = s3, s4
            sg_v[0, top, cs], sg_v[1, top, cs], sg_v[2, top, cs] = s1, s6, s7

    def prep_down(step):
        steps = HF // FC
        n = HF // 16 // steps
        lo, hi = pl.ds(0, HD), pl.ds(HD, HD)
        for k in range(n):
            top, bot = rows(step * n + k, 8), rows((steps + step) * n + k, 8)
            s1, s3, s4, s6, s7 = _rhs_terms(wd_v[top, lo], wd_v[top, hi], wd_v[bot, lo], wd_v[bot, hi])
            wd_v[top, hi], wd_v[bot, lo] = s3, s4
            sd_v[0, top, lo], sd_v[1, top, lo], sd_v[2, top, lo] = s1, s6, s7

    def prefetch(g):
        nxt = [qkv_cp(g + 1, t) for t in range(3)] if g + 1 < HG else []
        for cp in nxt + [mod_cp(g + 2)] + [w_cps[k] for k in ((1,), (2,), (3,), (0,))[g]]:
            cp.start()

    x_cp(0).wait()
    ln1(0)
    prep_qkv(0)

    def first_body(i, carry):
        @pl.when(i + 1 < nb1)
        def _():
            x_cp(i + 1).wait()

        @pl.when(i == PF0)
        def _():
            prefetch(0)
        _mix(proj(0, i))
        ln1(jnp.minimum(i + 1, nb1 - 1))
        return carry
    lax.fori_loop(0, nb1, first_body, 0)

    half = nb1 // 2
    jpb = NJ // half

    def loads(g, j0, nj):
        for u in range(nj):
            yield from att_load(g, j0 + u, u)
            if g + 1 < HG:
                yield from mod_vpu(g + 2, j0 + u)

    def cores(g, i):
        dst, base = (o_v, g * 2) if g + 1 < HG else (o3_v, 0)
        for u in range(jpb):
            yield from att_core(dst, base, i * jpb + u, u)

    def wo_part(i, tie=False):
        for n in range(D // GW):
            cs = pl.ds(n * GW, GW)
            o = o_cols(o_v, rows(i, TM1 // 2))
            if tie and n == D // GW - 1:
                o = tied(o, i, TIW)
            x1_v[rows(i, TM1), cs] = _dot(pltpu.bitcast(o, BF16), pltpu.bitcast(wo_v[pl.ds(0, (HG - 1) * GW // 2), cs], BF16))
            yield

    def overlapped(g, matmul, steps, na, prep):
        nj = NJ // na

        def body_a(i, c):
            if prep is not None:
                prep(i)
            _mix(matmul(i), steps, loads(g, i * nj, nj), (4 if g + 1 < HG else 3) * nj)
            return c
        lax.fori_loop(0, na, body_a, 0)

        def body_b(i, carry):
            dep[0] = None
            _mix(cores(g, i))
            _mix(matmul(na + i, True))
            return carry
        lax.fori_loop(0, half, body_b, 0)

    for g in range(1, HG):
        mod_cp(g + 1).wait()
        prefetch(g)
        prep_qkv(g)
        for k in ((), (), (1, 2), ())[g]:
            w_cps[k].wait()
        overlapped(g - 1, lambda i, tie=False, g=g: proj(g, i, tie), 3, half,
                   (None, None, prep_gate_up, lambda i: prep_gate_up(half + i))[g])

    mod_cp(5).wait()
    w_cps[0].wait()
    nd = HD // DC
    nln = HM // LB
    nlate = TM // TM1
    overlapped(HG - 1, wo_part, D // GW, half - nlate, None)

    def late_body(i, c):
        for k in range(nln // nlate):
            ln2(0, i * (nln // nlate) + k)
        _mix(wo_part(nb1 - nlate + i))
        return c
    lax.fori_loop(0, nlate, late_body, 0)

    nb = S // TM
    w_cps[3].wait()

    def ffn_body(i, c):
        def gu(f, with_prep):
            if with_prep:
                prep_down(f)
                for k in range(2):
                    _mix(mod_vpu(5, 2 * jnp.minimum(f, NJ // 2 - 1) + k))
            act = []
            for half_ in range(2):
                cs = rows(half_ * (HF // FC) + f, FC)
                top, bot = pl.ds(0, HD // 2), pl.ds(HD // 2, HD // 2)
                rhs = (sg_v[0, :, cs], wg_v[top, cs], wu_v[top, cs], wg_v[bot, cs], wu_v[bot, cs],
                       sg_v[1, :, cs], sg_v[2, :, cs])
                g_top, u_top, g_bot, u_bot = _strassen([hs_v[k] for k in range(7)], rhs)
                act.append((g_top * jax.nn.sigmoid(g_top) * u_top, g_bot * jax.nn.sigmoid(g_bot) * u_bot))
            for k, t in enumerate(_lhs_terms(act[0][0], act[1][0], act[0][1], act[1][1])):
                as_v[k, :, rows(f, FC)] = t

        @pl.when(i == 0)
        def _():
            lax.fori_loop(0, HF // FC, lambda f, c2: gu(f, True), None)

        @pl.when(i > 0)
        def _():
            lax.fori_loop(0, HF // FC, lambda f, c2: gu(f, False), None)

        @pl.when(i >= 1)
        def _():
            for n in range(2 * nd):
                out_cp(i - 1, n).wait()

        def dn(n, with_ln):
            if with_ln:
                for k in range(nln // nd):
                    ln2(i + 1, n * (nln // nd) + k)
            lo, hi = rows(n, DC), rows(nd + n, DC)
            top, bot = pl.ds(0, HF // 2), pl.ds(HF // 2, HF // 2)
            rhs = (sd_v[0, :, lo], wd_v[top, lo], wd_v[top, hi], wd_v[bot, lo], wd_v[bot, hi],
                   sd_v[1, :, lo], sd_v[2, :, lo])
            c11, c12, c21, c22 = _strassen([as_v[k] for k in range(7)], rhs)
            for m, cs, y_top, y_bot in ((n, lo, c11, c21), (nd + n, hi, c12, c22)):
                gate = mod_v[5, pl.ds(0, 1), cs]
                for r, y in ((pl.ds(0, HM), y_top), (pl.ds(HM, HM), y_bot)):
                    ob_v[m, r, :] = (x2_v[i % 2, r, cs] + gate * y).astype(BF16)
            out_cp(i, n).start()
            out_cp(i, nd + n).start()

        @pl.when(i < nb - 1)
        def _():
            lax.fori_loop(0, nd, lambda n, c2: dn(n, True), None)

        @pl.when(i == nb - 1)
        def _():
            lax.fori_loop(0, nd, lambda n, c2: dn(n, False), None)
        return c
    lax.fori_loop(0, nb, ffn_body, 0)
    for n in range(2 * nd):
        out_cp(nb - 1, n).wait()


@jax.jit
def pallas_adaLN_cond__sliding_local_dilated__swiglu_ffn__prompt_kernel(
    A_x: jax.Array,
    A_wqkv: jax.Array,
    A_wo: jax.Array,
    B_x: jax.Array,
    B_w_gate: jax.Array,
    B_w_up: jax.Array,
    B_w_down: jax.Array,
    c: jax.Array,
    w_mod: jax.Array,
):
    del B_x
    hbm = pl.BlockSpec(memory_space=pl.ANY)
    dma = pltpu.SemaphoreType.DMA
    out = pl.pallas_call(
        _kernel,
        out_shape=jax.ShapeDtypeStruct((S, D), BF16),
        in_specs=[hbm] * 6 + [pl.BlockSpec(memory_space=pltpu.VMEM), hbm],
        out_specs=hbm,
        scratch_shapes=[
            pltpu.VMEM((S, D), BF16),
            pltpu.VMEM((HG, D // 2, 3 * GW), U32),
            pltpu.VMEM((D // 2, D), U32),
            pltpu.VMEM((D // 2, F), U32),
            pltpu.VMEM((D // 2, F), U32),
            pltpu.VMEM((F // 2, D), U32),
            pltpu.VMEM((6, D, D), BF16),
            pltpu.VMEM((7, S // 4, HD), U32),
            pltpu.VMEM((HG, 3, HD // 2, 3 * 128), U32),
            pltpu.VMEM((6, S // 2, 128), U32),
            pltpu.VMEM((6, S // 2, 128), U32),
            pltpu.VMEM((12, 8 * HP, 128), U32),
            pltpu.VMEM((2, NJ, GW, 128), F32),
            pltpu.VMEM((2, 2 * NJ, GW, 128), F32),
            pltpu.VMEM((2, 2 * NJ, GW, 128), F32),
            pltpu.VMEM((2, 8 * HP, 128), U32),
            pltpu.VMEM((2 * HG - 2, S // 2, 128), U32),
            pltpu.VMEM((2, S // 2, 128), U32),
            pltpu.VMEM((S, D), F32),
            pltpu.VMEM((2, TM, D), F32),
            pltpu.VMEM((7, HM // 2, HD), U32),
            pltpu.VMEM((7, HM // 2, HF), U32),
            pltpu.VMEM((3, HD // 2, F), U32),
            pltpu.VMEM((3, HF // 2, HD), U32),
            pltpu.VMEM((D // DC, TM, DC), BF16),
            pltpu.VMEM((D, 128), F32),
            pltpu.VMEM((6, 8, D), F32),
            dma((S // TM1,)), dma((HG * 3,)), dma((6,)), dma((2 * D // MC,)), dma((4,)), dma((D // DC,)),
        ],
        compiler_params=pltpu.CompilerParams(vmem_limit_bytes=120 * 1024 * 1024,
            flags={"XLA_TPU_EVENLY_DISTRIBUTE_CRITICAL_NODES": True}),
    )(A_x.reshape(S, D), A_wqkv, A_wo, B_w_gate, B_w_up, B_w_down, c, w_mod)
    return out.reshape(1, S, D)
```

```python
import jax
import jax.numpy as jnp
from jax import lax
from jax.experimental import pallas as pl
from jax.experimental.pallas import tpu as pltpu

S, D, F = 2048, 1024, 3584
DH, W = 32, 8
HG, GW = 4, 256
NJ = 8
TM1 = 256
TM = 512
FC = 256
DC = 128
HM, HD, HF = TM // 2, D // 2, F // 2
HQ = TM1 // 2
LB = 64
HP = 36
CFG = (((2, 4), 1), ((2, 4), 1))
MC = 512
STAGE = (4, 4, 6, 8, 99)
PF0 = 0
LR = 128
TIE, TIW = 4, 768
PC = 128
EPS = 1e-5
F32, BF16, U32 = jnp.float32, jnp.bfloat16, jnp.uint32


def _dot(a, b):
    return jnp.dot(a, b, preferred_element_type=F32)


def _ln_mod(x, scale1, shift):
    m = jnp.mean(x, axis=-1, keepdims=True)
    xc = x - m
    v = jnp.mean(xc * xc, axis=-1, keepdims=True)
    return xc * lax.rsqrt(v + EPS) * scale1 + shift


def _unpack(w):
    lo = lax.bitcast_convert_type(w << 16, F32)
    hi = lax.bitcast_convert_type(w & jnp.uint32(0xFFFF0000), F32)
    return lo, hi


def _ld(ref, r):
    return pltpu.bitcast(ref[r, :], BF16)


def _mix(a, na=1, b=(), nb=0):
    b = iter(b)
    done = 0
    for k, _ in enumerate(a):
        while done * na < (k + 1) * nb:
            next(b)
            done += 1
    for _ in b:
        pass


def _lhs_terms(a11, a12, a21, a22):
    terms = (a11 + a22, a21 + a22, a11, a22, a11 + a12, a21 - a11, a12 - a22)
    return [pltpu.bitcast(t.astype(BF16), U32) for t in terms]


def _rhs_terms(b11, b12, b21, b22):
    halves = [(b11 + b22, b12 - b22, b21 - b11, b11 + b12, b21 + b22)
              for b11, b12, b21, b22 in zip(*(_unpack(b) for b in (b11, b12, b21, b22)))]
    return [pltpu.pack_elementwise([lo, hi], packed_dtype=BF16) for lo, hi in zip(*halves)]


def _strassen(lhs, rhs):
    def p(k):
        return _dot(pltpu.bitcast(lhs[k - 1], BF16), pltpu.bitcast(rhs[k - 1], BF16))
    p1, p4, p5, p7, p2, p3, p6 = (p(k) for k in (1, 4, 5, 7, 2, 3, 6))
    return p1 + p4 - p5 + p7, p3 + p5, p2 + p4, p1 - p2 + p3 + p6


def _kernel(x_hbm, wqkv_hbm, wo_hbm, wg_hbm, wu_hbm, wd_hbm, c_ref, wmod_hbm, out_hbm,
            x_v, wqkv_v, wo_v, wg_v, wu_v, wd_v, wmod_v, h_v, sq_v, qkv0_v, qkv1_v, t_v, q_s, k_s, v_s,
            ot_v, o_v, o3_v, x1_v, x2_v, hs_v, as_v, sg_v, sd_v, ob_v, scol_v, mod_v, sem_x, sem_qkv, sem_mod, sem_head, sem_w, sem_o):
    nb1 = S // TM1
    qkv_v = (qkv0_v, qkv1_v)

    def x_cp(i):
        r = pl.ds(i * TM1, TM1)
        return pltpu.make_async_copy(x_hbm.at[r], x_v.at[r], sem_x.at[i])

    def qkv_cp(g, t):
        return pltpu.make_async_copy(wqkv_hbm.at[:, pl.ds(t * D + g * GW, GW)],
                                     wqkv_v.at[g].bitcast(BF16).at[:, pl.ds(t * GW, GW)], sem_qkv.at[g * 3 + t])

    def mod_cp(i):
        return pltpu.make_async_copy(wmod_hbm.at[:, pl.ds(i * D, D)], wmod_v.at[i], sem_mod.at[i])

    def mod_head_cp(i):
        return pltpu.make_async_copy(wmod_hbm.at[:, pl.ds(i * MC, MC)],
                                     wmod_v.at[i * MC // D, :, pl.ds(i * MC % D, MC)], sem_head.at[i])

    w_cps = [pltpu.make_async_copy(s, d, sem_w.at[i]) for i, (s, d) in enumerate(
        ((wo_hbm, wo_v.bitcast(BF16)), (wg_hbm, wg_v.bitcast(BF16)), (wu_hbm, wu_v.bitcast(BF16)), (wd_hbm, wd_v.bitcast(BF16))))]

    def out_cp(i, n):
        cs = pl.ds(pl.multiple_of(n * DC, DC), DC)
        return pltpu.make_async_copy(ob_v.at[n], out_hbm.at[pl.ds(i * TM, TM), cs], sem_o.at[n])

    nm = 2 * D // MC
    head = [mod_head_cp(i) for i in range(nm)] + [x_cp(0)] + [qkv_cp(0, t) for t in range(3)]
    head += [x_cp(i) for i in range(1, nb1)]
    for cp in head[:STAGE[0]]:
        cp.start()

    cf = c_ref[...].astype(F32)
    sc = (cf * jax.nn.sigmoid(cf)).astype(BF16)
    scol_v[...] = jnp.broadcast_to(sc.astype(F32), (128, D)).T
    sc8 = jnp.broadcast_to(sc, (16, D))
    for i in range(nm):
        mod_head_cp(i).wait()
        for cp in head[STAGE[i]:STAGE[i + 1]]:
            cp.start()
        cs = pl.ds(i * MC % D, MC)
        mod_v[i * MC // D, :, cs] = _dot(sc8, wmod_v[i * MC // D, :, cs])[:8]

    def mod_vpu(i, n):
        cs = pl.ds(pl.multiple_of(n * 128, 128), 128)
        p = wmod_v[i, :, cs].astype(F32) * scol_v[...]
        mod_v[i, :, cs] = jnp.broadcast_to(jnp.sum(p, axis=0, keepdims=True), (8, 128))
        yield

    def mod_row(i):
        return mod_v[i, pl.ds(0, 1), :]

    dep = [None]

    def rows(i, n):
        return pl.ds(pl.multiple_of(i * n, n), n)

    def tied(h, i, n):
        k0 = h.shape[1] - n
        late = jnp.tile(lax.bitcast_convert_type(dep[0], U32), (h.shape[0] // 8, n // 128))
        late = jnp.where(i < 0, late, h[:, k0:])
        return jnp.concatenate([h[:, :k0], late], axis=1) if k0 else late

    def proj(g, i, tie=False):
        top, bot = pl.ds(0, HD // 2), pl.ds(HD // 2, HD // 2)
        for t in range(3):
            lhs = [h_v[k, rows(i, HQ // 2), :] for k in range(7)]
            if tie and t == 2:
                lhs = lhs[:TIE] + [tied(h, i, HD) for h in lhs[TIE:]]
            lo, hi = pl.ds(t * 128, 128), pl.ds((3 + t) * 128, 128)
            rhs = (sq_v[g, 0, :, lo], wqkv_v[g, top, lo], wqkv_v[g, top, hi], wqkv_v[g, bot, lo],
                   wqkv_v[g, bot, hi], sq_v[g, 1, :, lo], sq_v[g, 2, :, lo])
            c11, c12, c21, c22 = _strassen(lhs, rhs)
            for n, m, y in ((t, 0, c11), (3 + t, 0, c12), (t, 1, c21), (3 + t, 1, c22)):
                qkv_v[g % 2][n, rows(2 * i + m, HQ // 2), :] = pltpu.bitcast(y.astype(BF16), U32)
            yield

    def prep_qkv(g):
        def step(k, c):
            top, bot = rows(k, 32), rows(HD // 64 + k, 32)
            for t in range(3):
                lo, hi = pl.ds(t * 128, 128), pl.ds((3 + t) * 128, 128)
                s1, s3, s4, s6, s7 = _rhs_terms(wqkv_v[g, top, lo], wqkv_v[g, top, hi],
                                                wqkv_v[g, bot, lo], wqkv_v[g, bot, hi])
                wqkv_v[g, top, hi], wqkv_v[g, bot, lo] = s3, s4
                sq_v[g, 0, top, lo], sq_v[g, 1, top, lo], sq_v[g, 2, top, lo] = s1, s6, s7
            return c
        for t in range(3):
            qkv_cp(g, t).wait()
        lax.fori_loop(0, HD // 64, step, 0)

    def att_load(g, j, u):
        for t, dst in enumerate((q_s, k_s, v_s)):
            for n in range(2):
                w = qkv_v[g % 2][t * 2 + n, pl.ds(j, 128, stride=NJ), :]
                wt = w.T
                for h in range(4):
                    t_v[u * 3 + t, pl.ds((n * 4 + h) * HP, DH), :] = wt[h * DH:(h + 1) * DH]
            for d in range(DH):
                w = t_v[u * 3 + t, pl.ds(d, 8, stride=HP), :]
                r = pl.ds(d * 8, 8)
                if t == 0:
                    dst[0, j, r, :], dst[1, j, r, :] = _unpack(w)
                else:
                    dst[0, NJ + j, r, :], dst[1, NJ + j, r, :] = _unpack(w)
                    dst[0, j, r, :], dst[1, j, r, :] = _unpack(pltpu.roll(w, 1, 1))
            yield

    def att_core(dst, base, j, u):
        qws, ch = CFG[u]
        lane0 = lax.broadcasted_iota(jnp.int32, (8, 128), 1) == 0
        probs = []
        for p in range(2):
            acc = [None] * W
            qw = qws[p]
            for w0 in range(0, W, qw):
                for d in range(DH):
                    r = pl.ds(d * 8, 8)
                    q = q_s[p, j, r, :]
                    if d == 0 and dep[0] is not None:
                        q = jnp.where(j < 0, dep[0], q)
                    for w in range(w0, w0 + qw):
                        t = q * k_s[p, j + (NJ - w), r, :]
                        acc[w] = t if d == 0 else acc[w] + t
                dep[0] = acc[w0]
            lg = [acc[0] * DH ** -0.5]
            for w in range(1, W):
                lg.append(jnp.where(jnp.logical_and(lane0, j < w), -1e9, acc[w] * DH ** -0.5))
            m = lg[0]
            for w in range(1, W):
                m = jnp.maximum(m, lg[w])
            e = [jnp.exp(l - m) for l in lg]
            den = e[0]
            for w in range(1, W):
                den = den + e[w]
            inv = 1.0 / den
            probs.append([x * inv for x in e])
            dep[0] = inv
            yield
        for d in range(DH):
            r = pl.ds(d * 8, 8)
            o = []
            for p in range(2):
                acc = probs[p][0] * v_s[p, j + NJ, r, :]
                for w in range(1, W):
                    acc = acc + probs[p][w] * v_s[p, j + (NJ - w), r, :]
                o.append(acc)
                if d % ch == ch - 1:
                    probs[p][0] = jnp.where(j < 0, acc, probs[p][0])
                    dep[0] = acc
            ot_v[u, pl.ds(d, 8, stride=HP), :] = pltpu.pack_elementwise(o, packed_dtype=BF16)
        for n in range(2):
            ot = jnp.concatenate([ot_v[u, pl.ds((n * 4 + h) * HP, DH), :] for h in range(4)], axis=0)
            dst[base + n, pl.ds(j, 128, stride=NJ), :] = ot.T
        yield

    def o_cols(ref, r):
        return jnp.concatenate([ref[n, r, :] for n in range(ref.shape[0])], axis=1)

    def ln1(i):
        top, bot = (_ln_mod(x_v[rows(2 * i + m, HQ), :].astype(F32), 1.0 + mod_row(1), mod_row(0))
                    for m in range(2))
        for k, t in enumerate(_lhs_terms(top[:, :HD], top[:, HD:], bot[:, :HD], bot[:, HD:])):
            h_v[k, rows(i, HQ // 2), :] = t

    def ln2(blk, n):
        starts = [blk * (TM // LB) + half_ * (HM // LB) + n for half_ in range(2)]
        o = jnp.concatenate([o_cols(o3_v, rows(b, LB // 2)) for b in starts], axis=0)
        y = _dot(pltpu.bitcast(o, BF16), _ld(wo_v, pl.ds((HG - 1) * GW // 2, GW // 2)))
        hs = []
        for k, b in enumerate(starts):
            r = rows(b, LB)
            x1 = x_v[r, :].astype(F32) + mod_row(2) * (x1_v[r, :] + y[k * LB:(k + 1) * LB])
            x2_v[blk % 2, rows(k * (HM // LB) + n, LB), :] = x1
            hs.append(_ln_mod(x1, 1.0 + mod_row(4), mod_row(3)))
        terms = _lhs_terms(hs[0][:, :HD], hs[0][:, HD:], hs[1][:, :HD], hs[1][:, HD:])
        for k, t in enumerate(terms):
            hs_v[k, rows(n, LB // 2), :] = t

    def prep_gate_up(step):
        n = HD // 16
        top, bot = rows(step, n), rows(8 + step, n)
        for k in range(F // PC):
            cs = pl.ds(k * PC, PC)
            s1, s3, s4, s6, s7 = _rhs_terms(wg_v[top, cs], wu_v[top, cs], wg_v[bot, cs], wu_v[bot, cs])
            wu_v[top, cs], wg_v[bot, cs] = s3, s4
            sg_v[0, top, cs], sg_v[1, top, cs], sg_v[2, top, cs] = s1, s6, s7

    def prep_down(step):
        steps = HF // FC
        n = HF // 16 // steps
        lo, hi = pl.ds(0, HD), pl.ds(HD, HD)
        for k in range(n):
            top, bot = rows(step * n + k, 8), rows((steps + step) * n + k, 8)
            s1, s3, s4, s6, s7 = _rhs_terms(wd_v[top, lo], wd_v[top, hi], wd_v[bot, lo], wd_v[bot, hi])
            wd_v[top, hi], wd_v[bot, lo] = s3, s4
            sd_v[0, top, lo], sd_v[1, top, lo], sd_v[2, top, lo] = s1, s6, s7

    def prefetch(g):
        nxt = [qkv_cp(g + 1, t) for t in range(3)] if g + 1 < HG else []
        for cp in nxt + [mod_cp(g + 2)] + [w_cps[k] for k in ((1,), (2,), (3,), (0,))[g]]:
            cp.start()

    x_cp(0).wait()
    ln1(0)
    prep_qkv(0)

    def first_body(i, carry):
        @pl.when(i + 1 < nb1)
        def _():
            x_cp(i + 1).wait()

        @pl.when(i == PF0)
        def _():
            prefetch(0)
        _mix(proj(0, i))
        ln1(jnp.minimum(i + 1, nb1 - 1))
        return carry
    lax.fori_loop(0, nb1, first_body, 0)

    half = nb1 // 2
    jpb = NJ // half

    def loads(g, j0, nj):
        for u in range(nj):
            yield from att_load(g, j0 + u, u)
            if g + 1 < HG:
                yield from mod_vpu(g + 2, j0 + u)

    def cores(g, i):
        dst, base = (o_v, g * 2) if g + 1 < HG else (o3_v, 0)
        for u in range(jpb):
            yield from att_core(dst, base, i * jpb + u, u)

    def wo_part(i, tie=False):
        for n in range(D // GW):
            cs = pl.ds(n * GW, GW)
            o = o_cols(o_v, rows(i, TM1 // 2))
            if tie and n == D // GW - 1:
                o = tied(o, i, TIW)
            x1_v[rows(i, TM1), cs] = _dot(pltpu.bitcast(o, BF16), pltpu.bitcast(wo_v[pl.ds(0, (HG - 1) * GW // 2), cs], BF16))
            yield

    def overlapped(g, matmul, steps, na, prep):
        nj = NJ // na

        def body_a(i, c):
            if prep is not None:
                prep(i)
            _mix(matmul(i), steps, loads(g, i * nj, nj), (4 if g + 1 < HG else 3) * nj)
            return c
        lax.fori_loop(0, na, body_a, 0)

        def body_b(i, carry):
            dep[0] = None
            _mix(cores(g, i))
            _mix(matmul(na + i, True))
            return carry
        lax.fori_loop(0, half, body_b, 0)

    for g in range(1, HG):
        mod_cp(g + 1).wait()
        prefetch(g)
        prep_qkv(g)
        for k in ((), (), (1, 2), ())[g]:
            w_cps[k].wait()
        overlapped(g - 1, lambda i, tie=False, g=g: proj(g, i, tie), 3, half,
                   (None, None, prep_gate_up, lambda i: prep_gate_up(half + i))[g])

    mod_cp(5).wait()
    w_cps[0].wait()
    nd = HD // DC
    nln = HM // LB
    nlate = TM // TM1
    overlapped(HG - 1, wo_part, D // GW, half - nlate, None)

    def late_body(i, c):
        for k in range(nln // nlate):
            ln2(0, i * (nln // nlate) + k)
        _mix(wo_part(nb1 - nlate + i))
        return c
    lax.fori_loop(0, nlate, late_body, 0)

    nb = S // TM
    w_cps[3].wait()

    def ffn_body(i, c):
        def gu(f, with_prep):
            if with_prep:
                prep_down(f)
                for k in range(2):
                    _mix(mod_vpu(5, 2 * jnp.minimum(f, NJ // 2 - 1) + k))
            for q in range(FC // 128):
                act = []
                for half_ in range(2):
                    cs = rows((half_ * (HF // FC) + f) * (FC // 128) + q, 128)
                    top, bot = pl.ds(0, HD // 2), pl.ds(HD // 2, HD // 2)
                    rhs = (sg_v[0, :, cs], wg_v[top, cs], wu_v[top, cs], wg_v[bot, cs], wu_v[bot, cs],
                           sg_v[1, :, cs], sg_v[2, :, cs])
                    g_top, u_top, g_bot, u_bot = _strassen([hs_v[k] for k in range(7)], rhs)
                    act.append((g_top * jax.nn.sigmoid(g_top) * u_top, g_bot * jax.nn.sigmoid(g_bot) * u_bot))
                for k, t in enumerate(_lhs_terms(act[0][0], act[1][0], act[0][1], act[1][1])):
                    as_v[k, :, rows(f * (FC // 128) + q, 128)] = t

        @pl.when(i == 0)
        def _():
            lax.fori_loop(0, HF // FC, lambda f, c2: gu(f, True), None)

        @pl.when(i > 0)
        def _():
            lax.fori_loop(0, HF // FC, lambda f, c2: gu(f, False), None)

        @pl.when(i >= 1)
        def _():
            for n in range(2 * nd):
                out_cp(i - 1, n).wait()

        def dn(n, with_ln):
            if with_ln:
                for k in range(nln // nd):
                    ln2(i + 1, n * (nln // nd) + k)
            lo, hi = rows(n, DC), rows(nd + n, DC)
            top, bot = pl.ds(0, HF // 2), pl.ds(HF // 2, HF // 2)
            rhs = (sd_v[0, :, lo], wd_v[top, lo], wd_v[top, hi], wd_v[bot, lo], wd_v[bot, hi],
                   sd_v[1, :, lo], sd_v[2, :, lo])
            c11, c12, c21, c22 = _strassen([as_v[k] for k in range(7)], rhs)
            for m, cs, y_top, y_bot in ((n, lo, c11, c21), (nd + n, hi, c12, c22)):
                gate = mod_v[5, pl.ds(0, 1), cs]
                for r, y in ((pl.ds(0, HM), y_top), (pl.ds(HM, HM), y_bot)):
                    ob_v[m, r, :] = (x2_v[i % 2, r, cs] + gate * y).astype(BF16)
            out_cp(i, n).start()
            out_cp(i, nd + n).start()

        @pl.when(i < nb - 1)
        def _():
            lax.fori_loop(0, nd, lambda n, c2: dn(n, True), None)

        @pl.when(i == nb - 1)
        def _():
            lax.fori_loop(0, nd, lambda n, c2: dn(n, False), None)
        return c
    lax.fori_loop(0, nb, ffn_body, 0)
    for n in range(2 * nd):
        out_cp(nb - 1, n).wait()


@jax.jit
def pallas_adaLN_cond__sliding_local_dilated__swiglu_ffn__prompt_kernel(
    A_x: jax.Array,
    A_wqkv: jax.Array,
    A_wo: jax.Array,
    B_x: jax.Array,
    B_w_gate: jax.Array,
    B_w_up: jax.Array,
    B_w_down: jax.Array,
    c: jax.Array,
    w_mod: jax.Array,
):
    del B_x
    hbm = pl.BlockSpec(memory_space=pl.ANY)
    dma = pltpu.SemaphoreType.DMA
    out = pl.pallas_call(
        _kernel,
        out_shape=jax.ShapeDtypeStruct((S, D), BF16),
        in_specs=[hbm] * 6 + [pl.BlockSpec(memory_space=pltpu.VMEM), hbm],
        out_specs=hbm,
        scratch_shapes=[
            pltpu.VMEM((S, D), BF16),
            pltpu.VMEM((HG, D // 2, 3 * GW), U32),
            pltpu.VMEM((D // 2, D), U32),
            pltpu.VMEM((D // 2, F), U32),
            pltpu.VMEM((D // 2, F), U32),
            pltpu.VMEM((F // 2, D), U32),
            pltpu.VMEM((6, D, D), BF16),
            pltpu.VMEM((7, S // 4, HD), U32),
            pltpu.VMEM((HG, 3, HD // 2, 3 * 128), U32),
            pltpu.VMEM((6, S // 2, 128), U32),
            pltpu.VMEM((6, S // 2, 128), U32),
            pltpu.VMEM((12, 8 * HP, 128), U32),
            pltpu.VMEM((2, NJ, GW, 128), F32),
            pltpu.VMEM((2, 2 * NJ, GW, 128), F32),
            pltpu.VMEM((2, 2 * NJ, GW, 128), F32),
            pltpu.VMEM((2, 8 * HP, 128), U32),
            pltpu.VMEM((2 * HG - 2, S // 2, 128), U32),
            pltpu.VMEM((2, S // 2, 128), U32),
            pltpu.VMEM((S, D), F32),
            pltpu.VMEM((2, TM, D), F32),
            pltpu.VMEM((7, HM // 2, HD), U32),
            pltpu.VMEM((7, HM // 2, HF), U32),
            pltpu.VMEM((3, HD // 2, F), U32),
            pltpu.VMEM((3, HF // 2, HD), U32),
            pltpu.VMEM((D // DC, TM, DC), BF16),
            pltpu.VMEM((D, 128), F32),
            pltpu.VMEM((6, 8, D), F32),
            dma((S // TM1,)), dma((HG * 3,)), dma((6,)), dma((2 * D // MC,)), dma((4,)), dma((D // DC,)),
        ],
        compiler_params=pltpu.CompilerParams(vmem_limit_bytes=120 * 1024 * 1024,
            flags={"XLA_TPU_EVENLY_DISTRIBUTE_CRITICAL_NODES": True}),
    )(A_x.reshape(S, D), A_wqkv, A_wo, B_w_gate, B_w_up, B_w_down, c, w_mod)
    return out.reshape(1, S, D)
```

```python
import jax
import jax.numpy as jnp
from jax import lax
from jax.experimental import pallas as pl
from jax.experimental.pallas import tpu as pltpu

S, D, F = 2048, 1024, 3584
DH, W = 32, 8
HG, GW = 4, 256
NJ = 8
TM1 = 256
TM = 512
FC = 256
DC = 128
HM, HD, HF = TM // 2, D // 2, F // 2
HQ = TM1 // 2
LB = 64
HP = 36
CFG = (((2, 4), 1), ((2, 4), 1))
MC = 512
STAGE = (4, 4, 6, 8, 99)
TIE, TIW = 4, 768
PC = 128
EPS = 1e-5
F32, BF16, U32 = jnp.float32, jnp.bfloat16, jnp.uint32


def _dot(a, b):
    return jnp.dot(a, b, preferred_element_type=F32)


def _ln_mod(x, scale1, shift):
    m = jnp.mean(x, axis=-1, keepdims=True)
    xc = x - m
    v = jnp.mean(xc * xc, axis=-1, keepdims=True)
    return xc * lax.rsqrt(v + EPS) * scale1 + shift


def _unpack(w):
    lo = lax.bitcast_convert_type(w << 16, F32)
    hi = lax.bitcast_convert_type(w & jnp.uint32(0xFFFF0000), F32)
    return lo, hi


def _ld(ref, r):
    return pltpu.bitcast(ref[r, :], BF16)


def _mix(a, na=1, b=(), nb=0):
    b = iter(b)
    done = 0
    for k, _ in enumerate(a):
        while done * na < (k + 1) * nb:
            next(b)
            done += 1
    for _ in b:
        pass


def _lhs_terms(a11, a12, a21, a22):
    terms = (a11 + a22, a21 + a22, a11, a22, a11 + a12, a21 - a11, a12 - a22)
    return [pltpu.bitcast(t.astype(BF16), U32) for t in terms]


def _rhs_terms(b11, b12, b21, b22):
    halves = [(b11 + b22, b12 - b22, b21 - b11, b11 + b12, b21 + b22)
              for b11, b12, b21, b22 in zip(*(_unpack(b) for b in (b11, b12, b21, b22)))]
    return [pltpu.pack_elementwise([lo, hi], packed_dtype=BF16) for lo, hi in zip(*halves)]


def _strassen(lhs, rhs):
    def p(k):
        return _dot(pltpu.bitcast(lhs[k - 1], BF16), pltpu.bitcast(rhs[k - 1], BF16))
    p1, p4, p5, p7, p2, p3, p6 = (p(k) for k in (1, 4, 5, 7, 2, 3, 6))
    return p1 + p4 - p5 + p7, p3 + p5, p2 + p4, p1 - p2 + p3 + p6


def _kernel(x_hbm, wqkv_hbm, wo_hbm, wg_hbm, wu_hbm, wd_hbm, c_ref, wmod_hbm, out_hbm,
            x_v, wqkv_v, wo_v, wg_v, wu_v, wd_v, wmod_v, h_v, sq_v, qkv0_v, qkv1_v, t_v, q_s, k_s, v_s,
            ot_v, o_v, o3_v, x1_v, x2_v, hs_v, as_v, sg_v, sd_v, ob_v, scol_v, mod_v, sem_x, sem_qkv, sem_mod, sem_head, sem_w, sem_o):
    nb1 = S // TM1
    qkv_v = (qkv0_v, qkv1_v)

    def x_cp(i):
        r = pl.ds(i * TM1, TM1)
        return pltpu.make_async_copy(x_hbm.at[r], x_v.at[r], sem_x.at[i])

    def qkv_cp(g, t):
        return pltpu.make_async_copy(wqkv_hbm.at[:, pl.ds(t * D + g * GW, GW)],
                                     wqkv_v.at[g].bitcast(BF16).at[:, pl.ds(t * GW, GW)], sem_qkv.at[g * 3 + t])

    def mod_cp(i):
        return pltpu.make_async_copy(wmod_hbm.at[:, pl.ds(i * D, D)], wmod_v.at[i], sem_mod.at[i])

    def mod_head_cp(i):
        return pltpu.make_async_copy(wmod_hbm.at[:, pl.ds(i * MC, MC)],
                                     wmod_v.at[i * MC // D, :, pl.ds(i * MC % D, MC)], sem_head.at[i])

    w_cps = [pltpu.make_async_copy(s, d, sem_w.at[i]) for i, (s, d) in enumerate(
        ((wo_hbm, wo_v.bitcast(BF16)), (wg_hbm, wg_v.bitcast(BF16)), (wu_hbm, wu_v.bitcast(BF16)), (wd_hbm, wd_v.bitcast(BF16))))]

    def out_cp(i, n):
        cs = pl.ds(pl.multiple_of(n * DC, DC), DC)
        return pltpu.make_async_copy(ob_v.at[n], out_hbm.at[pl.ds(i * TM, TM), cs], sem_o.at[n])

    nm = 2 * D // MC
    head = [mod_head_cp(i) for i in range(nm)] + [x_cp(0)] + [qkv_cp(0, t) for t in range(3)]
    head += [x_cp(i) for i in range(1, nb1)]
    for cp in head[:STAGE[0]]:
        cp.start()

    cf = c_ref[...].astype(F32)
    sc = (cf * jax.nn.sigmoid(cf)).astype(BF16)
    scol_v[...] = jnp.broadcast_to(sc.astype(F32), (128, D)).T
    sc8 = jnp.broadcast_to(sc, (16, D))
    for i in range(nm):
        mod_head_cp(i).wait()
        for cp in head[STAGE[i]:STAGE[i + 1]]:
            cp.start()
        cs = pl.ds(i * MC % D, MC)
        mod_v[i * MC // D, :, cs] = _dot(sc8, wmod_v[i * MC // D, :, cs])[:8]

    def mod_vpu(i, n):
        cs = pl.ds(pl.multiple_of(n * 128, 128), 128)
        p = wmod_v[i, :, cs].astype(F32) * scol_v[...]
        mod_v[i, :, cs] = jnp.broadcast_to(jnp.sum(p, axis=0, keepdims=True), (8, 128))
        yield

    def mod_row(i):
        return mod_v[i, pl.ds(0, 1), :]

    dep = [None]

    def rows(i, n):
        return pl.ds(pl.multiple_of(i * n, n), n)

    def tied(h, i, n):
        k0 = h.shape[1] - n
        late = jnp.tile(lax.bitcast_convert_type(dep[0], U32), (h.shape[0] // 8, n // 128))
        late = jnp.where(i < 0, late, h[:, k0:])
        return jnp.concatenate([h[:, :k0], late], axis=1) if k0 else late

    def proj(g, i, tie=False):
        top, bot = pl.ds(0, HD // 2), pl.ds(HD // 2, HD // 2)
        for t in range(3):
            lhs = [h_v[k, rows(i, HQ // 2), :] for k in range(7)]
            if tie and t == 2:
                lhs = lhs[:TIE] + [tied(h, i, HD) for h in lhs[TIE:]]
            lo, hi = pl.ds(t * 128, 128), pl.ds((3 + t) * 128, 128)
            rhs = (sq_v[g, 0, :, lo], wqkv_v[g, top, lo], wqkv_v[g, top, hi], wqkv_v[g, bot, lo],
                   wqkv_v[g, bot, hi], sq_v[g, 1, :, lo], sq_v[g, 2, :, lo])
            c11, c12, c21, c22 = _strassen(lhs, rhs)
            for n, m, y in ((t, 0, c11), (3 + t, 0, c12), (t, 1, c21), (3 + t, 1, c22)):
                qkv_v[g % 2][n, rows(2 * i + m, HQ // 2), :] = pltpu.bitcast(y.astype(BF16), U32)
            yield

    def prep_qkv(g):
        def step(k, c):
            top, bot = rows(k, 32), rows(HD // 64 + k, 32)
            for t in range(3):
                lo, hi = pl.ds(t * 128, 128), pl.ds((3 + t) * 128, 128)
                s1, s3, s4, s6, s7 = _rhs_terms(wqkv_v[g, top, lo], wqkv_v[g, top, hi],
                                                wqkv_v[g, bot, lo], wqkv_v[g, bot, hi])
                wqkv_v[g, top, hi], wqkv_v[g, bot, lo] = s3, s4
                sq_v[g, 0, top, lo], sq_v[g, 1, top, lo], sq_v[g, 2, top, lo] = s1, s6, s7
            return c
        for t in range(3):
            qkv_cp(g, t).wait()
        lax.fori_loop(0, HD // 64, step, 0)

    def att_load(g, j, u):
        for t, dst in enumerate((q_s, k_s, v_s)):
            for n in range(2):
                w = qkv_v[g % 2][t * 2 + n, pl.ds(j, 128, stride=NJ), :]
                wt = w.T
                for h in range(4):
                    t_v[u * 3 + t, pl.ds((n * 4 + h) * HP, DH), :] = wt[h * DH:(h + 1) * DH]
            for d in range(DH):
                w = t_v[u * 3 + t, pl.ds(d, 8, stride=HP), :]
                r = pl.ds(d * 8, 8)
                if t == 0:
                    dst[0, j, r, :], dst[1, j, r, :] = _unpack(w)
                else:
                    dst[0, NJ + j, r, :], dst[1, NJ + j, r, :] = _unpack(w)
                    dst[0, j, r, :], dst[1, j, r, :] = _unpack(pltpu.roll(w, 1, 1))
            yield

    def att_core(dst, base, j, u):
        qws, ch = CFG[u]
        lane0 = lax.broadcasted_iota(jnp.int32, (8, 128), 1) == 0
        probs = []
        for p in range(2):
            acc = [None] * W
            qw = qws[p]
            for w0 in range(0, W, qw):
                for d in range(DH):
                    r = pl.ds(d * 8, 8)
                    q = q_s[p, j, r, :]
                    if d == 0 and dep[0] is not None:
                        q = jnp.where(j < 0, dep[0], q)
                    for w in range(w0, w0 + qw):
                        t = q * k_s[p, j + (NJ - w), r, :]
                        acc[w] = t if d == 0 else acc[w] + t
                dep[0] = acc[w0]
            lg = [acc[0] * DH ** -0.5]
            for w in range(1, W):
                lg.append(jnp.where(jnp.logical_and(lane0, j < w), -1e9, acc[w] * DH ** -0.5))
            m = lg[0]
            for w in range(1, W):
                m = jnp.maximum(m, lg[w])
            e = [jnp.exp(l - m) for l in lg]
            den = e[0]
            for w in range(1, W):
                den = den + e[w]
            inv = 1.0 / den
            probs.append([x * inv for x in e])
            dep[0] = inv
            yield
        for d in range(DH):
            r = pl.ds(d * 8, 8)
            o = []
            for p in range(2):
                acc = probs[p][0] * v_s[p, j + NJ, r, :]
                for w in range(1, W):
                    acc = acc + probs[p][w] * v_s[p, j + (NJ - w), r, :]
                o.append(acc)
                if d % ch == ch - 1:
                    probs[p][0] = jnp.where(j < 0, acc, probs[p][0])
                    dep[0] = acc
            ot_v[u, pl.ds(d, 8, stride=HP), :] = pltpu.pack_elementwise(o, packed_dtype=BF16)
        for n in range(2):
            ot = jnp.concatenate([ot_v[u, pl.ds((n * 4 + h) * HP, DH), :] for h in range(4)], axis=0)
            dst[base + n, pl.ds(j, 128, stride=NJ), :] = ot.T
        yield

    def o_cols(ref, r):
        return jnp.concatenate([ref[n, r, :] for n in range(ref.shape[0])], axis=1)

    def ln1(i):
        top, bot = (_ln_mod(x_v[rows(2 * i + m, HQ), :].astype(F32), 1.0 + mod_row(1), mod_row(0))
                    for m in range(2))
        for k, t in enumerate(_lhs_terms(top[:, :HD], top[:, HD:], bot[:, :HD], bot[:, HD:])):
            h_v[k, rows(i, HQ // 2), :] = t

    def ln2(blk, n):
        starts = [blk * (TM // LB) + half_ * (HM // LB) + n for half_ in range(2)]
        o = jnp.concatenate([o_cols(o3_v, rows(b, LB // 2)) for b in starts], axis=0)
        y = _dot(pltpu.bitcast(o, BF16), _ld(wo_v, pl.ds((HG - 1) * GW // 2, GW // 2)))
        hs = []
        for k, b in enumerate(starts):
            r = rows(b, LB)
            x1 = x_v[r, :].astype(F32) + mod_row(2) * (x1_v[r, :] + y[k * LB:(k + 1) * LB])
            x2_v[blk % 2, rows(k * (HM // LB) + n, LB), :] = x1
            hs.append(_ln_mod(x1, 1.0 + mod_row(4), mod_row(3)))
        terms = _lhs_terms(hs[0][:, :HD], hs[0][:, HD:], hs[1][:, :HD], hs[1][:, HD:])
        for k, t in enumerate(terms):
            hs_v[k, rows(n, LB // 2), :] = t

    def prep_gate_up(step):
        n = HD // 16
        top, bot = rows(step, n), rows(8 + step, n)
        for k in range(F // PC):
            cs = pl.ds(k * PC, PC)
            s1, s3, s4, s6, s7 = _rhs_terms(wg_v[top, cs], wu_v[top, cs], wg_v[bot, cs], wu_v[bot, cs])
            wu_v[top, cs], wg_v[bot, cs] = s3, s4
            sg_v[0, top, cs], sg_v[1, top, cs], sg_v[2, top, cs] = s1, s6, s7

    def prep_down(step):
        steps = HF // FC
        n = HF // 16 // steps
        lo, hi = pl.ds(0, HD), pl.ds(HD, HD)
        for k in range(n):
            top, bot = rows(step * n + k, 8), rows((steps + step) * n + k, 8)
            s1, s3, s4, s6, s7 = _rhs_terms(wd_v[top, lo], wd_v[top, hi], wd_v[bot, lo], wd_v[bot, hi])
            wd_v[top, hi], wd_v[bot, lo] = s3, s4
            sd_v[0, top, lo], sd_v[1, top, lo], sd_v[2, top, lo] = s1, s6, s7

    def prefetch(g):
        nxt = [qkv_cp(g + 1, t) for t in range(3)] if g + 1 < HG else []
        for cp in nxt + [mod_cp(g + 2)] + [w_cps[k] for k in ((1,), (2,), (3,), (0,))[g]]:
            cp.start()

    x_cp(0).wait()
    ln1(0)
    prep_qkv(0)
    prefetch(0)

    def first_body(i, carry):
        @pl.when(i + 1 < nb1)
        def _():
            x_cp(i + 1).wait()

        _mix(proj(0, i))
        ln1(jnp.minimum(i + 1, nb1 - 1))
        return carry
    lax.fori_loop(0, nb1, first_body, 0)

    half = nb1 // 2
    jpb = NJ // half

    def loads(g, j0, nj):
        for u in range(nj):
            yield from att_load(g, j0 + u, u)
            if g + 1 < HG:
                yield from mod_vpu(g + 2, j0 + u)

    def cores(g, i):
        dst, base = (o_v, g * 2) if g + 1 < HG else (o3_v, 0)
        for u in range(jpb):
            yield from att_core(dst, base, i * jpb + u, u)

    def wo_part(i, tie=False):
        for n in range(D // GW):
            cs = pl.ds(n * GW, GW)
            o = o_cols(o_v, rows(i, TM1 // 2))
            if tie and n == D // GW - 1:
                o = tied(o, i, TIW)
            x1_v[rows(i, TM1), cs] = _dot(pltpu.bitcast(o, BF16), pltpu.bitcast(wo_v[pl.ds(0, (HG - 1) * GW // 2), cs], BF16))
            yield

    def overlapped(g, matmul, steps, na, prep):
        nj = NJ // na

        def body_a(i, c):
            if prep is not None:
                prep(i)
            _mix(matmul(i), steps, loads(g, i * nj, nj), (4 if g + 1 < HG else 3) * nj)
            return c
        lax.fori_loop(0, na, body_a, 0)

        def body_b(i, carry):
            dep[0] = None
            _mix(cores(g, i))
            _mix(matmul(na + i, True))
            return carry
        lax.fori_loop(0, half, body_b, 0)

    for g in range(1, HG):
        mod_cp(g + 1).wait()
        prefetch(g)
        prep_qkv(g)
        for k in ((), (), (1, 2), ())[g]:
            w_cps[k].wait()
        overlapped(g - 1, lambda i, tie=False, g=g: proj(g, i, tie), 3, half,
                   (None, None, prep_gate_up, lambda i: prep_gate_up(half + i))[g])

    mod_cp(5).wait()
    w_cps[0].wait()
    nd = HD // DC
    nln = HM // LB
    nlate = TM // TM1
    overlapped(HG - 1, wo_part, D // GW, half - nlate, None)

    def late_body(i, c):
        for k in range(nln // nlate):
            ln2(0, i * (nln // nlate) + k)
        _mix(wo_part(nb1 - nlate + i))
        return c
    lax.fori_loop(0, nlate, late_body, 0)

    nb = S // TM
    w_cps[3].wait()

    def ffn_body(i, c):
        def gu(f, with_prep):
            if with_prep:
                prep_down(f)
                for k in range(2):
                    _mix(mod_vpu(5, 2 * jnp.minimum(f, NJ // 2 - 1) + k))
            for q in range(FC // 128):
                act = []
                for half_ in range(2):
                    cs = rows((half_ * (HF // FC) + f) * (FC // 128) + q, 128)
                    top, bot = pl.ds(0, HD // 2), pl.ds(HD // 2, HD // 2)
                    rhs = (sg_v[0, :, cs], wg_v[top, cs], wu_v[top, cs], wg_v[bot, cs], wu_v[bot, cs],
                           sg_v[1, :, cs], sg_v[2, :, cs])
                    g_top, u_top, g_bot, u_bot = _strassen([hs_v[k] for k in range(7)], rhs)
                    act.append((g_top * jax.nn.sigmoid(g_top) * u_top, g_bot * jax.nn.sigmoid(g_bot) * u_bot))
                for k, t in enumerate(_lhs_terms(act[0][0], act[1][0], act[0][1], act[1][1])):
                    as_v[k, :, rows(f * (FC // 128) + q, 128)] = t

        @pl.when(i == 0)
        def _():
            lax.fori_loop(0, HF // FC, lambda f, c2: gu(f, True), None)

        @pl.when(i > 0)
        def _():
            lax.fori_loop(0, HF // FC, lambda f, c2: gu(f, False), None)

        @pl.when(i >= 1)
        def _():
            for n in range(2 * nd):
                out_cp(i - 1, n).wait()

        def dn(n, with_ln):
            if with_ln:
                for k in range(nln // nd):
                    ln2(i + 1, n * (nln // nd) + k)
            lo, hi = rows(n, DC), rows(nd + n, DC)
            top, bot = pl.ds(0, HF // 2), pl.ds(HF // 2, HF // 2)
            rhs = (sd_v[0, :, lo], wd_v[top, lo], wd_v[top, hi], wd_v[bot, lo], wd_v[bot, hi],
                   sd_v[1, :, lo], sd_v[2, :, lo])
            c11, c12, c21, c22 = _strassen([as_v[k] for k in range(7)], rhs)
            for m, cs, y_top, y_bot in ((n, lo, c11, c21), (nd + n, hi, c12, c22)):
                gate = mod_v[5, pl.ds(0, 1), cs]
                for r, y in ((pl.ds(0, HM), y_top), (pl.ds(HM, HM), y_bot)):
                    ob_v[m, r, :] = (x2_v[i % 2, r, cs] + gate * y).astype(BF16)
            out_cp(i, n).start()
            out_cp(i, nd + n).start()

        @pl.when(i < nb - 1)
        def _():
            lax.fori_loop(0, nd, lambda n, c2: dn(n, True), None)

        @pl.when(i == nb - 1)
        def _():
            lax.fori_loop(0, nd, lambda n, c2: dn(n, False), None)
        return c
    lax.fori_loop(0, nb, ffn_body, 0)
    for n in range(2 * nd):
        out_cp(nb - 1, n).wait()


@jax.jit
def pallas_adaLN_cond__sliding_local_dilated__swiglu_ffn__prompt_kernel(
    A_x: jax.Array,
    A_wqkv: jax.Array,
    A_wo: jax.Array,
    B_x: jax.Array,
    B_w_gate: jax.Array,
    B_w_up: jax.Array,
    B_w_down: jax.Array,
    c: jax.Array,
    w_mod: jax.Array,
):
    del B_x
    hbm = pl.BlockSpec(memory_space=pl.ANY)
    dma = pltpu.SemaphoreType.DMA
    out = pl.pallas_call(
        _kernel,
        out_shape=jax.ShapeDtypeStruct((S, D), BF16),
        in_specs=[hbm] * 6 + [pl.BlockSpec(memory_space=pltpu.VMEM), hbm],
        out_specs=hbm,
        scratch_shapes=[
            pltpu.VMEM((S, D), BF16),
            pltpu.VMEM((HG, D // 2, 3 * GW), U32),
            pltpu.VMEM((D // 2, D), U32),
            pltpu.VMEM((D // 2, F), U32),
            pltpu.VMEM((D // 2, F), U32),
            pltpu.VMEM((F // 2, D), U32),
            pltpu.VMEM((6, D, D), BF16),
            pltpu.VMEM((7, S // 4, HD), U32),
            pltpu.VMEM((HG, 3, HD // 2, 3 * 128), U32),
            pltpu.VMEM((6, S // 2, 128), U32),
            pltpu.VMEM((6, S // 2, 128), U32),
            pltpu.VMEM((12, 8 * HP, 128), U32),
            pltpu.VMEM((2, NJ, GW, 128), F32),
            pltpu.VMEM((2, 2 * NJ, GW, 128), F32),
            pltpu.VMEM((2, 2 * NJ, GW, 128), F32),
            pltpu.VMEM((2, 8 * HP, 128), U32),
            pltpu.VMEM((2 * HG - 2, S // 2, 128), U32),
            pltpu.VMEM((2, S // 2, 128), U32),
            pltpu.VMEM((S, D), F32),
            pltpu.VMEM((2, TM, D), F32),
            pltpu.VMEM((7, HM // 2, HD), U32),
            pltpu.VMEM((7, HM // 2, HF), U32),
            pltpu.VMEM((3, HD // 2, F), U32),
            pltpu.VMEM((3, HF // 2, HD), U32),
            pltpu.VMEM((D // DC, TM, DC), BF16),
            pltpu.VMEM((D, 128), F32),
            pltpu.VMEM((6, 8, D), F32),
            dma((S // TM1,)), dma((HG * 3,)), dma((6,)), dma((2 * D // MC,)), dma((4,)), dma((D // DC,)),
        ],
        compiler_params=pltpu.CompilerParams(vmem_limit_bytes=120 * 1024 * 1024,
            flags={"XLA_TPU_EVENLY_DISTRIBUTE_CRITICAL_NODES": True}),
    )(A_x.reshape(S, D), A_wqkv, A_wo, B_w_gate, B_w_up, B_w_down, c, w_mod)
    return out.reshape(1, S, D)
```

```python
import jax
import jax.numpy as jnp
from jax import lax
from jax.experimental import pallas as pl
from jax.experimental.pallas import tpu as pltpu

S, D, F = 2048, 1024, 3584
DH, W = 32, 8
HG, GW = 4, 256
NJ = 8
TM1 = 256
TM = 512
FC = 256
DC = 128
HM, HD, HF = TM // 2, D // 2, F // 2
HQ = TM1 // 2
LB = 64
HP = 36
CFG = (((2, 4), 1), ((2, 4), 1))
MC = 512
STAGE = (4, 4, 6, 8, 99)
TIE, TIW = 4, 768
PC = 128
EPS = 1e-5
F32, BF16, U32 = jnp.float32, jnp.bfloat16, jnp.uint32


def _dot(a, b):
    return jnp.dot(a, b, preferred_element_type=F32)


def _ln_mod(x, scale1, shift):
    m = jnp.mean(x, axis=-1, keepdims=True)
    xc = x - m
    v = jnp.mean(xc * xc, axis=-1, keepdims=True)
    return xc * lax.rsqrt(v + EPS) * scale1 + shift


def _unpack(w):
    lo = lax.bitcast_convert_type(w << 16, F32)
    hi = lax.bitcast_convert_type(w & jnp.uint32(0xFFFF0000), F32)
    return lo, hi


def _ld(ref, r):
    return pltpu.bitcast(ref[r, :], BF16)


def _mix(a, na=1, b=(), nb=0):
    b = iter(b)
    done = 0
    for k, _ in enumerate(a):
        while done * na < (k + 1) * nb:
            next(b)
            done += 1
    for _ in b:
        pass


def _lhs_terms(a11, a12, a21, a22):
    terms = (a11 + a22, a21 + a22, a11, a22, a11 + a12, a21 - a11, a12 - a22)
    return [pltpu.bitcast(t.astype(BF16), U32) for t in terms]


def _rhs_terms(b11, b12, b21, b22):
    halves = [(b11 + b22, b12 - b22, b21 - b11, b11 + b12, b21 + b22)
              for b11, b12, b21, b22 in zip(*(_unpack(b) for b in (b11, b12, b21, b22)))]
    return [pltpu.pack_elementwise([lo, hi], packed_dtype=BF16) for lo, hi in zip(*halves)]


def _strassen(lhs, rhs):
    def p(k):
        return _dot(pltpu.bitcast(lhs[k - 1], BF16), pltpu.bitcast(rhs[k - 1], BF16))
    p1, p4, p5, p7, p2, p3, p6 = (p(k) for k in (1, 4, 5, 7, 2, 3, 6))
    return p1 + p4 - p5 + p7, p3 + p5, p2 + p4, p1 - p2 + p3 + p6


def _kernel(x_hbm, wqkv_hbm, wo_hbm, wg_hbm, wu_hbm, wd_hbm, c_ref, wmod_hbm, out_hbm,
            x_v, wqkv_v, wo_v, wg_v, wu_v, wd_v, wmod_v, h_v, sq_v, qkv0_v, qkv1_v, t_v, q_s, k_s, v_s,
            ot_v, o_v, o3_v, x1_v, x2_v, hs_v, as_v, sg_v, sd_v, ob_v, scol_v, mod_v, sem_x, sem_qkv, sem_mod, sem_head, sem_w, sem_o):
    nb1 = S // TM1
    qkv_v = (qkv0_v, qkv1_v)

    def x_cp(i):
        r = pl.ds(i * TM1, TM1)
        return pltpu.make_async_copy(x_hbm.at[r], x_v.at[r], sem_x.at[i])

    def qkv_cp(g, t):
        return pltpu.make_async_copy(wqkv_hbm.at[:, pl.ds(t * D + g * GW, GW)],
                                     wqkv_v.at[g, t].bitcast(BF16), sem_qkv.at[g * 3 + t])

    def mod_cp(i):
        return pltpu.make_async_copy(wmod_hbm.at[:, pl.ds(i * D, D)], wmod_v.at[i], sem_mod.at[i])

    def mod_head_cp(i):
        return pltpu.make_async_copy(wmod_hbm.at[:, pl.ds(i * MC, MC)],
                                     wmod_v.at[i * MC // D, :, pl.ds(i * MC % D, MC)], sem_head.at[i])

    w_cps = [pltpu.make_async_copy(s, d, sem_w.at[i]) for i, (s, d) in enumerate(
        ((wo_hbm, wo_v.bitcast(BF16)), (wg_hbm, wg_v.bitcast(BF16)), (wu_hbm, wu_v.bitcast(BF16)), (wd_hbm, wd_v.bitcast(BF16))))]

    def out_cp(i, n):
        cs = pl.ds(pl.multiple_of(n * DC, DC), DC)
        return pltpu.make_async_copy(ob_v.at[n], out_hbm.at[pl.ds(i * TM, TM), cs], sem_o.at[n])

    nm = 2 * D // MC
    head = [mod_head_cp(i) for i in range(nm)] + [x_cp(0)] + [qkv_cp(0, t) for t in range(3)]
    head += [x_cp(i) for i in range(1, nb1)]
    for cp in head[:STAGE[0]]:
        cp.start()

    cf = c_ref[...].astype(F32)
    sc = (cf * jax.nn.sigmoid(cf)).astype(BF16)
    scol_v[...] = jnp.broadcast_to(sc.astype(F32), (128, D)).T
    sc8 = jnp.broadcast_to(sc, (16, D))
    for i in range(nm):
        mod_head_cp(i).wait()
        for cp in head[STAGE[i]:STAGE[i + 1]]:
            cp.start()
        cs = pl.ds(i * MC % D, MC)
        mod_v[i * MC // D, :, cs] = _dot(sc8, wmod_v[i * MC // D, :, cs])[:8]

    def mod_vpu(i, n):
        cs = pl.ds(pl.multiple_of(n * 128, 128), 128)
        p = wmod_v[i, :, cs].astype(F32) * scol_v[...]
        mod_v[i, :, cs] = jnp.broadcast_to(jnp.sum(p, axis=0, keepdims=True), (8, 128))
        yield

    def mod_row(i):
        return mod_v[i, pl.ds(0, 1), :]

    dep = [None]

    def rows(i, n):
        return pl.ds(pl.multiple_of(i * n, n), n)

    def tied(h, i, n):
        k0 = h.shape[1] - n
        late = jnp.tile(lax.bitcast_convert_type(dep[0], U32), (h.shape[0] // 8, n // 128))
        late = jnp.where(i < 0, late, h[:, k0:])
        return jnp.concatenate([h[:, :k0], late], axis=1) if k0 else late

    def wq(g, r, n):
        return g, n // 2, r, pl.ds(n % 2 * 128, 128)

    def proj(g, i, tie=False):
        top, bot = pl.ds(0, HD // 2), pl.ds(HD // 2, HD // 2)
        for t in range(3):
            lhs = [h_v[k, rows(i, HQ // 2), :] for k in range(7)]
            if tie and t == 2:
                lhs = lhs[:TIE] + [tied(h, i, HD) for h in lhs[TIE:]]
            lo = pl.ds(t * 128, 128)
            rhs = (sq_v[g, 0, :, lo], wqkv_v[wq(g, top, t)], wqkv_v[wq(g, top, 3 + t)], wqkv_v[wq(g, bot, t)],
                   wqkv_v[wq(g, bot, 3 + t)], sq_v[g, 1, :, lo], sq_v[g, 2, :, lo])
            c11, c12, c21, c22 = _strassen(lhs, rhs)
            for n, m, y in ((t, 0, c11), (3 + t, 0, c12), (t, 1, c21), (3 + t, 1, c22)):
                qkv_v[g % 2][n, rows(2 * i + m, HQ // 2), :] = pltpu.bitcast(y.astype(BF16), U32)
            yield

    def prep_qkv(g):
        def step(k, c):
            top, bot = rows(k, 32), rows(HD // 64 + k, 32)
            for t in range(3):
                lo = pl.ds(t * 128, 128)
                s1, s3, s4, s6, s7 = _rhs_terms(wqkv_v[wq(g, top, t)], wqkv_v[wq(g, top, 3 + t)],
                                                wqkv_v[wq(g, bot, t)], wqkv_v[wq(g, bot, 3 + t)])
                wqkv_v[wq(g, top, 3 + t)], wqkv_v[wq(g, bot, t)] = s3, s4
                sq_v[g, 0, top, lo], sq_v[g, 1, top, lo], sq_v[g, 2, top, lo] = s1, s6, s7
            return c
        for t in range(3):
            qkv_cp(g, t).wait()
        lax.fori_loop(0, HD // 64, step, 0)

    def att_load(g, j, u):
        for t, dst in enumerate((q_s, k_s, v_s)):
            for n in range(2):
                w = qkv_v[g % 2][t * 2 + n, pl.ds(j, 128, stride=NJ), :]
                wt = w.T
                for h in range(4):
                    t_v[u * 3 + t, pl.ds((n * 4 + h) * HP, DH), :] = wt[h * DH:(h + 1) * DH]
            for d in range(DH):
                w = t_v[u * 3 + t, pl.ds(d, 8, stride=HP), :]
                r = pl.ds(d * 8, 8)
                if t == 0:
                    dst[0, j, r, :], dst[1, j, r, :] = _unpack(w)
                else:
                    dst[0, NJ + j, r, :], dst[1, NJ + j, r, :] = _unpack(w)
                    dst[0, j, r, :], dst[1, j, r, :] = _unpack(pltpu.roll(w, 1, 1))
            yield

    def att_core(dst, base, j, u):
        qws, ch = CFG[u]
        lane0 = lax.broadcasted_iota(jnp.int32, (8, 128), 1) == 0
        probs = []
        for p in range(2):
            acc = [None] * W
            qw = qws[p]
            for w0 in range(0, W, qw):
                for d in range(DH):
                    r = pl.ds(d * 8, 8)
                    q = q_s[p, j, r, :]
                    if d == 0 and dep[0] is not None:
                        q = jnp.where(j < 0, dep[0], q)
                    for w in range(w0, w0 + qw):
                        t = q * k_s[p, j + (NJ - w), r, :]
                        acc[w] = t if d == 0 else acc[w] + t
                dep[0] = acc[w0]
            lg = [acc[0] * DH ** -0.5]
            for w in range(1, W):
                lg.append(jnp.where(jnp.logical_and(lane0, j < w), -1e9, acc[w] * DH ** -0.5))
            m = lg[0]
            for w in range(1, W):
                m = jnp.maximum(m, lg[w])
            e = [jnp.exp(l - m) for l in lg]
            den = e[0]
            for w in range(1, W):
                den = den + e[w]
            inv = 1.0 / den
            probs.append([x * inv for x in e])
            dep[0] = inv
            yield
        for d in range(DH):
            r = pl.ds(d * 8, 8)
            o = []
            for p in range(2):
                acc = probs[p][0] * v_s[p, j + NJ, r, :]
                for w in range(1, W):
                    acc = acc + probs[p][w] * v_s[p, j + (NJ - w), r, :]
                o.append(acc)
                if d % ch == ch - 1:
                    probs[p][0] = jnp.where(j < 0, acc, probs[p][0])
                    dep[0] = acc
            ot_v[u, pl.ds(d, 8, stride=HP), :] = pltpu.pack_elementwise(o, packed_dtype=BF16)
        for n in range(2):
            ot = jnp.concatenate([ot_v[u, pl.ds((n * 4 + h) * HP, DH), :] for h in range(4)], axis=0)
            dst[base + n, pl.ds(j, 128, stride=NJ), :] = ot.T
        yield

    def o_cols(ref, r):
        return jnp.concatenate([ref[n, r, :] for n in range(ref.shape[0])], axis=1)

    def ln1(i):
        top, bot = (_ln_mod(x_v[rows(2 * i + m, HQ), :].astype(F32), 1.0 + mod_row(1), mod_row(0))
                    for m in range(2))
        for k, t in enumerate(_lhs_terms(top[:, :HD], top[:, HD:], bot[:, :HD], bot[:, HD:])):
            h_v[k, rows(i, HQ // 2), :] = t

    def ln2(blk, n):
        starts = [blk * (TM // LB) + half_ * (HM // LB) + n for half_ in range(2)]
        o = jnp.concatenate([o_cols(o3_v, rows(b, LB // 2)) for b in starts], axis=0)
        y = _dot(pltpu.bitcast(o, BF16), _ld(wo_v, pl.ds((HG - 1) * GW // 2, GW // 2)))
        hs = []
        for k, b in enumerate(starts):
            r = rows(b, LB)
            x1 = x_v[r, :].astype(F32) + mod_row(2) * (x1_v[r, :] + y[k * LB:(k + 1) * LB])
            x2_v[blk % 2, rows(k * (HM // LB) + n, LB), :] = x1
            hs.append(_ln_mod(x1, 1.0 + mod_row(4), mod_row(3)))
        terms = _lhs_terms(hs[0][:, :HD], hs[0][:, HD:], hs[1][:, :HD], hs[1][:, HD:])
        for k, t in enumerate(terms):
            hs_v[k, rows(n, LB // 2), :] = t

    def prep_gate_up(step):
        n = HD // 16
        top, bot = rows(step, n), rows(8 + step, n)
        for k in range(F // PC):
            cs = pl.ds(k * PC, PC)
            s1, s3, s4, s6, s7 = _rhs_terms(wg_v[top, cs], wu_v[top, cs], wg_v[bot, cs], wu_v[bot, cs])
            wu_v[top, cs], wg_v[bot, cs] = s3, s4
            sg_v[0, top, cs], sg_v[1, top, cs], sg_v[2, top, cs] = s1, s6, s7

    def prep_down(step):
        steps = HF // FC
        n = HF // 16 // steps
        lo, hi = pl.ds(0, HD), pl.ds(HD, HD)
        for k in range(n):
            top, bot = rows(step * n + k, 8), rows((steps + step) * n + k, 8)
            s1, s3, s4, s6, s7 = _rhs_terms(wd_v[top, lo], wd_v[top, hi], wd_v[bot, lo], wd_v[bot, hi])
            wd_v[top, hi], wd_v[bot, lo] = s3, s4
            sd_v[0, top, lo], sd_v[1, top, lo], sd_v[2, top, lo] = s1, s6, s7

    def prefetch(g):
        nxt = [qkv_cp(g + 1, t) for t in range(3)] if g + 1 < HG else []
        for cp in nxt + [mod_cp(g + 2)] + [w_cps[k] for k in ((1,), (2,), (3,), (0,))[g]]:
            cp.start()

    x_cp(0).wait()
    ln1(0)
    prep_qkv(0)
    prefetch(0)

    def first_body(i, carry):
        @pl.when(i + 1 < nb1)
        def _():
            x_cp(i + 1).wait()

        _mix(proj(0, i))
        ln1(jnp.minimum(i + 1, nb1 - 1))
        return carry
    lax.fori_loop(0, nb1, first_body, 0)

    half = nb1 // 2
    jpb = NJ // half

    def loads(g, j0, nj):
        for u in range(nj):
            yield from att_load(g, j0 + u, u)
            if g + 1 < HG:
                yield from mod_vpu(g + 2, j0 + u)

    def cores(g, i):
        dst, base = (o_v, g * 2) if g + 1 < HG else (o3_v, 0)
        for u in range(jpb):
            yield from att_core(dst, base, i * jpb + u, u)

    def wo_part(i, tie=False):
        for n in range(D // GW):
            cs = pl.ds(n * GW, GW)
            o = o_cols(o_v, rows(i, TM1 // 2))
            if tie and n == D // GW - 1:
                o = tied(o, i, TIW)
            x1_v[rows(i, TM1), cs] = _dot(pltpu.bitcast(o, BF16), pltpu.bitcast(wo_v[pl.ds(0, (HG - 1) * GW // 2), cs], BF16))
            yield

    def overlapped(g, matmul, steps, na, prep):
        nj = NJ // na

        def body_a(i, c):
            if prep is not None:
                prep(i)
            _mix(matmul(i), steps, loads(g, i * nj, nj), (4 if g + 1 < HG else 3) * nj)
            return c
        lax.fori_loop(0, na, body_a, 0)

        def body_b(i, carry):
            dep[0] = None
            _mix(cores(g, i))
            _mix(matmul(na + i, True))
            return carry
        lax.fori_loop(0, half, body_b, 0)

    for g in range(1, HG):
        mod_cp(g + 1).wait()
        prefetch(g)
        prep_qkv(g)
        for k in ((), (), (1, 2), ())[g]:
            w_cps[k].wait()
        overlapped(g - 1, lambda i, tie=False, g=g: proj(g, i, tie), 3, half,
                   (None, None, prep_gate_up, lambda i: prep_gate_up(half + i))[g])

    mod_cp(5).wait()
    w_cps[0].wait()
    nd = HD // DC
    nln = HM // LB
    nlate = TM // TM1
    overlapped(HG - 1, wo_part, D // GW, half - nlate, None)

    def late_body(i, c):
        for k in range(nln // nlate):
            ln2(0, i * (nln // nlate) + k)
        _mix(wo_part(nb1 - nlate + i))
        return c
    lax.fori_loop(0, nlate, late_body, 0)

    nb = S // TM
    w_cps[3].wait()

    def ffn_body(i, c):
        def gu(f, with_prep):
            if with_prep:
                prep_down(f)
                for k in range(2):
                    _mix(mod_vpu(5, 2 * jnp.minimum(f, NJ // 2 - 1) + k))
            for q in range(FC // 128):
                act = []
                for half_ in range(2):
                    cs = rows((half_ * (HF // FC) + f) * (FC // 128) + q, 128)
                    top, bot = pl.ds(0, HD // 2), pl.ds(HD // 2, HD // 2)
                    rhs = (sg_v[0, :, cs], wg_v[top, cs], wu_v[top, cs], wg_v[bot, cs], wu_v[bot, cs],
                           sg_v[1, :, cs], sg_v[2, :, cs])
                    g_top, u_top, g_bot, u_bot = _strassen([hs_v[k] for k in range(7)], rhs)
                    act.append((g_top * jax.nn.sigmoid(g_top) * u_top, g_bot * jax.nn.sigmoid(g_bot) * u_bot))
                for k, t in enumerate(_lhs_terms(act[0][0], act[1][0], act[0][1], act[1][1])):
                    as_v[k, :, rows(f * (FC // 128) + q, 128)] = t

        @pl.when(i == 0)
        def _():
            lax.fori_loop(0, HF // FC, lambda f, c2: gu(f, True), None)

        @pl.when(i > 0)
        def _():
            lax.fori_loop(0, HF // FC, lambda f, c2: gu(f, False), None)

        @pl.when(i >= 1)
        def _():
            for n in range(2 * nd):
                out_cp(i - 1, n).wait()

        def dn(n, with_ln):
            if with_ln:
                for k in range(nln // nd):
                    ln2(i + 1, n * (nln // nd) + k)
            lo, hi = rows(n, DC), rows(nd + n, DC)
            top, bot = pl.ds(0, HF // 2), pl.ds(HF // 2, HF // 2)
            rhs = (sd_v[0, :, lo], wd_v[top, lo], wd_v[top, hi], wd_v[bot, lo], wd_v[bot, hi],
                   sd_v[1, :, lo], sd_v[2, :, lo])
            c11, c12, c21, c22 = _strassen([as_v[k] for k in range(7)], rhs)
            for m, cs, y_top, y_bot in ((n, lo, c11, c21), (nd + n, hi, c12, c22)):
                gate = mod_v[5, pl.ds(0, 1), cs]
                for r, y in ((pl.ds(0, HM), y_top), (pl.ds(HM, HM), y_bot)):
                    ob_v[m, r, :] = (x2_v[i % 2, r, cs] + gate * y).astype(BF16)
            out_cp(i, n).start()
            out_cp(i, nd + n).start()

        @pl.when(i < nb - 1)
        def _():
            lax.fori_loop(0, nd, lambda n, c2: dn(n, True), None)

        @pl.when(i == nb - 1)
        def _():
            lax.fori_loop(0, nd, lambda n, c2: dn(n, False), None)
        return c
    lax.fori_loop(0, nb, ffn_body, 0)
    for n in range(2 * nd):
        out_cp(nb - 1, n).wait()


@jax.jit
def pallas_adaLN_cond__sliding_local_dilated__swiglu_ffn__prompt_kernel(
    A_x: jax.Array,
    A_wqkv: jax.Array,
    A_wo: jax.Array,
    B_x: jax.Array,
    B_w_gate: jax.Array,
    B_w_up: jax.Array,
    B_w_down: jax.Array,
    c: jax.Array,
    w_mod: jax.Array,
):
    del B_x
    hbm = pl.BlockSpec(memory_space=pl.ANY)
    dma = pltpu.SemaphoreType.DMA
    out = pl.pallas_call(
        _kernel,
        out_shape=jax.ShapeDtypeStruct((S, D), BF16),
        in_specs=[hbm] * 6 + [pl.BlockSpec(memory_space=pltpu.VMEM), hbm],
        out_specs=hbm,
        scratch_shapes=[
            pltpu.VMEM((S, D), BF16),
            pltpu.VMEM((HG, 3, D // 2, GW), U32),
            pltpu.VMEM((D // 2, D), U32),
            pltpu.VMEM((D // 2, F), U32),
            pltpu.VMEM((D // 2, F), U32),
            pltpu.VMEM((F // 2, D), U32),
            pltpu.VMEM((6, D, D), BF16),
            pltpu.VMEM((7, S // 4, HD), U32),
            pltpu.VMEM((HG, 3, HD // 2, 3 * 128), U32),
            pltpu.VMEM((6, S // 2, 128), U32),
            pltpu.VMEM((6, S // 2, 128), U32),
            pltpu.VMEM((12, 8 * HP, 128), U32),
            pltpu.VMEM((2, NJ, GW, 128), F32),
            pltpu.VMEM((2, 2 * NJ, GW, 128), F32),
            pltpu.VMEM((2, 2 * NJ, GW, 128), F32),
            pltpu.VMEM((2, 8 * HP, 128), U32),
            pltpu.VMEM((2 * HG - 2, S // 2, 128), U32),
            pltpu.VMEM((2, S // 2, 128), U32),
            pltpu.VMEM((S, D), F32),
            pltpu.VMEM((2, TM, D), F32),
            pltpu.VMEM((7, HM // 2, HD), U32),
            pltpu.VMEM((7, HM // 2, HF), U32),
            pltpu.VMEM((3, HD // 2, F), U32),
            pltpu.VMEM((3, HF // 2, HD), U32),
            pltpu.VMEM((D // DC, TM, DC), BF16),
            pltpu.VMEM((D, 128), F32),
            pltpu.VMEM((6, 8, D), F32),
            dma((S // TM1,)), dma((HG * 3,)), dma((6,)), dma((2 * D // MC,)), dma((4,)), dma((D // DC,)),
        ],
        compiler_params=pltpu.CompilerParams(vmem_limit_bytes=120 * 1024 * 1024,
            flags={"XLA_TPU_EVENLY_DISTRIBUTE_CRITICAL_NODES": True}),
    )(A_x.reshape(S, D), A_wqkv, A_wo, B_w_gate, B_w_up, B_w_down, c, w_mod)
    return out.reshape(1, S, D)
```
